```python
import jax
import jax.numpy as jnp

def _softmax(x, axis=-1):
    return jax.nn.softmax(x, axis=axis)

def _gelu(x):
    return jax.nn.gelu(x, approximate=True)

def _silu(x):
    return jax.nn.silu(x)

def _sigmoid(x):
    return jax.nn.sigmoid(x)

def _layernorm(x, axis=-1, eps=1e-05):
    m = jnp.mean(x, axis=axis, keepdims=True)
    v = jnp.var(x, axis=axis, keepdims=True)
    return (x - m) / jnp.sqrt(v + eps)

def _scatter_add(tgt, idx, src, axis=0):
    return tgt.at[idx].add(src)

def _segment_sum(src, seg, n):
    return jax.ops.segment_sum(src, seg, n)

class _Rng:

    def __init__(self, key):
        self._k = key

    def _next(self):
        self._k, sub = jax.random.split(self._k)
        return sub

    def normal(self, shape):
        return jax.random.normal(self._next(), shape, dtype=jnp.bfloat16)

    def randint(self, lo, hi, shape):
        return jax.random.randint(self._next(), shape, lo, hi, dtype=jnp.int32)

    def uniform(self, shape, lo=0.0, hi=1.0):
        return jax.random.uniform(self._next(), shape, jnp.bfloat16, lo, hi)

    def permutation(self, n):
        return jax.random.permutation(self._next(), n)
kernel_name = 'parallel_sum__memory_aug_infini_attn__moe_arch_mod__prompt'

def setup_inputs():
    _rng = _Rng(jax.random.key(int.from_bytes(__import__("os").urandom(4), "little")))
    _w = lambda a: (lambda t: t.astype(jnp.bfloat16) if jnp.issubdtype(t.dtype, jnp.floating) else t)(jnp.asarray(a))

    def _A_setup():
        B, S, D, H = (1, 2048, 576, 32)
        N = 4
        L = max(1, S // N)
        sc = D ** (-0.5)
        return {'x': _w((lambda *s: _rng.normal(s) * 0.05)(B, N * L, D)), 'wq': _w((lambda *s: _rng.normal(s) * 0.05)(D, D) * sc), 'wk': _w((lambda *s: _rng.normal(s) * 0.05)(D, D) * sc), 'wv': _w((lambda *s: _rng.normal(s) * 0.05)(D, D) * sc), 'wo': _w((lambda *s: _rng.normal(s) * 0.05)(D, D) * sc), 'beta': _w((lambda *s: _rng.normal(s) * 0.05)(H))}
    _A_in = _A_setup()

    def _B_setup():
        B, S, D, F, C = (1, 2048, 576, 4608, 2)
        return {'x': _w((lambda *s: _rng.normal(s) * 0.05)(B, S, D)), 'w_r': _w((lambda *s: _rng.normal(s) * 0.05)(D)), 'w_gate': _w((lambda *s: _rng.normal(s) * 0.05)(D, F)), 'w_up': _w((lambda *s: _rng.normal(s) * 0.05)(D, F)), 'w_down': _w((lambda *s: _rng.normal(s) * 0.05)(F, D))}
    _B_in = _B_setup()
    return {'A_x': _A_in['x'], 'A_wq': _A_in['wq'], 'A_wk': _A_in['wk'], 'A_wv': _A_in['wv'], 'A_wo': _A_in['wo'], 'A_beta': _A_in['beta'], 'B_x': _B_in['x'], 'B_w_r': _B_in['w_r'], 'B_w_gate': _B_in['w_gate'], 'B_w_up': _B_in['w_up'], 'B_w_down': _B_in['w_down']}

def reference(A_x, A_wq, A_wk, A_wv, A_wo, A_beta, B_x, B_w_r, B_w_gate, B_w_up, B_w_down):

    def _A_ref(x, wq, wk, wv, wo, beta):
        B, S, D = x.shape
        H = 32
        Dh = D // H
        N = 4
        L = S // N
        q = (lambda x, *d: x.transpose(*d))((x @ wq).reshape(B, S, H, Dh), 0, 2, 1, 3).reshape(B, H, N, L, Dh)
        k = (lambda x, *d: x.transpose(*d))((x @ wk).reshape(B, S, H, Dh), 0, 2, 1, 3).reshape(B, H, N, L, Dh)
        v = (lambda x, *d: x.transpose(*d))((x @ wv).reshape(B, S, H, Dh), 0, 2, 1, 3).reshape(B, H, N, L, Dh)
        phi = lambda t: jnp.where(t > 0, t + 1.0, jnp.exp(t))
        scale = Dh ** (-0.5)
        ar = jnp.arange(L)
        mask = (lambda x, dt: x.astype(dt))(ar[:, None] < ar[None, :], x.dtype) * -1000000000.0
        g = _sigmoid(beta).reshape(1, H, 1, 1)
        M = jnp.einsum('bhd,bhe->bhde', q[:, :, 0, 0, :] * 0.0, q[:, :, 0, 0, :] * 0.0)
        z = q[:, :, 0, 0, :] * 0.0
        outs = []
        for s in range(N):
            qs, ks, vs = (q[:, :, s].copy(), k[:, :, s].copy(), v[:, :, s].copy())
            logits = jnp.einsum('bhqd,bhkd->bhqk', qs, ks) * scale + mask
            p = _softmax(logits, axis=-1)
            a_dot = jnp.einsum('bhqk,bhkd->bhqd', p, vs)
            pq = phi(qs)
            num = jnp.einsum('bhld,bhde->bhle', pq, M)
            den = jnp.einsum('bhld,bhd->bhl', pq, z)[..., None] + 1e-06
            a_mem = num / den
            o = g * a_mem + (1.0 - g) * a_dot
            outs.append(o)
            pk = phi(ks)
            M = M + jnp.einsum('bhld,bhle->bhde', pk, vs)
            z = z + jnp.einsum('bhld->bhd', pk)
        o = (lambda x, *d: x.transpose(*d))(jnp.stack(outs, 2).reshape(B, H, S, Dh), 0, 2, 1, 3).reshape(B, S, D)
        return o @ wo

    def _B_ref(x, w_r, w_gate, w_up, w_down):
        B, S, D = x.shape
        C = 2
        r = x @ w_r
        idx = jnp.argsort(-r, axis=-1)[:, :C]
        idx_e = jnp.repeat(idx.reshape(B, C, 1), D, axis=2)
        x_sel = jnp.take_along_axis(x, idx_e, axis=1)
        g = _silu(x_sel @ w_gate)
        u = x_sel @ w_up
        y = g * u @ w_down
        r_sel = _sigmoid(jnp.take_along_axis(r, idx, axis=1))
        y = y * r_sel.reshape(B, C, 1)
        b_off = (jnp.arange(B) * S).reshape(B, 1)
        flat_idx = (idx + b_off).reshape(B * C)
        zero = (x * 0.0).reshape(B * S, D)
        upd = _scatter_add(zero, flat_idx, y.reshape(B * C, D), axis=0)
        return x + upd.reshape(B, S, D)
    x = A_x
    xn = _layernorm(x, axis=-1)
    return x + _A_ref(xn, A_wq, A_wk, A_wv, A_wo, A_beta) + _B_ref(xn, B_w_r, B_w_gate, B_w_up, B_w_down)
```

```python
import math

import jax
import jax.numpy as jnp
from jax import lax
import jax.experimental.pallas as pl
import jax.experimental.pallas.tpu as pltpu

S = 2048
D = 576
H = 32
DH = D // H
NSEG = 4
L = S // NSEG
F = 4608
T = 128
GH = 8
NG = H // GH
GR = GH * DH
WR = GR // 2
QSCALE = (DH ** -0.5) * math.log2(math.e)
NEG = -1e30
SKEW = 12
NS = 32

F32 = jnp.float32
BF16 = jnp.bfloat16
U32 = jnp.uint32
NN = (((1,), (0,)), ((), ()))
NT = (((1,), (1,)), ((), ()))


def _dot(a, b, dims=NN):
    return lax.dot_general(a, b, dims, preferred_element_type=F32)


def _bf(x):
    return pltpu.bitcast(x, BF16)


def _u(x):
    return pltpu.bitcast(x, U32)


def _round(x):
    return x.astype(BF16).astype(F32)


def _phi(t):
    return jnp.where(t > 0, t + 1.0, jnp.exp(t))


def _iota(shape, dim):
    return lax.broadcasted_iota(jnp.int32, shape, dim)


def _kernel(beta_ref, wr_ref, x_hbm, wq_hbm, wk_hbm, wv_hbm, wo_hbm, wg_hbm, wu_hbm, wd_hbm,
            out_hbm,
            x_v, w_v, wg_v, wu_v, wd_v, wt, wot, xn, qs, kn, pq, pk, vv, rr, ot, sc, mem, gt,
            out_v, sem_x, sem_w, sem_f, sem_o):

    def x_copy(s):
        c = pl.ds(s * L, L)
        return pltpu.make_async_copy(x_hbm.at[:, c], x_v.at[:, c], sem_x.at[s])

    def o_copy(s):
        c = pl.ds(s * L, L)
        return pltpu.make_async_copy(out_v.at[:, c], out_hbm.at[:, c], sem_o.at[s])

    w_copies = [pltpu.make_async_copy(w, w_v.at[i], sem_w.at[i])
                for i, w in enumerate((wq_hbm, wk_hbm, wv_hbm, wo_hbm))]
    f_copies = [pltpu.make_async_copy(a, b, sem_f.at[i])
                for i, (a, b) in enumerate(((wg_hbm, wg_v), (wu_hbm, wu_v), (wd_hbm, wd_v)))]

    x_copy(0).start()
    for c in w_copies[:3]:
        c.start()
    for s in range(1, NSEG):
        x_copy(s).start()
    w_copies[3].start()
    for c in f_copies:
        c.start()

    g = jax.nn.sigmoid(beta_ref[...].astype(F32)).reshape(1, H)
    gcol = jnp.sum(jnp.where(_iota((H, H), 0) == _iota((H, H), 1), jnp.broadcast_to(g, (H, H)), 0.0),
                   axis=1, keepdims=True)
    gt[...] = jnp.broadcast_to(gcol, (H, T))
    wr = jnp.broadcast_to(wr_ref[...].astype(F32).reshape(1, D), (16, D)).astype(BF16)
    wt[3 * D // 2:, :] = _u(wr)

    def layernorm(c0):
        for n in range(L // T):
            c = pl.ds(pl.multiple_of(c0 + n * T, T), T)
            x = x_v[:, c].astype(F32)
            mean = jnp.sum(x, axis=0, keepdims=True) * (1.0 / D)
            xc = x - mean
            var = jnp.sum(xc * xc, axis=0, keepdims=True) * (1.0 / D)
            sd = _round(jnp.sqrt(_round(_round(var) + _round(jnp.full((1, T), 1e-5, F32)))))
            y = _round(x - _round(mean)) * (1.0 / sd)
            xn[:, c] = _u(y.astype(BF16))

    def project(s):
        c = pl.ds(pl.multiple_of(s * L, L), L)
        rhs = _bf(xn[:, c])
        q = _dot(_bf(wt[0:D // 2, :]), rhs)
        qs[:, c] = _u((q * QSCALE).astype(BF16))
        pq[:, c] = _phi(q)
        k = _dot(_bf(wt[D // 2:D, :]), rhs)
        pk[:, c] = _phi(k)
        kb = _u(k.astype(BF16))
        for gi in range(NG):
            for w in range(2):
                r0 = gi * WR + 8 * w
                for n in range(L // T):
                    blk = _bf(kb[r0:r0 + T // 2, n * T:(n + 1) * T])
                    kn[2 * gi + w, pl.ds(pl.multiple_of(s * (L // 2) + n * (T // 2), T // 2), T // 2), :] = _u(blk.T)
        vr = _dot(_bf(wt[D:, :]), rhs)
        vv[:, c] = vr[0:D]
        rr[:, c] = vr[D:D + 8]

    x_copy(0).wait()
    layernorm(0)
    for i in range(3):
        w_copies[i].wait()
        wt[i * D // 2:(i + 1) * D // 2, :] = _u(w_v[i].T)

    def phase1(s, carry):
        x_copy(s + 1).wait()
        layernorm((s + 1) * L)
        project(s)
        return carry

    lax.fori_loop(0, NSEG - 1, phase1, 0)
    project(NSEG - 1)

    r = _round(rr[...])
    pos = _iota((8, S), 1).astype(F32)
    r0 = jnp.max(r)
    i0 = jnp.min(jnp.where(r == r0, pos, float(S)))
    r_rest = jnp.where(pos == i0, -jnp.inf, r)
    r1 = jnp.max(r_rest)
    i1 = jnp.min(jnp.where((r_rest == r1) & (pos != i0), pos, float(S)))
    idx = [jnp.clip(i.astype(jnp.int32), 0, S - 1) for i in (i0, i1)]

    xsel = None
    for t in range(2):
        tile = idx[t] // T
        onehot = ((_iota((8, T), 0) == t) & (_iota((8, T), 1) == idx[t] - tile * T)).astype(F32)
        part = _dot(onehot, _bf(xn[:, pl.ds(pl.multiple_of(tile * T, T), T)]), NT)
        xsel = part if xsel is None else xsel + part

    for c in f_copies:
        c.wait()
    w_copies[3].wait()
    FC = 512

    def ffn(i, y):
        c = pl.ds(pl.multiple_of(i * FC, FC), FC)
        a = _dot(xsel, wg_v[:, c])
        b = _dot(xsel, wu_v[:, c])
        hid = a * jax.nn.sigmoid(a) * b
        return y + _dot(hid, wd_v[:, c], NT)

    y = lax.fori_loop(0, F // FC, ffn, jnp.zeros((8, D), F32))
    gate = jax.nn.sigmoid(jnp.where(_iota((8, D), 0) == 0, r0, r1))
    y = jnp.where(_iota((8, D), 0) < 2, y * gate, 0.0)
    wot[:, 0:4 * T] = _u(w_v[3, 0:4 * T, :].T)
    tail = jnp.concatenate(
        [w_v[3, 4 * T:D, :], jnp.concatenate([y, jnp.zeros((8, D), F32)], axis=0).astype(BF16)], axis=0)
    wot[:, 4 * T:] = _u(tail.T)

    causal = _iota((T, T), 0) <= _iota((T, T), 1)
    tiles = [(h, j, i) for h in range(GH) for j in range(L // T) for i in range(j + 1)]

    def attend(s, gi, with_mem):
        c0 = s * L
        g8 = gt[pl.ds(pl.multiple_of(gi * GH, GH), GH), :]
        row8 = _iota((8, T), 0)

        def col(j):
            return pl.ds(pl.multiple_of(c0 + j * T, T), T)

        def rows(w, off, n):
            return pl.ds(pl.multiple_of(gi * GR + w * WR + off, 8), n)

        state = [None, None]
        if with_mem:
            e = _iota((WR + 8, WR), 0)
            d = _iota((WR + 8, WR), 1)
            blk = jnp.zeros((WR + 8, WR), jnp.bool_)
            for i in range(4):
                in_d = (d >= DH * i) & (d < DH * (i + 1))
                blk = blk | (in_d & (((e >= DH * i) & (e < DH * (i + 1))) | (e == WR + i)))
            prev = pl.ds(pl.multiple_of(c0 - L, L), L)
            for w in range(2):
                lhs = jnp.concatenate([vv[rows(w, 0, WR), prev], jnp.ones((8, L), F32)], axis=0)
                upd = _dot(lhs, pk[rows(w, 0, WR), prev], NT)
                state[w] = jnp.where(blk, mem[2 * gi + w] + upd, 0.0)
                mem[2 * gi + w] = state[w]

        qtile, mx, acc, retr = {}, {}, {}, {}
        for t in range(len(tiles) + SKEW):
            if t < len(tiles):
                h, j, i = tiles[t]
                w = h // 4
                if i == 0:
                    q2 = qs[pl.ds(pl.multiple_of(gi * WR + 8 * h, 8), 16), col(j)]
                    r16 = _iota((16, T), 0)
                    q2 = jnp.where((r16 >= h) & (r16 < h + DH // 2), q2, jnp.uint32(0))
                    parts = [jnp.zeros((8 * (h - w), T), U32)] if h - w else []
                    parts.append(q2)
                    if 6 - (h - w):
                        parts.append(jnp.zeros((8 * (6 - (h - w)), T), U32))
                    qtile[h, j] = _bf(jnp.concatenate(parts, axis=0))
                kk = _bf(kn[2 * gi + w, pl.ds(pl.multiple_of(s * (L // 2) + i * (T // 2), T // 2), T // 2), :])
                z = _dot(kk, qtile[h, j])
                if i == j:
                    z = jnp.where(causal, z, NEG)
                sc[t % NS] = z
                m8 = z[0:8]
                for rb in range(1, T // 8):
                    m8 = jnp.maximum(m8, z[8 * rb:8 * rb + 8])
                if i > 0:
                    m8 = jnp.maximum(m8, mx[h, j])
                if i == j:
                    m8 = jnp.max(m8, axis=0, keepdims=True)
                mx[h, j] = m8
            if t >= SKEW:
                h, j, i = tiles[t - SKEW]
                w, hi = h // 4, h % 4
                p = jnp.exp2(sc[(t - SKEW) % NS] - mx[h, j]).astype(BF16)
                v3 = vv[rows(w, 16 * hi, 24), col(i)]
                if hi < 3:
                    v3 = jnp.concatenate([v3[0:16], jnp.where(row8 == 7, 1.0, v3[16:24])], axis=0)
                else:
                    v3 = jnp.concatenate([jnp.where(row8 == 0, 1.0, v3[0:8]), v3[8:24]], axis=0)
                o = _dot(v3, p)
                if i > 0:
                    o = o + acc[h, j]
                acc[h, j] = o
                if i == j:
                    gh = g8[h:h + 1, :]
                    den = o[23:24] if hi < 3 else o[0:1]
                    res = o * ((1.0 - gh) / den)
                    if with_mem:
                        if hi == 0:
                            retr[w, j] = _dot(state[w], pq[rows(w, 0, WR), col(j)])
                        rt = retr[w, j]
                        res = res + rt[16 * hi:16 * hi + 24] * (gh / (rt[WR + hi:WR + hi + 1] + 1e-6))
                    ot[gi, h * DH:(h + 1) * DH, col(j)] = res[2 * hi:2 * hi + DH]

    mem[...] = jnp.zeros(mem.shape, F32)

    def first_segment(gi, carry):
        attend(0, gi, False)
        return carry

    def later_segments(u, carry):
        attend(1 + u // NG, u % NG, True)
        return carry

    lax.fori_loop(0, NG, first_segment, 0)
    lax.fori_loop(0, (NSEG - 1) * NG, later_segments, 0)

    def phase4(s, carry):
        c = pl.ds(pl.multiple_of(s * L, L), L)
        tok = _iota((16, L), 1) + s * L
        r16 = _iota((16, L), 0)
        onehot = (((r16 == 0) & (tok == idx[0])) | ((r16 == 1) & (tok == idx[1]))).astype(F32)
        rhs = jnp.concatenate([ot[gi, :, c] for gi in range(NG)] + [onehot], axis=0).astype(BF16)
        a = _dot(_bf(wot[...]), rhs)
        out_v[:, c] = (a + (x_v[:, c].astype(F32) + _bf(xn[:, c]).astype(F32))).astype(BF16)
        o_copy(s).start()
        return carry

    lax.fori_loop(0, NSEG, phase4, 0)
    for s in range(NSEG):
        o_copy(s).wait()


@jax.jit
def pallas_parallel_sum__memory_aug_infini_attn__moe_arch_mod__prompt_kernel(
    A_x: jax.Array,
    A_wq: jax.Array,
    A_wk: jax.Array,
    A_wv: jax.Array,
    A_wo: jax.Array,
    A_beta: jax.Array,
    B_x: jax.Array,
    B_w_r: jax.Array,
    B_w_gate: jax.Array,
    B_w_up: jax.Array,
    B_w_down: jax.Array,
):
    del B_x
    hbm = pl.BlockSpec(memory_space=pltpu.HBM)
    vmem = pl.BlockSpec(memory_space=pltpu.VMEM)
    out_t = pl.pallas_call(
        _kernel,
        in_specs=[vmem, vmem] + [hbm] * 8,
        out_specs=hbm,
        out_shape=jax.ShapeDtypeStruct((D, S), BF16),
        scratch_shapes=[
            pltpu.VMEM((D, S), BF16),
            pltpu.VMEM((4, D, D), BF16),
            pltpu.VMEM((D, F), BF16),
            pltpu.VMEM((D, F), BF16),
            pltpu.VMEM((D, F), BF16),
            pltpu.VMEM((3 * D // 2 + 8, D), U32),
            pltpu.VMEM((D // 2, D + 16), U32),
            pltpu.VMEM((D // 2, S), U32),
            pltpu.VMEM((D // 2, S), U32),
            pltpu.VMEM((2 * NG, S // 2, T), U32),
            pltpu.VMEM((D, S), F32),
            pltpu.VMEM((D, S), F32),
            pltpu.VMEM((D, S), F32),
            pltpu.VMEM((8, S), F32),
            pltpu.VMEM((NG, GR, S), F32),
            pltpu.VMEM((NS, T, T), F32),
            pltpu.VMEM((2 * NG, WR + 8, WR), F32),
            pltpu.VMEM((H, T), F32),
            pltpu.VMEM((D, S), BF16),
            pltpu.SemaphoreType.DMA((NSEG,)),
            pltpu.SemaphoreType.DMA((4,)),
            pltpu.SemaphoreType.DMA((3,)),
            pltpu.SemaphoreType.DMA((NSEG,)),
        ],
        compiler_params=pltpu.CompilerParams(vmem_limit_bytes=100 * 1024 * 1024),
        name="infini_mod",
    )(A_beta, B_w_r, A_x[0].T, A_wq, A_wk, A_wv, A_wo, B_w_gate, B_w_up, B_w_down.T)
    return out_t.T[None]
```

```python
import math

import jax
import jax.numpy as jnp
from jax import lax
import jax.experimental.pallas as pl
import jax.experimental.pallas.tpu as pltpu

S = 2048
D = 576
H = 32
DH = D // H
NSEG = 4
L = S // NSEG
F = 4608
T = 128
GH = 8
NG = H // GH
WR = 4 * DH
NW = H // 4
QSCALE = (DH ** -0.5) * math.log2(math.e)
NEG = -1e30
SKEW = 12
NS = 32
FFN_EVERY = 10
FFN_START = 12

F32 = jnp.float32
BF16 = jnp.bfloat16
U32 = jnp.uint32
NN = (((1,), (0,)), ((), ()))
NT = (((1,), (1,)), ((), ()))


def _dot(a, b, dims=NN):
    return lax.dot_general(a, b, dims, preferred_element_type=F32)


def _bf(x):
    return pltpu.bitcast(x, BF16)


def _u(x):
    return pltpu.bitcast(x, U32)


def _round(x):
    return x.astype(BF16).astype(F32)


def _phi(t):
    return jnp.where(t > 0, t + 1.0, jnp.exp(t))


def _iota(shape, dim):
    return lax.broadcasted_iota(jnp.int32, shape, dim)


def _ds(start, size, align):
    return pl.ds(start if isinstance(start, int) else pl.multiple_of(start, align), size)


def _kernel(beta_hbm, wr_hbm, x_hbm, wq_hbm, wk_hbm, wv_hbm, wo_hbm, wg_hbm, wu_hbm, wd_hbm,
            out_hbm,
            beta_v, wr_v, x_v, w_v, wg_v, wu_v, wd_v, wt, wot, xn, qs, kn, pq, pk, vv, rr, ot, sc, mem, gt,
            out_v, sem_s, sem_x, sem_w, sem_f, sem_o):

    def seg(s):
        return _ds(s * L, L, L)

    s_copies = [pltpu.make_async_copy(a, b, sem_s.at[i])
                for i, (a, b) in enumerate(((beta_hbm, beta_v), (wr_hbm, wr_v)))]
    x_copies = [pltpu.make_async_copy(x_hbm.at[:, seg(s)], x_v.at[:, seg(s)], sem_x.at[s])
                for s in range(NSEG)]
    o_copies = [pltpu.make_async_copy(out_v.at[:, seg(s)], out_hbm.at[:, seg(s)], sem_o.at[s])
                for s in range(NSEG)]
    w_copies = [pltpu.make_async_copy(w, w_v.at[i], sem_w.at[i])
                for i, w in enumerate((wq_hbm, wk_hbm, wv_hbm, wo_hbm))]
    f_copies = [pltpu.make_async_copy(a, b, sem_f.at[i])
                for i, (a, b) in enumerate(((wg_hbm, wg_v), (wu_hbm, wu_v), (wd_hbm, wd_v)))]

    def layernorm(s):
        for n in range(L // T):
            c = slice(s * L + n * T, s * L + (n + 1) * T)
            x = x_v[:, c].astype(F32)
            mean = jnp.sum(x, axis=0, keepdims=True) * (1.0 / D)
            xc = x - mean
            var = jnp.sum(xc * xc, axis=0, keepdims=True) * (1.0 / D)
            sd = _round(jnp.sqrt(_round(_round(var) + _round(jnp.full((1, T), 1e-5, F32)))))
            y = _round(x - _round(mean)) * (1.0 / sd)
            xn[:, c] = _u(y.astype(BF16))

    def load_weight(i):
        wt[i * D // 2:(i + 1) * D // 2, :] = _u(w_v[i].T)

    def project_q(s, sync=lambda: None):
        q = _dot(_bf(wt[0:D // 2, :]), _bf(xn[:, seg(s)]))
        sync()
        qs[:, seg(s)] = _u((q * QSCALE).astype(BF16))
        if s > 0:
            pq[:, seg(s)] = _phi(q)

    def project_k(s, sync=lambda: None):
        k = _dot(_bf(wt[D // 2:D, :]), _bf(xn[:, seg(s)]))
        sync()
        pk[:, seg(s)] = _phi(k) if s < NSEG - 1 else k
        kb = _u(k.astype(BF16))
        for w in range(NW):
            r0 = (w // 2) * WR + 8 * (w % 2)
            for n in range(L // T):
                blk = _bf(kb[r0:r0 + T // 2, n * T:(n + 1) * T])
                t0 = (s * L + n * T) // 2
                kn[w, t0:t0 + T // 2, :] = _u(blk.T)

    def project_v(s, router=True):
        vr = _dot(_bf(wt[D:, :]), _bf(xn[:, seg(s)]))
        vv[:, seg(s)] = vr[0:D]
        rr[:, seg(s)] = vr[D:D + 8]

    w_copies[0].start()
    x_copies[0].start()
    for c in s_copies:
        c.start()
    w_copies[0].wait()
    w_copies[1].start()
    x_copies[0].wait()
    for c in s_copies:
        c.wait()
    g = jax.nn.sigmoid(beta_v[...].astype(F32)).reshape(1, H)
    gcol = jnp.sum(jnp.where(_iota((H, H), 0) == _iota((H, H), 1), jnp.broadcast_to(g, (H, H)), 0.0),
                   axis=1, keepdims=True)
    gt[...] = jnp.broadcast_to(gcol, (H, T))
    wr = jnp.broadcast_to(wr_v[...].astype(F32).reshape(1, D), (16, D)).astype(BF16)
    wt[3 * D // 2:, :] = _u(wr)
    layernorm(0)
    load_weight(0)
    for c in w_copies[2:3] + x_copies[1:] + w_copies[3:]:
        c.start()
    w_copies[1].wait()

    def sync1():
        w_copies[2].wait()

    def sync2():
        for c in f_copies:
            c.start()
        for c in x_copies[1:] + w_copies[3:]:
            c.wait()

    load_weight(1)
    project_q(0, sync1)
    load_weight(2)
    project_k(0, sync2)
    project_v(0)
    layernorm(1)
    project_v(1)
    layernorm(2)
    project_v(2)
    layernorm(3)
    project_v(3)
    project_q(1)

    r = _round(rr[...])
    pos = _iota((8, S), 1).astype(F32)
    r0 = jnp.max(r)
    i0 = jnp.min(jnp.where(r == r0, pos, float(S)))
    r_rest = jnp.where(pos == i0, -jnp.inf, r)
    r1 = jnp.max(r_rest)
    i1 = jnp.min(jnp.where((r_rest == r1) & (pos != i0), pos, float(S)))
    idx = [jnp.clip(i.astype(jnp.int32), 0, S - 1) for i in (i0, i1)]
    project_k(1)
    xsel = None
    for t in range(2):
        tile = idx[t] // T
        onehot = ((_iota((8, T), 0) == t) & (_iota((8, T), 1) == idx[t] - tile * T)).astype(F32)
        part = _dot(onehot, _bf(xn[:, _ds(tile * T, T, T)]), NT)
        xsel = part if xsel is None else xsel + part
    wot[:, 0:4 * T] = _u(w_v[3, 0:4 * T, :].T)
    for s in range(2, NSEG):
        project_q(s)
        project_k(s, lambda: [c.wait() for c in f_copies] if s == NSEG - 1 else None)

    def ffn_steps(s, box):
        n = F // T // NSEG
        hid = {}
        for i in range(n + 1):
            if i < n:
                c = _ds((s * n + i) * T, T, T)
                a = _dot(xsel, wg_v[:, c])
                yield
                b = _dot(xsel, wu_v[:, c])
                hid[i] = a * jax.nn.sigmoid(a) * b
                yield
            if i > 0:
                box[0] = box[0] + _dot(hid.pop(i - 1), wd_v[:, _ds((s * n + i - 1) * T, T, T)], NT)
                yield

    tiles = [(h, j, i) for h in range(H) for j in range(L // T) for i in range(j + 1)]

    def attend(s, y, first):
        causal = _iota((T, T), 0) <= _iota((T, T), 1)
        row8 = _iota((8, T), 0)
        qtile, mx, acc, retr = {}, {}, {}, {}

        def col(j):
            return _ds(s * L + j * T, T, T)

        def scores(t):
            h, j, i = tiles[t]
            gi, hg, w = h // GH, h % GH, h // 4
            if i == 0:
                q2 = qs[gi * WR + 8 * hg:gi * WR + 8 * hg + 16, col(j)]
                r16 = _iota((16, T), 0)
                q2 = jnp.where((r16 >= hg) & (r16 < hg + DH // 2), q2, jnp.uint32(0))
                lead = hg - w % 2
                parts = [jnp.zeros((8 * lead, T), U32)] if lead else []
                parts.append(q2)
                if 6 - lead:
                    parts.append(jnp.zeros((8 * (6 - lead), T), U32))
                qtile[0] = _bf(jnp.concatenate(parts, axis=0))
            z = _dot(_bf(kn[w, _ds((s * L + i * T) // 2, T // 2, T // 2), :]), qtile[0])
            if i == j:
                z = jnp.where(causal, z, NEG)
            sc[t % NS] = z
            m8 = z[0:8]
            for rb in range(1, T // 8):
                m8 = jnp.maximum(m8, z[8 * rb:8 * rb + 8])
            if i > 0:
                m8 = jnp.maximum(m8, mx[h, j])
            if i == j:
                m8 = jnp.max(m8, axis=0, keepdims=True)
            mx[h, j] = m8

        def values(t):
            h, j, i = tiles[t]
            w, hi = h // 4, h % 4
            p = jnp.exp2(sc[t % NS] - mx[h, j]).astype(BF16)
            v3 = vv[w * WR + 16 * hi:w * WR + 16 * hi + 24, col(i)]
            if hi < 3:
                v3 = jnp.concatenate([v3[0:16], jnp.where(row8 == 7, 1.0, v3[16:24])], axis=0)
            else:
                v3 = jnp.concatenate([jnp.where(row8 == 0, 1.0, v3[0:8]), v3[8:24]], axis=0)
            o = _dot(v3, p)
            if i > 0:
                o = o + acc[0]
            acc[0] = o
            if not first and hi == 0 and i == 0:
                retr[j] = _dot(mem[w], pq[w * WR:(w + 1) * WR, col(j)])
            if i == j:
                gh = gt[h:h + 1, :]
                den = o[23:24] if hi < 3 else o[0:1]
                res = o * ((1.0 - gh) / den)
                if not first:
                    rt = retr[j]
                    res = res + rt[16 * hi:16 * hi + 24] * (gh / (rt[WR + hi:WR + hi + 1] + 1e-6))
                ot[h * DH:(h + 1) * DH, col(j)] = res[2 * hi:2 * hi + DH]

        def update(w):
            e = _iota((WR + 8, WR), 0)
            d = _iota((WR + 8, WR), 1)
            same_head = None
            for i in range(4):
                in_d = (d >= DH * i) & (d < DH * (i + 1))
                m = in_d & (((e >= DH * i) & (e < DH * (i + 1))) | (e == WR + i))
                same_head = m if same_head is None else same_head | m
            lhs = jnp.concatenate([vv[w * WR:(w + 1) * WR, seg(s)], jnp.ones((8, L), F32)], axis=0)
            upd = jnp.where(same_head, _dot(lhs, pk[w * WR:(w + 1) * WR, seg(s)], NT), 0.0)
            mem[w] = upd if first else mem[w] + upd

        box = [y]
        ffn = ffn_steps(s, box)
        for t in range(len(tiles) + SKEW):
            if t < len(tiles):
                scores(t)
            elif t - len(tiles) < NW:
                update(t - len(tiles))
            if t >= SKEW:
                values(t - SKEW)
            if t >= FFN_START and (t - FFN_START) % FFN_EVERY == 0:
                next(ffn, None)
        assert next(ffn, "done") == "done"
        return box[0]

    y = attend(0, jnp.zeros((8, D), F32), True)
    y = lax.fori_loop(1, NSEG, lambda s, y: attend(s, y, False), y)

    gate = jax.nn.sigmoid(jnp.where(_iota((8, D), 0) == 0, r0, r1))
    y = jnp.where(_iota((8, D), 0) < 2, y * gate, 0.0)
    tail = jnp.concatenate(
        [w_v[3, 4 * T:D, :], jnp.concatenate([y, jnp.zeros((8, D), F32)], axis=0).astype(BF16)], axis=0)
    wot[:, 4 * T:] = _u(tail.T)
    for s in range(NSEG):
        tok = _iota((16, L), 1) + s * L
        r16 = _iota((16, L), 0)
        onehot = (((r16 == 0) & (tok == idx[0])) | ((r16 == 1) & (tok == idx[1]))).astype(F32)
        rhs = jnp.concatenate([ot[:, seg(s)], onehot], axis=0).astype(BF16)
        a = _dot(_bf(wot[...]), rhs)
        out_v[:, seg(s)] = (a + (x_v[:, seg(s)].astype(F32) + _bf(xn[:, seg(s)]).astype(F32))).astype(BF16)
        o_copies[s].start()
    for c in o_copies:
        c.wait()


@jax.jit
def pallas_parallel_sum__memory_aug_infini_attn__moe_arch_mod__prompt_kernel(
    A_x: jax.Array,
    A_wq: jax.Array,
    A_wk: jax.Array,
    A_wv: jax.Array,
    A_wo: jax.Array,
    A_beta: jax.Array,
    B_x: jax.Array,
    B_w_r: jax.Array,
    B_w_gate: jax.Array,
    B_w_up: jax.Array,
    B_w_down: jax.Array,
):
    del B_x
    hbm = pl.BlockSpec(memory_space=pltpu.HBM)
    out_t = pl.pallas_call(
        _kernel,
        in_specs=[hbm] * 10,
        out_specs=hbm,
        out_shape=jax.ShapeDtypeStruct((D, S), BF16),
        scratch_shapes=[
            pltpu.VMEM((H,), BF16),
            pltpu.VMEM((D,), BF16),
            pltpu.VMEM((D, S), BF16),
            pltpu.VMEM((4, D, D), BF16),
            pltpu.VMEM((D, F), BF16),
            pltpu.VMEM((D, F), BF16),
            pltpu.VMEM((D, F), BF16),
            pltpu.VMEM((3 * D // 2 + 8, D), U32),
            pltpu.VMEM((D // 2, D + 16), U32),
            pltpu.VMEM((D // 2, S), U32),
            pltpu.VMEM((D // 2, S), U32),
            pltpu.VMEM((NW, S // 2, T), U32),
            pltpu.VMEM((D, S), F32),
            pltpu.VMEM((D, S), F32),
            pltpu.VMEM((D, S), F32),
            pltpu.VMEM((8, S), F32),
            pltpu.VMEM((D, S), F32),
            pltpu.VMEM((NS, T, T), F32),
            pltpu.VMEM((NW, WR + 8, WR), F32),
            pltpu.VMEM((H, T), F32),
            pltpu.VMEM((D, S), BF16),
            pltpu.SemaphoreType.DMA((2,)),
            pltpu.SemaphoreType.DMA((NSEG,)),
            pltpu.SemaphoreType.DMA((4,)),
            pltpu.SemaphoreType.DMA((3,)),
            pltpu.SemaphoreType.DMA((NSEG,)),
        ],
        compiler_params=pltpu.CompilerParams(vmem_limit_bytes=100 * 1024 * 1024),
        name="infini_mod",
    )(A_beta, B_w_r, A_x[0].T, A_wq, A_wk, A_wv, A_wo, B_w_gate, B_w_up, B_w_down.T)
    return out_t.T[None]
```

```python
import math

import jax
import jax.numpy as jnp
from jax import lax
import jax.experimental.pallas as pl
import jax.experimental.pallas.tpu as pltpu

S = 2048
D = 576
H = 32
DH = D // H
NSEG = 4
L = S // NSEG
F = 4608
T = 128
HT = T // 2
NT_L = L // T
GH = 8
NG = H // GH
GR = GH * DH
WR = 4 * DH
NW = H // 4
WK = 80
FC = F // (NSEG - 1)
QSCALE = (DH ** -0.5) * math.log2(math.e)
NEG = -1e30
NB = 64
LAG = 1024
LAG0 = 2200
SYNC1 = 2

F32 = jnp.float32
BF16 = jnp.bfloat16
U32 = jnp.uint32
NN = (((1,), (0,)), ((), ()))
NT = (((1,), (1,)), ((), ()))
KT = [(k, min(k + T, D)) for k in range(0, D, T)]


def _dot(a, b, dims=NN):
    return lax.dot_general(a, b, dims, preferred_element_type=F32)


def _bf(x):
    return pltpu.bitcast(x, BF16)


def _u(x):
    return pltpu.bitcast(x, U32)


def _pack(x):
    return _u(x.astype(BF16))


def _round(x):
    return x.astype(BF16).astype(F32)


def _phi(t):
    return jnp.where(t > 0, t + 1.0, jnp.exp(t))


def _iota(shape, dim):
    return lax.broadcasted_iota(jnp.int32, shape, dim)


def _ds(start, size, align):
    return pl.ds(start if isinstance(start, int) else pl.multiple_of(start, align), size)


def _interleave(main, fillers, per_step=4):
    fillers = list(fillers)
    for _ in main:
        for _ in range(per_step):
            while fillers and next(fillers[0], "done") == "done":
                fillers.pop(0)
    for f in fillers:
        for _ in f:
            pass


def _attention_schedule():
    qk, pv = [], []
    for hp in range(0, H, 2):
        for j in range(NT_L):
            qk.append(("x", hp, j, j * T + HT, HT))
            for h in (hp, hp + 1):
                qk += [("m", h, j, i * T, T) for i in range(j)] + [("m", h, j, j * T, HT)]
            pv += [(hp, j, i) for i in range(j)] + [(hp + 1, j, i) for i in range(j)]
            pv += [(hp, j, j), (hp + 1, j, j)]
    return qk, pv


def _kernel(beta_hbm, wr_hbm, x_hbm, wq_hbm, wk_hbm, wv_hbm, wo_hbm, wg_hbm, wu_hbm, wd_hbm,
            out_hbm,
            beta_v, wr_v, x_v, w_v, wg_v, wu_v, wd_v, wt, wot, xn, qs, kn, pq, pk, vv, rr, ot, sc, mem, gt, bias,
            out_v, sem_s, sem_x, sem_w, sem_f, sem_o):

    def seg(s):
        return _ds(s * L, L, L)

    def col(s, j):
        return _ds(s * L + j * T, T, T)

    s_copies = [pltpu.make_async_copy(a, b, sem_s.at[i])
                for i, (a, b) in enumerate(((beta_hbm, beta_v), (wr_hbm, wr_v)))]
    x_parts = [seg(0), seg(1), slice(2 * L, S)]
    x_copies = [pltpu.make_async_copy(x_hbm.at[:, c], x_v.at[:, c], sem_x.at[i]) for i, c in enumerate(x_parts)]
    w_copies = [pltpu.make_async_copy(w, w_v.at[i], sem_w.at[i])
                for i, w in enumerate((wq_hbm, wk_hbm, wv_hbm, wo_hbm))]

    f_copies = [[pltpu.make_async_copy(a.at[:, c], b.at[:, c], sem_f.at[3 * i + n])
                 for n, (a, b) in enumerate(((wg_hbm, wg_v), (wu_hbm, wu_v), (wd_hbm, wd_v)))]
                for i, c in enumerate((slice(0, 2 * FC), slice(2 * FC, F)))]

    o_parts = [(slice(0, D), seg(s)) for s in range(NSEG - 1)]
    o_parts += [(slice(g * GR, (g + 1) * GR), seg(NSEG - 1)) for g in range(NG)]
    o_copies = [pltpu.make_async_copy(out_v.at[r, c], out_hbm.at[r, c], sem_o.at[i])
                for i, (r, c) in enumerate(o_parts)]

    def layernorm(s, n):
        x = x_v[:, col(s, n)].astype(F32)
        mean = jnp.sum(x, axis=0, keepdims=True) * (1.0 / D)
        xc = x - mean
        var = jnp.sum(xc * xc, axis=0, keepdims=True) * (1.0 / D)
        sd = _round(jnp.sqrt(_round(_round(var) + _round(jnp.full((1, T), 1e-5, F32)))))
        y = _round(x - _round(mean)) * (1.0 / sd)
        xn[:, col(s, n)] = _u(y.astype(BF16))

    def load_weight(i):
        wt[i * D // 2:(i + 1) * D // 2, :] = _u(w_v[i].T)

    def finish_q(s, g, n, q):
        qs[g * GR // 2:(g + 1) * GR // 2, col(s, n)] = _u((q * QSCALE).astype(BF16))
        if s > 0:
            pq[g * GR:(g + 1) * GR, col(0, n)] = _phi(q)

    def finish_k(s, g, n, k):
        if s < NSEG - 1:
            pk[g * GR:(g + 1) * GR, col(s, n)] = _phi(k)
        kb = _u(k.astype(BF16))
        for w in range(2):
            blk = _bf(kb[w * (GR - WK) // 2:w * (GR - WK) // 2 + WK // 2])
            kn[2 * g + w, _ds((s * L + n * T) // 2, HT, HT), :] = _u(blk.T)

    def project_group(i, s, g, finish, sync=None):
        rows = slice((i * D + g * GR) // 2, (i * D + (g + 1) * GR) // 2)
        tail = _dot(_bf(wt[rows, 4 * T:D]), _bf(xn[2 * T:D // 2, seg(s)]))
        yield
        held = []
        for n in range(NT_L):
            held.append(_dot(_bf(wt[rows, 0:4 * T]), _bf(xn[0:2 * T, col(s, n)])) + tail[:, n * T:(n + 1) * T])
            yield
            if sync is None:
                finish(s, g, n, held[n])
        if sync is not None:
            sync()
            for n in range(NT_L):
                finish(s, g, n, held[n])

    for c in [x_copies[0], w_copies[1]] + s_copies:
        c.start()

    def touch(i, carry):
        rows = pl.ds(pl.multiple_of(i * 8, 8), 8)
        for ref in (wt, wot, qs, pq, pk, vv, ot, gt):
            ref[rows, 0:T] = jnp.zeros((8, T), ref.dtype)
        for ref in (kn, sc, mem, bias):
            ref[0, rows, :] = jnp.zeros((8, ref.shape[2]), ref.dtype)
        return carry

    lax.fori_loop(0, 2, touch, 0)
    r64, c64 = _iota((HT, T), 0), _iota((HT, T), 1)
    bias[0] = jnp.where((c64 < HT) | (r64 <= c64 - HT), 0.0, NEG)
    bias[1] = jnp.where(r64 <= c64, 0.0, NEG)
    bias[2] = jnp.where(r64 <= c64 % HT, 0.0, NEG)
    x_copies[0].wait()
    w_copies[0].start()
    w_copies[2].start()
    for c in s_copies:
        c.wait()
    g = jax.nn.sigmoid(beta_v[...].astype(F32)).reshape(1, H)
    own = _iota((H, H), 0) == _iota((H, H), 1)
    gcol = jnp.sum(jnp.where(own, jnp.broadcast_to(g, (H, H)), 0.0), axis=1, keepdims=True)
    gt[...] = jnp.broadcast_to(gcol, (H, T))
    wt[3 * D // 2:, :] = _pack(jnp.broadcast_to(wr_v[...].astype(F32).reshape(1, D), (16, D)))
    for n in range(NT_L):
        layernorm(0, n)
    w_copies[1].wait()
    load_weight(1)

    def sync1():
        w_copies[0].wait()
        x_copies[1].start()
        x_copies[2].start()
        w_copies[2].wait()
        load_weight(0)
        load_weight(2)

    def sync2():
        x_copies[1].wait()
        for c in f_copies[0]:
            c.start()
        x_copies[2].wait()

    for g in range(NG):
        _interleave(project_group(1, 0, g, finish_k, sync1 if g == SYNC1 else None), [])
    for g in range(NG):
        _interleave(project_group(0, 0, g, finish_q, sync2 if g == NG - 1 else None), [])
    for s in range(NSEG):
        v = _dot(_bf(wt[D:, :]), _bf(xn[:, seg(s)]))
        vv[:, seg(s)] = v[0:D]
        rr[:, seg(s)] = v[D:D + 8]
        if s < NSEG - 1:
            for n in range(NT_L):
                layernorm(s + 1, n)

    r = _round(rr[...])
    pos = _iota((8, S), 1).astype(F32)
    r0 = jnp.max(r)
    i0 = jnp.min(jnp.where(r == r0, pos, float(S)))
    r_rest = jnp.where(pos == i0, -jnp.inf, r)
    r1 = jnp.max(r_rest)
    i1 = jnp.min(jnp.where((r_rest == r1) & (pos != i0), pos, float(S)))
    idx = [jnp.clip(i.astype(jnp.int32), 0, S - 1) for i in (i0, i1)]

    picked = []

    def gather():
        parts = []
        for t in range(2):
            tile = idx[t] // T
            onehot = ((_iota((8, T), 0) == t) & (_iota((8, T), 1) == idx[t] - tile * T)).astype(F32)
            parts.append(_dot(onehot, _bf(xn[:, _ds(tile * T, T, T)]), NT))
        picked.append(parts[0] + parts[1])

    arrived = []

    def ffn_steps(i, ys):
        n = FC // T
        hid = {}
        while len(arrived) <= i:
            yield
        for f in range(n + 1):
            if f < n:
                ab = []
                for w in (wg_v, wu_v):
                    a = None
                    for k0, k1 in KT:
                        d = _dot(picked[0][:, k0:k1], w[k0:k1, _ds(i * FC + f * T, T, T)])
                        a = d if a is None else a + d
                        yield
                    ab.append(a)
                hid[f] = ab[0] * jax.nn.sigmoid(ab[0]) * ab[1]
            if f > 0:
                h = hid.pop(f - 1)
                for q, (k0, k1) in enumerate(KT):
                    ys[q] = ys[q] + _dot(h, wd_v[k0:k1, _ds(i * FC + (f - 1) * T, T, T)], NT)
                    yield

    qk, pv = _attention_schedule()

    def attend(s):
        row8 = _iota((8, T), 0)
        low = _iota((8, T), 1) < HT
        low32 = _iota((HT // 2, T), 1) < HT
        zero = jnp.uint32(0)
        qtile, mx, acc, slot, px = {}, {}, {}, {}, {}

        def q_rows(h, j):
            hg = h % GH
            r0 = (h // GH) * GR // 2 + 8 * hg
            q2 = qs[r0:r0 + 16, col(s, j)]
            if h % 2 == 0:
                q2 = pltpu.roll(q2, HT, 1)
            r16 = _iota((16, T), 0)
            return jnp.where((r16 >= hg) & (r16 < hg + DH // 2), q2, zero)

        def q_pad(q, h):
            return _bf(jnp.concatenate([jnp.zeros((8 * (h % 4), T), U32), q], axis=0) if h % 4 else q)

        def scores(kind, h, j, k0, n):
            if kind == "x":
                qa, qb = q_rows(h, j), q_rows(h + 1, j)
                qtile[h], qtile[h + 1] = q_pad(qa, h), q_pad(qb, h + 1)
                rhs = q_pad(jnp.concatenate([jnp.where(low, qa[0:8], zero), jnp.where(low, qa[8:16], qb[0:8]),
                                             jnp.where(low, zero, qb[8:16])], axis=0), h)
            else:
                rhs = qtile[h]
            z = _dot(_bf(kn[h // 4, _ds((s * L + k0) // 2, n // 2, HT // 2), 0:rhs.shape[0]]), rhs)
            m8 = None
            for b in range(n // HT):
                zb = z[b * HT:(b + 1) * HT]
                key = k0 + b * HT
                if key >= j * T:
                    zb = zb + bias[2 if kind == "x" else h % 2]
                slot[kind, h, j, key] = len(slot) % NB
                sc[slot[kind, h, j, key]] = zb
                for rb in range(HT // 8):
                    m8 = zb[8 * rb:8 * rb + 8] if m8 is None else jnp.maximum(m8, zb[8 * rb:8 * rb + 8])
            if kind == "x":
                mx[h, j] = jnp.where(low, m8, NEG)
                mx[h + 1, j] = jnp.where(low, NEG, m8)
            else:
                m8 = jnp.maximum(m8, mx[h, j])
                mx[h, j] = jnp.max(m8, axis=0, keepdims=True) if k0 + n > j * T else m8

        def probs(key, m):
            assert len(slot) - list(slot).index(key) <= NB
            return jnp.exp2(sc[slot[key]] - m)

        def values(h, j, i):
            w, hi = h // 4, h % 4
            if i < j:
                p = jnp.concatenate([probs(("m", h, j, i * T + b * HT), mx[h, j]) for b in range(2)], axis=0)
                p = p.astype(BF16)
            else:
                if h % 2 == 0:
                    px[0] = _pack(probs(("x", h, j, j * T + HT), jnp.where(low[0:1], mx[h, j], mx[h + 1, j])))
                    upper = jnp.where(low32, px[0], zero)
                else:
                    upper = jnp.where(low32, zero, px[0])
                p = _bf(jnp.concatenate([_pack(probs(("m", h, j, j * T), mx[h, j])), upper], axis=0))
            v3 = vv[w * WR + 16 * hi:w * WR + 16 * hi + 24, col(s, i)]
            if hi < 3:
                v3 = jnp.concatenate([v3[0:16], jnp.where(row8 == 7, 1.0, v3[16:24])], axis=0)
            else:
                v3 = jnp.concatenate([jnp.where(row8 == 0, 1.0, v3[0:8]), v3[8:24]], axis=0)
            o = _dot(v3, p)
            if i > 0:
                o = o + acc[h]
            acc[h] = o
            if i == j:
                if h % 2 == 0:
                    o = pltpu.roll(o, HT, 1)
                den = o[23:24] if hi < 3 else o[0:1]
                inv = pl.reciprocal(den, approx=True)
                res = o * ((1.0 - gt[h:h + 1, :]) * (inv * (2.0 - den * inv)))
                if s == 0:
                    ot[h * DH:(h + 1) * DH, col(s, j)] = res[2 * hi:2 * hi + DH]
                else:
                    ot[h * DH:(h + 1) * DH, col(s, j)] += res[2 * hi:2 * hi + DH]

        total, ready = 0, {}
        for _, h, j, _, n in qk:
            total += n
            ready[h, j] = total
        issued, tv = 0, 0
        for piece in qk:
            scores(*piece)
            issued += piece[4]
            while True:
                h, j, i = pv[tv]
                need = ready[h | 1, j] if i == j else ready[h, j]
                if issued < max(need + LAG, LAG0 + tv * total / len(pv)):
                    break
                values(h, j, i)
                tv += 1

        def drain():
            for tile in pv[tv:]:
                values(*tile)
                yield

        return drain()

    def memory_update(s, w):
        e = _iota((WR + 8, WR), 0)
        d = _iota((WR + 8, WR), 1)
        same_head = None
        for i in range(4):
            m = (d >= DH * i) & (d < DH * (i + 1)) & (((e >= DH * i) & (e < DH * (i + 1))) | (e == WR + i))
            same_head = m if same_head is None else same_head | m
        lhs = jnp.concatenate([vv[w * WR:(w + 1) * WR, seg(s)], jnp.ones((8, L), F32)], axis=0)
        return jnp.where(same_head, _dot(lhs, pk[w * WR:(w + 1) * WR, seg(s)], NT), 0.0)

    def memory_read(s, w):
        rt = _dot(mem[w], pq[w * WR:(w + 1) * WR, :])
        r8 = _iota((8, T), 0)
        g4 = jnp.zeros((8, T), F32)
        for i in range(4):
            g4 = jnp.where(r8 == i, gt[4 * w + i:4 * w + i + 1, :], g4)
        for n in range(NT_L):
            part = rt[:, n * T:(n + 1) * T]
            scale = g4 / (part[WR:WR + 8] + 1e-6)
            rows = []
            for b in range(WR // 8):
                lo, hi = 8 * b // DH, (8 * b + 7) // DH
                c = scale[lo:lo + 1]
                if hi != lo:
                    c = jnp.where(r8 < hi * DH - 8 * b, c, scale[hi:hi + 1])
                rows.append(part[8 * b:8 * b + 8] * c)
            ot[w * WR:(w + 1) * WR, col(s, n)] = jnp.concatenate(rows, axis=0)

    def next_segment(s):
        if s == 0:
            gather()
        held = []
        for w in range(NW):
            held.append(memory_update(s, w))
            yield
        if s == 0:
            for c in f_copies[0][:2]:
                c.wait()
            for c in f_copies[1] + w_copies[3:]:
                c.start()
            f_copies[0][2].wait()
            arrived.extend((0, 1))
        elif s == 2:
            for c in f_copies[1] + w_copies[3:]:
                c.wait()
            arrived.append(2)
        for w in range(NW):
            mem[w] = held[w] if s == 0 else mem[w] + held[w]
        for g in range(NG):
            yield from project_group(0, s + 1, g, finish_q)
        for g in range(NG):
            yield from project_group(1, s + 1, g, finish_k)
            for w in (2 * g, 2 * g + 1):
                memory_read(s + 1, w)
                yield

    def segment(s, y):
        ys = [y[:, k0:k1] for k0, k1 in KT]
        _interleave(next_segment(s), [attend(s), ffn_steps(s, ys)])
        return jnp.concatenate(ys, axis=1)

    y = jnp.zeros((8, D), F32)
    for s in range(NSEG - 1):
        y = segment(s, y)

    gate = jax.nn.sigmoid(jnp.where(_iota((8, D), 0) == 0, r0, r1))
    y = jnp.where(_iota((8, D), 0) < 2, y * gate, 0.0)
    wot[:, 0:4 * T] = _u(w_v[3, 0:4 * T, :].T)
    tail = jnp.concatenate(
        [w_v[3, 4 * T:D, :], jnp.concatenate([y, jnp.zeros((8, D), F32)], axis=0).astype(BF16)], axis=0)
    wot[:, 4 * T:] = _u(tail.T)

    def project_out(i):
        s = min(i, NSEG - 1)
        rows = o_parts[i][0]
        half = slice(rows.start // 2, rows.stop // 2)
        tok = _iota((16, L), 1) + s * L
        r16 = _iota((16, L), 0)
        onehot = (((r16 == 0) & (tok == idx[0])) | ((r16 == 1) & (tok == idx[1]))).astype(F32)
        rhs = jnp.concatenate([ot[4 * T:D, seg(s)], onehot], axis=0).astype(BF16)
        last = _dot(_bf(wot[half, 4 * T:]), rhs)
        yield
        for n in range(NT_L):
            a = _dot(_bf(wot[half, 0:4 * T]), ot[0:4 * T, col(s, n)].astype(BF16)) + last[:, n * T:(n + 1) * T]
            res = x_v[rows, col(s, n)].astype(F32) + _bf(xn[half, col(s, n)]).astype(F32)
            out_v[rows, col(s, n)] = (a + res).astype(BF16)
            yield
        o_copies[i].start()

    drain = attend(NSEG - 1)
    _interleave(project_out(0), [drain])
    for i in range(1, len(o_parts)):
        _interleave(project_out(i), [])
    for c in o_copies:
        c.wait()


@jax.jit
def pallas_parallel_sum__memory_aug_infini_attn__moe_arch_mod__prompt_kernel(
    A_x: jax.Array,
    A_wq: jax.Array,
    A_wk: jax.Array,
    A_wv: jax.Array,
    A_wo: jax.Array,
    A_beta: jax.Array,
    B_x: jax.Array,
    B_w_r: jax.Array,
    B_w_gate: jax.Array,
    B_w_up: jax.Array,
    B_w_down: jax.Array,
):
    del B_x
    hbm = pl.BlockSpec(memory_space=pltpu.HBM)
    out_t = pl.pallas_call(
        _kernel,
        in_specs=[hbm] * 10,
        out_specs=hbm,
        out_shape=jax.ShapeDtypeStruct((D, S), BF16),
        scratch_shapes=[
            pltpu.VMEM((H,), BF16),
            pltpu.VMEM((D,), BF16),
            pltpu.VMEM((D, S), BF16),
            pltpu.VMEM((4, D, D), BF16),
            pltpu.VMEM((D, F), BF16),
            pltpu.VMEM((D, F), BF16),
            pltpu.VMEM((D, F), BF16),
            pltpu.VMEM((3 * D // 2 + 8, D), U32),
            pltpu.VMEM((D // 2, D + 16), U32),
            pltpu.VMEM((D // 2, S), U32),
            pltpu.VMEM((D // 2, S), U32),
            pltpu.VMEM((NW, S // 2, WK), U32),
            pltpu.VMEM((D, L), F32),
            pltpu.VMEM((D, S), F32),
            pltpu.VMEM((D, S), F32),
            pltpu.VMEM((8, S), F32),
            pltpu.VMEM((D, S), F32),
            pltpu.VMEM((NB, HT, T), F32),
            pltpu.VMEM((NW, WR + 8, WR), F32),
            pltpu.VMEM((H, T), F32),
            pltpu.VMEM((3, HT, T), F32),
            pltpu.VMEM((D, S), BF16),
            pltpu.SemaphoreType.DMA((2,)),
            pltpu.SemaphoreType.DMA((3,)),
            pltpu.SemaphoreType.DMA((4,)),
            pltpu.SemaphoreType.DMA((6,)),
            pltpu.SemaphoreType.DMA((NSEG - 1 + NG,)),
        ],
        compiler_params=pltpu.CompilerParams(vmem_limit_bytes=100 * 1024 * 1024),
        name="infini_mod",
    )(A_beta, B_w_r, A_x[0].T, A_wq, A_wk, A_wv, A_wo, B_w_gate, B_w_up, B_w_down.T)
    return out_t.T[None]
```

```python
import math

import jax
import jax.numpy as jnp
from jax import lax
import jax.experimental.pallas as pl
import jax.experimental.pallas.tpu as pltpu

S = 2048
D = 576
H = 32
DH = D // H
NSEG = 4
L = S // NSEG
F = 4608
T = 128
HT = T // 2
NT_L = L // T
GH = 8
NG = H // GH
GR = GH * DH
WR = 4 * DH
NW = H // 4
WK = 80
FC = F // (NSEG - 1)
QSCALE = (DH ** -0.5) * math.log2(math.e)
NEG = -1e30
NB = 64
LAG = 1024
LAG0 = 2200
SYNC1 = 3
FFN_LAG = 2

F32 = jnp.float32
BF16 = jnp.bfloat16
U32 = jnp.uint32
NN = (((1,), (0,)), ((), ()))
NT = (((1,), (1,)), ((), ()))
KT = [(k, min(k + T, D)) for k in range(0, D, T)]


def _dot(a, b, dims=NN):
    return lax.dot_general(a, b, dims, preferred_element_type=F32)


def _bf(x):
    return pltpu.bitcast(x, BF16)


def _u(x):
    return pltpu.bitcast(x, U32)


def _pack(x):
    return _u(x.astype(BF16))


def _round(x):
    return x.astype(BF16).astype(F32)


def _phi(t):
    return jnp.where(t > 0, t + 1.0, jnp.exp(t))


def _iota(shape, dim):
    return lax.broadcasted_iota(jnp.int32, shape, dim)


def _ds(start, size, align):
    return pl.ds(start if isinstance(start, int) else pl.multiple_of(start, align), size)


def _interleave(main, fillers, per_step=4):
    fillers = list(fillers)
    for _ in main:
        for _ in range(per_step):
            while fillers and next(fillers[0], "done") == "done":
                fillers.pop(0)
    for f in fillers:
        for _ in f:
            pass


def _attention_schedule():
    qk, pv = [], []
    for hp in range(0, H, 2):
        for j in range(NT_L):
            qk.append(("x", hp, j, j * T + HT, HT))
            for h in (hp, hp + 1):
                qk += [("m", h, j, i * T, T) for i in range(j)] + [("m", h, j, j * T, HT)]
            pv += [(hp, j, i) for i in range(j)] + [(hp + 1, j, i) for i in range(j)]
            pv += [(hp, j, j), (hp + 1, j, j)]
    return qk, pv


def _kernel(beta_hbm, wr_hbm, x_hbm, wq_hbm, wk_hbm, wv_hbm, wo_hbm, wg_hbm, wu_hbm, wd_hbm,
            out_hbm,
            beta_v, wr_v, x_v, w_v, wg_v, wu_v, wd_v, wt, wot, xn, qs, kn, pq, pk, vv, rr, ot, ob, xs, vs, sc, mem, gt, bias,
            out_v, sem, fence):

    def seg(s):
        return _ds(s * L, L, L)

    def col(s, j):
        return _ds(s * L + j * T, T, T)

    def wide(ref, s, rows=slice(None)):
        return jnp.concatenate([ref[s * NT_L + n, rows, :] for n in range(NT_L)], axis=1)

    def put(ref, s, rows, value):
        for n in range(NT_L):
            ref[s * NT_L + n, rows, :] = value[:, n * T:(n + 1) * T]

    copy = pltpu.make_async_copy
    first_copies = [copy(beta_hbm, beta_v, sem.at[0]), copy(wr_hbm, wr_v, sem.at[0]),
                    copy(x_hbm.at[:, seg(0)], x_v.at[:, seg(0)], sem.at[0])]
    wk_copies = [copy(wk_hbm, w_v.at[1], sem.at[1])]
    wqv_copies = [copy(wq_hbm, w_v.at[0], sem.at[2]), copy(wv_hbm, w_v.at[2], sem.at[2])]
    x_copies = [copy(x_hbm.at[:, L:S], x_v.at[:, L:S], sem.at[3])]
    wo_copies = [copy(wo_hbm, w_v.at[3], sem.at[4])]

    def f_copies(i):
        return [copy(a.at[:, _ds(i * FC, FC, T)], b.at[i, :, 0:FC], sem.at[5 + i])
                for a, b in ((wg_hbm, wg_v), (wu_hbm, wu_v), (wd_hbm, wd_v))]

    o_parts = [(slice(0, D), seg(s)) for s in range(NSEG - 1)]
    o_parts += [(slice(g * GR, (g + 1) * GR), seg(NSEG - 1)) for g in range(NG)]
    o_copies = [copy(out_v.at[r, c], out_hbm.at[r, c], sem.at[0]) for r, c in o_parts]

    def wait(copies):
        for c in copies:
            c.wait()

    def layernorm(s, n):
        x = x_v[:, col(s, n)].astype(F32)
        mean = jnp.sum(x, axis=0, keepdims=True) * (1.0 / D)
        xc = x - mean
        var = jnp.sum(xc * xc, axis=0, keepdims=True) * (1.0 / D)
        sd = _round(jnp.sqrt(_round(_round(var) + _round(jnp.full((1, T), 1e-5, F32)))))
        y = _round(x - _round(mean)) * (1.0 / sd)
        xn[s * NT_L + n] = _u(y.astype(BF16))

    def load_weight(i):
        wt[i * D // 2:(i + 1) * D // 2, :] = _u(w_v[i].T)

    def finish_q(g, n, q, first=False):
        qs[n, g * GR // 2:(g + 1) * GR // 2, :] = _u((q * QSCALE).astype(BF16))
        if not first:
            pq[n, g * GR:(g + 1) * GR, :] = _phi(q)

    def finish_k(g, n, k):
        pk[n, g * GR:(g + 1) * GR, :] = _phi(k)
        kb = _u(k.astype(BF16))
        for w in range(2):
            blk = _bf(kb[w * (GR - WK) // 2:w * (GR - WK) // 2 + WK // 2])
            kn[2 * g + w, n * HT:(n + 1) * HT, :] = _u(blk.T)

    def project_group(i, g, finish, sync=None, s=None):
        src, s = (xs, 0) if s is None else (xn, s)
        rows = slice((i * D + g * GR) // 2, (i * D + (g + 1) * GR) // 2)
        tail = _dot(_bf(wt[rows, 4 * T:D]), _bf(wide(src, s, slice(2 * T, D // 2))))
        yield
        held = []
        for n in range(NT_L):
            held.append(_dot(_bf(wt[rows, 0:4 * T]), _bf(src[s * NT_L + n, 0:2 * T, :])) + tail[:, n * T:(n + 1) * T])
            yield
            if sync is None:
                finish(g, n, held[n])
        if sync is not None:
            sync()
            for n in range(NT_L):
                finish(g, n, held[n])

    for stage in (first_copies, wk_copies, wqv_copies, x_copies, f_copies(0), f_copies(1), f_copies(2), wo_copies):
        for c in stage:
            c.start()
        pl.semaphore_signal(fence, 1)
        pl.semaphore_wait(fence, 1)

    r64, c64 = _iota((HT, T), 0), _iota((HT, T), 1)
    bias[0] = jnp.where((c64 < HT) | (r64 <= c64 - HT), 0.0, NEG)
    bias[1] = jnp.where(r64 <= c64, 0.0, NEG)
    bias[2] = jnp.where(r64 <= c64 % HT, 0.0, NEG)
    mem[...] = jnp.zeros(mem.shape, F32)
    ot[...] = jnp.zeros(ot.shape, F32)
    wait(first_copies)
    g = jax.nn.sigmoid(beta_v[...].astype(F32)).reshape(1, H)
    own = _iota((H, H), 0) == _iota((H, H), 1)
    gcol = jnp.sum(jnp.where(own, jnp.broadcast_to(g, (H, H)), 0.0), axis=1, keepdims=True)
    gt[...] = jnp.broadcast_to(gcol, (H, T))
    wt[3 * D // 2:, :] = _pack(jnp.broadcast_to(wr_v[...].astype(F32).reshape(1, D), (16, D)))
    for n in range(NT_L):
        layernorm(0, n)
    wait(wk_copies)
    load_weight(1)

    def sync1():
        wait(wqv_copies)
        load_weight(0)
        load_weight(2)

    def first_q(g, sync=None):
        _interleave(project_group(0, g, lambda *a: finish_q(*a, first=True), sync, 0), [])

    for g in range(NG):
        _interleave(project_group(1, g, finish_k, sync1 if g == SYNC1 else None, 0), [])
    first_q(0)
    first_q(1)
    for s in range(NSEG):
        if s == 0:
            cut = 2 * GR
            put(vs, 0, slice(0, cut), _dot(_bf(wt[D:D + cut // 2, :]), _bf(wide(xn, 0))))
            first_q(2, lambda: wait(x_copies))
            v = _dot(_bf(wt[D + cut // 2:, :]), _bf(wide(xn, 0)))
            put(vs, 0, slice(cut, D), v[0:D - cut])
            rr[:, seg(0)] = v[D - cut:D - cut + 8]
        else:
            v = _dot(_bf(wt[D:, :]), _bf(wide(xn, s)))
            put(vv, s, slice(0, D), v[0:D])
            rr[:, seg(s)] = v[D:D + 8]
        if s < NSEG - 1:
            for n in range(NT_L):
                layernorm(s + 1, n)

    def top2():
        r = _round(rr[...])
        pos = _iota((8, S), 1).astype(F32)
        r0 = jnp.max(r, axis=1, keepdims=True)
        i0 = jnp.min(jnp.where(r == r0, pos, float(S)), axis=1, keepdims=True)
        r1 = jnp.max(jnp.where(pos == i0, -jnp.inf, r), axis=1, keepdims=True)
        i1 = jnp.min(jnp.where((r == r1) & (pos != i0), pos, float(S)), axis=1, keepdims=True)
        return (r0, r1), [jnp.clip(i[0, 0].astype(jnp.int32), 0, S - 1) for i in (i0, i1)]

    def gather(idx):
        parts = []
        for t in range(2):
            tile = idx[t] // T
            onehot = ((_iota((8, T), 0) == t) & (_iota((8, T), 1) == idx[t] - tile * T)).astype(F32)
            parts.append(_dot(onehot, _bf(xn[tile]), NT))
        return parts[0] + parts[1]

    (r0, r1), idx = top2()
    first_q(3)
    xsel = gather(idx)

    def ffn_steps(i, ys):
        n = FC // T
        hid = {}
        for f in range(n + FFN_LAG):
            if f < n:
                ab = []
                for w in (wg_v, wu_v):
                    a = None
                    for k0, k1 in KT:
                        d = _dot(xsel[:, k0:k1], w[i, k0:k1, f * T:(f + 1) * T])
                        a = d if a is None else a + d
                        yield
                    ab.append(a)
                hid[f] = ab[0] * jax.nn.sigmoid(ab[0]) * ab[1]
            if f >= FFN_LAG:
                h = hid.pop(f - FFN_LAG)
                for q, (k0, k1) in enumerate(KT):
                    ys[q] = ys[q] + _dot(h, wd_v[i, k0:k1, (f - FFN_LAG) * T:(f - FFN_LAG + 1) * T], NT)
                    yield

    qk, pv = _attention_schedule()

    def attend():
        row8 = _iota((8, T), 0)
        low = _iota((8, T), 1) < HT
        low32 = _iota((HT // 2, T), 1) < HT
        zero = jnp.uint32(0)
        qtile, mx, acc, slot, px = {}, {}, {}, {}, {}

        def q_rows(h, j):
            hg = h % GH
            r0 = (h // GH) * GR // 2 + 8 * hg
            q2 = qs[j, r0:r0 + 16, :]
            if h % 2 == 0:
                q2 = pltpu.roll(q2, HT, 1)
            r16 = _iota((16, T), 0)
            return jnp.where((r16 >= hg) & (r16 < hg + DH // 2), q2, zero)

        def q_pad(q, h):
            return _bf(jnp.concatenate([jnp.zeros((8 * (h % 4), T), U32), q], axis=0) if h % 4 else q)

        def scores(kind, h, j, k0, n):
            if kind == "x":
                qa, qb = q_rows(h, j), q_rows(h + 1, j)
                qtile[h], qtile[h + 1] = q_pad(qa, h), q_pad(qb, h + 1)
                rhs = q_pad(jnp.concatenate([jnp.where(low, qa[0:8], zero), jnp.where(low, qa[8:16], qb[0:8]),
                                             jnp.where(low, zero, qb[8:16])], axis=0), h)
            else:
                rhs = qtile[h]
            z = _dot(_bf(kn[h // 4, k0 // 2:(k0 + n) // 2, 0:rhs.shape[0]]), rhs)
            m8 = None
            for b in range(n // HT):
                zb = z[b * HT:(b + 1) * HT]
                key = k0 + b * HT
                if key >= j * T:
                    zb = zb + bias[2 if kind == "x" else h % 2]
                slot[kind, h, j, key] = len(slot) % NB
                sc[slot[kind, h, j, key]] = zb
                for rb in range(HT // 8):
                    m8 = zb[8 * rb:8 * rb + 8] if m8 is None else jnp.maximum(m8, zb[8 * rb:8 * rb + 8])
            if kind == "x":
                mx[h, j] = jnp.where(low, m8, NEG)
                mx[h + 1, j] = jnp.where(low, NEG, m8)
            else:
                m8 = jnp.maximum(m8, mx[h, j])
                mx[h, j] = jnp.max(m8, axis=0, keepdims=True) if k0 + n > j * T else m8

        def probs(key, m):
            assert len(slot) - list(slot).index(key) <= NB
            return jnp.exp2(sc[slot[key]] - m)

        def values(h, j, i):
            w, hi = h // 4, h % 4
            if i < j:
                p = jnp.concatenate([probs(("m", h, j, i * T + b * HT), mx[h, j]) for b in range(2)], axis=0)
                p = p.astype(BF16)
            else:
                if h % 2 == 0:
                    px[0] = _pack(probs(("x", h, j, j * T + HT), jnp.where(low[0:1], mx[h, j], mx[h + 1, j])))
                    upper = jnp.where(low32, px[0], zero)
                else:
                    upper = jnp.where(low32, zero, px[0])
                p = _bf(jnp.concatenate([_pack(probs(("m", h, j, j * T), mx[h, j])), upper], axis=0))
            v3 = vs[i, w * WR + 16 * hi:w * WR + 16 * hi + 24, :]
            if hi < 3:
                v3 = jnp.concatenate([v3[0:16], jnp.where(row8 == 7, 1.0, v3[16:24])], axis=0)
            else:
                v3 = jnp.concatenate([jnp.where(row8 == 0, 1.0, v3[0:8]), v3[8:24]], axis=0)
            o = _dot(v3, p)
            if i > 0:
                o = o + acc[h]
            acc[h] = o
            if i == j:
                if h % 2 == 0:
                    o = pltpu.roll(o, HT, 1)
                den = o[23:24] if hi < 3 else o[0:1]
                inv = pl.reciprocal(den, approx=True)
                res = o * ((1.0 - gt[h:h + 1, :]) * (inv * (2.0 - den * inv)))
                ot[j, h * DH:(h + 1) * DH, :] += res[2 * hi:2 * hi + DH]

        total, ready = 0, {}
        for _, h, j, _, n in qk:
            total += n
            ready[h, j] = total
        issued, tv = 0, 0
        for piece in qk:
            scores(*piece)
            issued += piece[4]
            while True:
                h, j, i = pv[tv]
                need = ready[h | 1, j] if i == j else ready[h, j]
                if issued < max(need + LAG, LAG0 + tv * total / len(pv)):
                    break
                values(h, j, i)
                tv += 1

        def drain():
            for tile in pv[tv:]:
                values(*tile)
                yield

        return drain()

    def memory_update(w):
        e = _iota((WR + 8, WR), 0)
        d = _iota((WR + 8, WR), 1)
        same_head = None
        for i in range(4):
            m = (d >= DH * i) & (d < DH * (i + 1)) & (((e >= DH * i) & (e < DH * (i + 1))) | (e == WR + i))
            same_head = m if same_head is None else same_head | m
        lhs = jnp.concatenate([wide(vs, 0, slice(w * WR, (w + 1) * WR)), jnp.ones((8, L), F32)], axis=0)
        return jnp.where(same_head, _dot(lhs, wide(pk, 0, slice(w * WR, (w + 1) * WR)), NT), 0.0)

    def memory_read(w):
        rt = _dot(mem[w], wide(pq, 0, slice(w * WR, (w + 1) * WR)))
        r8 = _iota((8, T), 0)
        g4 = jnp.zeros((8, T), F32)
        for i in range(4):
            g4 = jnp.where(r8 == i, gt[4 * w + i:4 * w + i + 1, :], g4)
        for n in range(NT_L):
            part = rt[:, n * T:(n + 1) * T]
            scale = g4 / (part[WR:WR + 8] + 1e-6)
            rows = []
            for b in range(WR // 8):
                lo, hi = 8 * b // DH, (8 * b + 7) // DH
                c = scale[lo:lo + 1]
                if hi != lo:
                    c = jnp.where(r8 < hi * DH - 8 * b, c, scale[hi:hi + 1])
                rows.append(part[8 * b:8 * b + 8] * c)
            ot[n, w * WR:(w + 1) * WR, :] = jnp.concatenate(rows, axis=0)

    def save_heads(s, g):
        for n in range(NT_L):
            ob[s * NT_L + n, g * GR // 2:(g + 1) * GR // 2, :] = _pack(ot[n, g * GR:(g + 1) * GR, :])

    def next_segment(s):
        for w in range(NW):
            upd = memory_update(w)
            yield
            mem[w] += upd
        for g in range(NG):
            yield from project_group(1, g, finish_k)
            save_heads(s, g)
            vs[g] = vv[(s + 1) * NT_L + g]
        for g, reads in enumerate(((), (), (0, 1), range(2, NW))):
            yield from project_group(0, g, finish_q)
            for w in reads:
                memory_read(w)
                yield

    def segment(s, y):
        wait(f_copies(s))
        for n in range(NT_L):
            xs[n] = xn[(s + 1) * NT_L + n]
        ys = [y[:, k0:k1] for k0, k1 in KT]
        _interleave(next_segment(s), [attend(), ffn_steps(s, ys)])
        return jnp.concatenate(ys, axis=1)

    y = lax.fori_loop(0, NSEG - 1, segment, jnp.zeros((8, D), F32))
    wait(wo_copies)

    gate = jax.nn.sigmoid(jnp.where(_iota((8, D), 0) == 0, r0, r1))
    y = jnp.where(_iota((8, D), 0) < 2, y * gate, 0.0)
    wot[:, 0:4 * T] = _u(w_v[3, 0:4 * T, :].T)
    tail = jnp.concatenate(
        [w_v[3, 4 * T:D, :], jnp.concatenate([y, jnp.zeros((8, D), F32)], axis=0).astype(BF16)], axis=0)
    wot[:, 4 * T:] = _u(tail.T)

    def project_out(i):
        s = min(i, NSEG - 1)
        rows = o_parts[i][0]
        half = slice(rows.start // 2, rows.stop // 2)
        tok = _iota((16, L), 1) + s * L
        r16 = _iota((16, L), 0)
        onehot = (((r16 == 0) & (tok == idx[0])) | ((r16 == 1) & (tok == idx[1]))).astype(F32)
        rhs = _bf(jnp.concatenate([wide(ob, s, slice(2 * T, D // 2)), _pack(onehot)], axis=0))
        last = _dot(_bf(wot[half, 4 * T:]), rhs)
        yield
        for n in range(NT_L):
            a = _dot(_bf(wot[half, 0:4 * T]), _bf(ob[s * NT_L + n, 0:2 * T, :])) + last[:, n * T:(n + 1) * T]
            res = x_v[rows, col(s, n)].astype(F32) + _bf(xn[s * NT_L + n, half, :]).astype(F32)
            out_v[rows, col(s, n)] = (a + res).astype(BF16)
            yield
        o_copies[i].start()

    drain = attend()
    _interleave(project_out(0), [drain])
    for g in range(NG):
        save_heads(NSEG - 1, g)
    for i in range(1, len(o_parts)):
        _interleave(project_out(i), [])
    wait(o_copies)


@jax.jit
def pallas_parallel_sum__memory_aug_infini_attn__moe_arch_mod__prompt_kernel(
    A_x: jax.Array,
    A_wq: jax.Array,
    A_wk: jax.Array,
    A_wv: jax.Array,
    A_wo: jax.Array,
    A_beta: jax.Array,
    B_x: jax.Array,
    B_w_r: jax.Array,
    B_w_gate: jax.Array,
    B_w_up: jax.Array,
    B_w_down: jax.Array,
):
    del B_x
    hbm = pl.BlockSpec(memory_space=pltpu.HBM)
    out_t = pl.pallas_call(
        _kernel,
        in_specs=[hbm] * 10,
        out_specs=hbm,
        out_shape=jax.ShapeDtypeStruct((D, S), BF16),
        scratch_shapes=[
            pltpu.VMEM((H,), BF16),
            pltpu.VMEM((D,), BF16),
            pltpu.VMEM((D, S + T), BF16),
            pltpu.VMEM((4, D, D), BF16),
            pltpu.VMEM((NSEG - 1, D, FC + T), BF16),
            pltpu.VMEM((NSEG - 1, D, FC + T), BF16),
            pltpu.VMEM((NSEG - 1, D, FC + T), BF16),
            pltpu.VMEM((3 * D // 2 + 8, D), U32),
            pltpu.VMEM((D // 2, D + 16), U32),
            pltpu.VMEM((S // T, D // 2, T), U32),
            pltpu.VMEM((NT_L, D // 2, T), U32),
            pltpu.VMEM((NW, L // 2, WK), U32),
            pltpu.VMEM((NT_L, D, T), F32),
            pltpu.VMEM((NT_L, D, T), F32),
            pltpu.VMEM((S // T, D, T), F32),
            pltpu.VMEM((8, S), F32),
            pltpu.VMEM((NT_L, D, T), F32),
            pltpu.VMEM((S // T, D // 2, T), U32),
            pltpu.VMEM((NT_L, D // 2, T), U32),
            pltpu.VMEM((NT_L, D, T), F32),
            pltpu.VMEM((NB, HT, T), F32),
            pltpu.VMEM((NW, WR + 8, WR), F32),
            pltpu.VMEM((H, T), F32),
            pltpu.VMEM((3, HT, T), F32),
            pltpu.VMEM((D, S + T), BF16),
            pltpu.SemaphoreType.DMA((5 + NSEG - 1,)),
            pltpu.SemaphoreType.REGULAR,
        ],
        compiler_params=pltpu.CompilerParams(vmem_limit_bytes=100 * 1024 * 1024),
        name="infini_mod",
    )(A_beta, B_w_r, A_x[0].T, A_wq, A_wk, A_wv, A_wo, B_w_gate, B_w_up, B_w_down.T)
    return out_t.T[None]
```

```python
import math

import jax
import jax.numpy as jnp
from jax import lax
import jax.experimental.pallas as pl
import jax.experimental.pallas.tpu as pltpu

S = 2048
D = 576
H = 32
DH = D // H
NSEG = 4
L = S // NSEG
F = 4608
T = 128
HT = T // 2
QT = T // 4
NT_L = L // T
GH = 8
NG = H // GH
GR = GH * DH
WR = 4 * DH
NW = H // 4
WK = 80
FC = F // (NSEG - 1)
QSCALE = (DH ** -0.5) * math.log2(math.e)
NEG = -1e30
NB = 192
MERGE = 0
LAG = 1024
LAG0 = 2800
SYNC1 = 3
FFN_LAG = 3

F32 = jnp.float32
BF16 = jnp.bfloat16
U32 = jnp.uint32
NN = (((1,), (0,)), ((), ()))
NT = (((1,), (1,)), ((), ()))
KT = [(k, min(k + T, D)) for k in range(0, D, T)]


def _dot(a, b, dims=NN):
    return lax.dot_general(a, b, dims, preferred_element_type=F32)


def _bf(x):
    return pltpu.bitcast(x, BF16)


def _u(x):
    return pltpu.bitcast(x, U32)


def _pack(x):
    return _u(x.astype(BF16))


def _round(x):
    return x.astype(BF16).astype(F32)


def _phi(t):
    return jnp.where(t > 0, t + 1.0, jnp.exp(t))


def _iota(shape, dim):
    return lax.broadcasted_iota(jnp.int32, shape, dim)


def _ds(start, size, align):
    return pl.ds(start if isinstance(start, int) else pl.multiple_of(start, align), size)


def _interleave(main, fillers, per_step=4):
    fillers = list(fillers)
    for _ in main:
        for _ in range(per_step):
            while fillers and next(fillers[0], "done") == "done":
                fillers.pop(0)
    for f in fillers:
        for _ in f:
            pass


ROT = (2, 0, 3, 1)
MIXES = {1: ((0, 0, 3, 0), (3, 1, 1, 1), (2, 2, 2, 3)), 2: ((0, 0, 1, 1), (3, 2, 2, 3)), 3: ((3, 0, 2, 1),)}
DIAG = [(0, (i,) * 4) for i in range(4)] + [(c, m) for c in MIXES for m in MIXES[c]]
assert all(sorted((m[p], (p - ROT[m[p]]) % 4) for cc, m in DIAG if cc == c for p in range(4))
           == [(i, a) for i in range(4) for a in range(c, 4)] for c in range(4))


def _attention_schedule():
    qk, pv = [], []
    for w in range(NW):
        for j in range(NT_L):
            qk += [(w, j, m, j * T + c * QT, QT) for c, m in DIAG[4:]]
            for i in range(4):
                own = [(t * T, T) for t in range(j)] + [(j * T, QT)]
                if MERGE and j > 0:
                    own = own[:-2] + [((j - 1) * T, T + QT)]
                qk += [(w, j, (i,) * 4, k0, n) for k0, n in own]
            pv += [(w, j, i, t) for i in range(4) for t in range(j)] + [(w, j, i, j) for i in range(4)]
    return qk, pv


def _kernel(beta_hbm, wr_hbm, x_hbm, wq_hbm, wk_hbm, wv_hbm, wo_hbm, wg_hbm, wu_hbm, wd_hbm,
            out_hbm,
            beta_v, wr_v, x_v, w_v, wg_v, wu_v, wd_v, wt, wvt, wot, xn, qs, kn, pq, pk, vv, rr, ot, ob, xs, vs, sc, mem, gt, bias, stat, zmem, ms,
            out_v, sem, fence):

    def seg(s):
        return _ds(s * L, L, L)

    def col(s, j):
        return _ds(s * L + j * T, T, T)

    def wide(ref, s, rows=slice(None)):
        return jnp.concatenate([ref[s * NT_L + n, rows, :] for n in range(NT_L)], axis=1)

    def put(ref, s, rows, value):
        for n in range(NT_L):
            ref[s * NT_L + n, rows, :] = value[:, n * T:(n + 1) * T]

    copy = pltpu.make_async_copy
    first_copies = [copy(beta_hbm, beta_v, sem.at[0]), copy(wr_hbm, wr_v, sem.at[0]),
                    copy(x_hbm.at[:, seg(0)], x_v.at[:, seg(0)], sem.at[0])]
    wk_copies = [copy(wk_hbm, w_v.at[1], sem.at[1])]
    wqv_copies = [copy(wq_hbm, w_v.at[0], sem.at[2]), copy(wv_hbm, w_v.at[2], sem.at[2])]
    x_copies = [copy(x_hbm.at[:, L:S], x_v.at[:, L:S], sem.at[3])]
    wo_copies = [copy(wo_hbm, w_v.at[3], sem.at[4])]

    def f_copies(i):
        return [copy(a.at[:, _ds(i * FC, FC, T)], b.at[i, :, 0:FC], sem.at[5 + i])
                for a, b in ((wg_hbm, wg_v), (wu_hbm, wu_v), (wd_hbm, wd_v))]

    o_parts = [(slice(0, D), s) for s in range(NSEG - 1)]
    o_parts += [(slice(g * GR, (g + 1) * GR), NSEG - 1) for g in range(NG)]
    o_copies = []

    def wait(copies):
        for c in copies:
            c.wait()

    def layernorm(s):
        def chunks(n):
            for r in range(0, D, 16):
                yield r, x_v[r:r + 16, col(s, n)].astype(F32)

        def total(parts):
            a = b = None
            for part in parts:
                a = part[0:8] if a is None else a + part[0:8]
                b = part[8:16] if b is None else b + part[8:16]
            return jnp.broadcast_to(jnp.sum(a + b, axis=0, keepdims=True) * (1.0 / D), (8, T))

        for n in range(NT_L):
            stat[0:8, col(0, n)] = total(x for _, x in chunks(n))
        for n in range(NT_L):
            mean = stat[0:1, col(0, n)]
            var = total(jnp.square(x - mean) for _, x in chunks(n))
            sd = _round(jnp.sqrt(_round(_round(var) + _round(jnp.full((8, T), 1e-5, F32)))))
            stat[8:16, col(0, n)] = 1.0 / sd
        for n in range(NT_L):
            mean, inv = _round(stat[0:1, col(0, n)]), stat[8:9, col(0, n)]
            for r, x in chunks(n):
                xn[s * NT_L + n, r // 2:r // 2 + 8, :] = _pack(_round(x - mean) * inv)

    def load_weight(i):
        wt[i * D // 2:(i + 1) * D // 2, :] = _u(w_v[i].T)

    def finish_q(g, n, q, first=False):
        qb = _pack(q * QSCALE)
        r16 = _iota((16, T), 0)
        for hg in range(GH):
            q2 = qb[8 * hg:8 * hg + 16]
            q2 = pltpu.roll(q2, ROT[hg % 4] * QT, 1) if ROT[hg % 4] else q2
            qs[n, g * GH + hg] = jnp.where((r16 >= hg) & (r16 < hg + DH // 2), q2, jnp.uint32(0))
        if not first:
            phi_q = _phi(q)
            pq[n, g * GR:(g + 1) * GR, :] = phi_q
            for w in range(2):
                memory_scale(2 * g + w, n, phi_q[w * WR:(w + 1) * WR])

    def finish_k(g, n, k):
        pk[n, g * GR:(g + 1) * GR, :] = _phi(k)
        kb = _u(k.astype(BF16))
        for w in range(2):
            blk = _bf(kb[w * (GR - WK) // 2:w * (GR - WK) // 2 + WK // 2])
            kn[2 * g + w, n * HT:(n + 1) * HT, :] = _u(blk.T)

    def project_group(i, g, finish, sync=None, s=None):
        src, s = (xs, 0) if s is None else (xn, s)
        rows = slice((i * D + g * GR) // 2, (i * D + (g + 1) * GR) // 2)
        tail = _dot(_bf(wt[rows, 4 * T:D]), _bf(wide(src, s, slice(2 * T, D // 2))))
        yield
        held = []
        for n in range(NT_L):
            held.append(_dot(_bf(wt[rows, 0:4 * T]), _bf(src[s * NT_L + n, 0:2 * T, :])) + tail[:, n * T:(n + 1) * T])
            yield
            if sync is None:
                finish(g, n, held[n])
        if sync is not None:
            sync()
            for n in range(NT_L):
                finish(g, n, held[n])

    for stage in (first_copies, wk_copies, wqv_copies, x_copies, f_copies(0), f_copies(1), f_copies(2), wo_copies):
        for c in stage:
            c.start()
        pl.semaphore_signal(fence, 1)
        pl.semaphore_wait(fence, 1)

    key, lane = _iota((QT, T), 0), _iota((QT, T), 1)
    for n, (c, mix) in enumerate(DIAG):
        hidden = key > lane % QT
        on_diag = [p for p in range(4) if (p - ROT[mix[p]]) % 4 == c]
        if len(on_diag) < 4:
            hidden = hidden & ((lane // QT == on_diag[0]) | (lane // QT == on_diag[-1]))
        bias[n] = jnp.where(hidden, NEG, 0.0)
    mem[...] = jnp.zeros(mem.shape, F32)
    zmem[...] = jnp.zeros(zmem.shape, F32)
    ot[...] = jnp.zeros(ot.shape, F32)
    wait(first_copies)
    g = jax.nn.sigmoid(beta_v[...].astype(F32)).reshape(1, H)
    own = _iota((H, H), 0) == _iota((H, H), 1)
    gcol = jnp.sum(jnp.where(own, jnp.broadcast_to(g, (H, H)), 0.0), axis=1, keepdims=True)
    gt[...] = jnp.broadcast_to(gcol, (H, T))
    wvt[D:, :] = jnp.broadcast_to(wr_v[...].astype(F32).reshape(1, D), (8, D))
    layernorm(0)
    wait(wk_copies)
    load_weight(1)

    def sync1():
        wait(wqv_copies)
        load_weight(0)
        wvt[0:D, :] = w_v[2].T.astype(F32)

    def first_q(g, sync=None):
        _interleave(project_group(0, g, lambda *a: finish_q(*a, first=True), sync, 0), [])

    for g in range(NG):
        _interleave(project_group(1, g, finish_k, sync1 if g == SYNC1 else None, 0), [])
    first_q(0)
    for s in range(NSEG):
        if s == 0:
            cut = 2 * GR
            put(vs, 0, slice(0, cut), _dot(wvt[0:cut, :], _bf(wide(xn, 0))))
            first_q(1, lambda: wait(x_copies))
            v = _dot(wvt[cut:, :], _bf(wide(xn, 0)))
            put(vs, 0, slice(cut, D), v[0:D - cut])
            rr[:, seg(0)] = v[D - cut:D - cut + 8]
            first_q(2)
        else:
            v = _dot(wvt[...], _bf(wide(xn, s)))
            put(vv, s, slice(0, D), v[0:D])
            rr[:, seg(s)] = v[D:D + 8]
        if s < NSEG - 1:
            layernorm(s + 1)

    def top2():
        r = _round(rr[...])
        pos = _iota((8, S), 1).astype(F32)
        r0 = jnp.max(r, axis=1, keepdims=True)
        i0 = jnp.min(jnp.where(r == r0, pos, float(S)), axis=1, keepdims=True)
        r1 = jnp.max(jnp.where(pos == i0, -jnp.inf, r), axis=1, keepdims=True)
        i1 = jnp.min(jnp.where((r == r1) & (pos != i0), pos, float(S)), axis=1, keepdims=True)
        return (r0, r1), (i0, i1)

    def gather(idx, xsel):
        for t in range(2):
            tile = idx[t] // T
            onehot = ((_iota((8, T), 0) == t) & (_iota((8, T), 1) == idx[t] - tile * T)).astype(F32)
            for q, (k0, k1) in enumerate(KT):
                part = _dot(onehot, _bf(xn[tile, k0 // 2:k1 // 2, :]), NT)
                xsel[q] = xsel[q] + part if t else part
                yield

    (r0, r1), picks = top2()
    first_q(3)
    idx = [jnp.clip(i[0, 0].astype(jnp.int32), 0, S - 1) for i in picks]

    def ffn_steps(i, xsel, ys):
        n = FC // T
        hid = {}
        for f in range(n + FFN_LAG):
            if f < n:
                ab = []
                for w in (wg_v, wu_v):
                    a = None
                    for q, (k0, k1) in enumerate(KT):
                        d = _dot(xsel[q], w[i, k0:k1, f * T:(f + 1) * T])
                        a = d if a is None else a + d
                        yield
                    ab.append(a)
                hid[f] = ab[0] * jax.nn.sigmoid(ab[0]) * ab[1]
            if f >= FFN_LAG:
                h = hid.pop(f - FFN_LAG)
                for q, (k0, k1) in enumerate(KT):
                    ys[q] = ys[q] + _dot(h, wd_v[i, k0:k1, (f - FFN_LAG) * T:(f - FFN_LAG + 1) * T], NT)
                    yield

    qk, pv = _attention_schedule()

    def attend():
        row8 = _iota((8, T), 0)
        zero = jnp.uint32(0)
        qrows, mx, acc, slot, mixed = {}, {}, {}, {}, {}

        def lanes(mix, i, rows):
            grp = _iota((rows, T), 1) // QT
            own = [p for p in range(4) if mix[p] == i]
            if len(own) > 2:
                return grp != [p for p in range(4) if p not in own][0]
            return (grp == own[0]) | (grp == own[-1])

        def q_operand(mix):
            blocks = []
            for r in range(max(mix) + 2):
                blk = jnp.zeros((8, T), U32)
                for i in (r - 1, r):
                    if i in mix:
                        part = qrows[i][8 * (r - i):8 * (r - i) + 8]
                        blk = part if len(set(mix)) == 1 else jnp.where(lanes(mix, i, 8), part, blk)
                blocks.append(blk)
            return _bf(jnp.concatenate(blocks, axis=0))

        def scores(w, j, mix, k0, n):
            if mix == DIAG[4][1]:
                for i in range(4):
                    qrows[i] = qs[j, 4 * w + i]
            rhs = q_operand(mix)
            z = _dot(_bf(kn[w, k0 // 2:(k0 + n) // 2, 0:rhs.shape[0]]), rhs)
            m8 = None
            for b in range(n // QT):
                zb = z[b * QT:(b + 1) * QT]
                key = k0 + b * QT
                if key >= j * T:
                    zb = zb + bias[DIAG.index(((key - j * T) // QT, mix))]
                slot[w, j, mix, key] = len(slot)
                sc[slot[w, j, mix, key] % NB] = zb
                for rb in range(QT // 8):
                    m8 = zb[8 * rb:8 * rb + 8] if m8 is None else jnp.maximum(m8, zb[8 * rb:8 * rb + 8])
            for i in sorted(set(mix)):
                mi = m8 if len(set(mix)) == 1 else jnp.where(lanes(mix, i, 8), m8, NEG)
                mx[w, j, i] = jnp.maximum(mx[w, j, i], mi) if (w, j, i) in mx else mi
            if len(set(mix)) == 1 and k0 + n > j * T:
                mx[w, j, mix[0]] = jnp.max(mx[w, j, mix[0]], axis=0, keepdims=True)

        def probs(w, j, mix, key):
            assert len(slot) - slot[w, j, mix, key] <= NB
            heads = sorted(set(mix))
            m = mx[w, j, heads[0]]
            for i in heads[1:]:
                m = jnp.where(lanes(mix, i, 1), mx[w, j, i], m)
            return jnp.exp2(sc[slot[w, j, mix, key] % NB] - m)

        def values(w, j, i, t):
            own = (i,) * 4
            if t < j:
                p = jnp.concatenate([probs(w, j, own, t * T + c * QT) for c in range(4)], axis=0).astype(BF16)
            else:
                parts = [_pack(probs(w, j, own, j * T))]
                for c in MIXES:
                    part = jnp.zeros((QT // 2, T), U32)
                    for m in MIXES[c]:
                        if i in m:
                            if (w, j, m) not in mixed:
                                mixed[w, j, m] = _pack(probs(w, j, m, j * T + c * QT))
                            part = jnp.where(lanes(m, i, QT // 2), mixed[w, j, m], part)
                    parts.append(part)
                p = _bf(jnp.concatenate(parts, axis=0))
            v3 = vs[t, w * WR + 16 * i:w * WR + 16 * i + 24, :]
            if i < 3:
                v3 = jnp.concatenate([v3[0:16], jnp.where(row8 == 7, 1.0, v3[16:24])], axis=0)
            else:
                v3 = jnp.concatenate([jnp.where(row8 == 0, 1.0, v3[0:8]), v3[8:24]], axis=0)
            o = _dot(v3, p)
            if t > 0:
                o = o + acc[i]
            acc[i] = o
            if t == j:
                h = 4 * w + i
                if ROT[i]:
                    o = pltpu.roll(o, T - ROT[i] * QT, 1)
                den = o[23:24] if i < 3 else o[0:1]
                inv = pl.reciprocal(den, approx=True)
                res = o * ((1.0 - gt[h:h + 1, :]) * (inv * (2.0 - den * inv)))
                ot[j, h * DH:(h + 1) * DH, :] += res[2 * i:2 * i + DH]

        total, ready = 0, {}
        for w, j, mix, _, n in qk:
            total += n
            ready[w, j, mix[0]] = total
        issued, tv = 0, 0
        for piece in qk:
            scores(*piece)
            issued += piece[4]
            while True:
                w, j, i, t = pv[tv]
                if issued < max(ready[w, j, 3 if t == j else i] + LAG, LAG0 + tv * total / len(pv)):
                    break
                values(w, j, i, t)
                tv += 1

        def drain():
            for tile in pv[tv:]:
                values(*tile)
                yield

        return drain()

    def memory_update(w):
        e = _iota((WR, WR), 0)
        d = _iota((WR, WR), 1)
        same_head = None
        for i in range(4):
            m = (d >= DH * i) & (d < DH * (i + 1)) & (e >= DH * i) & (e < DH * (i + 1))
            same_head = m if same_head is None else same_head | m
        rows = slice(w * WR, (w + 1) * WR)
        ksum = jnp.sum(sum(pk[n, rows, :] for n in range(1, NT_L)) + pk[0, rows, :], axis=1, keepdims=True)
        zmem[rows, :] += jnp.broadcast_to(ksum, (WR, T))
        return jnp.where(same_head, _dot(wide(vs, 0, rows), wide(pk, 0, rows), NT), 0.0)

    def by_head(b, of_head):
        lo, hi = 8 * b // DH, (8 * b + 7) // DH
        return of_head(lo) if lo == hi else jnp.where(_iota((8, T), 0) < hi * DH - 8 * b, of_head(lo), of_head(hi))

    def memory_scale(w, n, phi_q):
        prod = phi_q * zmem[w * WR:(w + 1) * WR, :]
        r8 = _iota((8, T), 0)
        den = gate = jnp.zeros((8, T), F32)
        for i in range(4):
            part = None
            for b in range(DH * i // 8, (DH * (i + 1) + 7) // 8):
                blk = prod[8 * b:8 * b + 8]
                if 8 * b < DH * i:
                    blk = jnp.where(r8 >= DH * i - 8 * b, blk, 0.0)
                elif 8 * b + 8 > DH * (i + 1):
                    blk = jnp.where(r8 < DH * (i + 1) - 8 * b, blk, 0.0)
                part = blk if part is None else part + blk
            den = jnp.where(r8 == i, jnp.sum(part, axis=0, keepdims=True), den)
            gate = jnp.where(r8 == i, gt[4 * w + i:4 * w + i + 1, :], gate)
        ms[n, w] = gate / (den + 1e-6)

    def memory_read(w):
        rt = _dot(mem[w], wide(pq, 0, slice(w * WR, (w + 1) * WR)))
        for n in range(NT_L):
            scale = ms[n, w]
            ot[n, w * WR:(w + 1) * WR, :] = jnp.concatenate(
                [rt[8 * b:8 * b + 8, n * T:(n + 1) * T] * by_head(b, lambda i: scale[i:i + 1])
                 for b in range(WR // 8)], axis=0)

    def save_heads(s, g):
        for n in range(NT_L):
            ob[s * NT_L + n, g * GR // 2:(g + 1) * GR // 2, :] = _pack(ot[n, g * GR:(g + 1) * GR, :])

    def next_segment(s):
        for w in range(NW):
            upd = memory_update(w)
            yield
            mem[w] += upd
        for g in range(NG):
            yield from project_group(1, g, finish_k)
            save_heads(s, g)
            vs[g] = vv[(s + 1) * NT_L + g]
        for g, reads in enumerate(((), (), (0, 1), range(2, NW))):
            yield from project_group(0, g, finish_q)
            for w in reads:
                memory_read(w)
                yield

    def segment(s, y):
        wait(f_copies(s))
        for n in range(NT_L):
            xs[n] = xn[(s + 1) * NT_L + n]
        ys = [y[:, k0:k1] for k0, k1 in KT]
        xsel = {}
        _interleave(next_segment(s), [gather(idx, xsel), attend(), ffn_steps(s, xsel, ys)])
        return jnp.concatenate(ys, axis=1)

    y = lax.fori_loop(0, NSEG - 1, segment, jnp.zeros((8, D), F32))
    wait(wo_copies)

    gate = jax.nn.sigmoid(jnp.where(_iota((8, D), 0) == 0, r0, r1))
    y = jnp.where(_iota((8, D), 0) < 2, y * gate, 0.0)
    wot[:, 0:4 * T] = _u(w_v[3, 0:4 * T, :].T)
    tail = jnp.concatenate(
        [w_v[3, 4 * T:D, :], jnp.concatenate([y, jnp.zeros((8, D), F32)], axis=0).astype(BF16)], axis=0)
    wot[:, 4 * T:] = _u(tail.T)

    def project_out(i):
        rows, s = o_parts[i]
        half = slice(rows.start // 2, rows.stop // 2)
        tok = _iota((16, L), 1) + s * L
        r16 = _iota((16, L), 0)
        onehot = (((r16 == 0) & (tok == idx[0])) | ((r16 == 1) & (tok == idx[1]))).astype(F32)
        rhs = _bf(jnp.concatenate([wide(ob, s, slice(2 * T, D // 2)), _pack(onehot)], axis=0))
        last = _dot(_bf(wot[half, 4 * T:]), rhs)
        yield
        for n in range(NT_L):
            a = _dot(_bf(wot[half, 0:4 * T]), _bf(ob[s * NT_L + n, 0:2 * T, :])) + last[:, n * T:(n + 1) * T]
            res = x_v[rows, col(s, n)].astype(F32) + _bf(xn[s * NT_L + n, half, :]).astype(F32)
            out_v[rows, col(s, n)] = (a + res).astype(BF16)
            last_part = i == len(o_parts) - 1 and n >= NT_L - 2
            if last_part or n == NT_L - 1:
                c = slice(s * L + (n * T if last_part and n == NT_L - 1 else 0), s * L + (n + 1) * T)
                o_copies.append(copy(out_v.at[rows, c], out_hbm.at[rows, c], sem.at[0]))
                o_copies[-1].start()
            yield

    drain = attend()
    _interleave(project_out(0), [drain])
    for g in range(NG):
        save_heads(NSEG - 1, g)
    for i in range(1, len(o_parts)):
        _interleave(project_out(i), [])
    wait(o_copies)


@jax.jit
def pallas_parallel_sum__memory_aug_infini_attn__moe_arch_mod__prompt_kernel(
    A_x: jax.Array,
    A_wq: jax.Array,
    A_wk: jax.Array,
    A_wv: jax.Array,
    A_wo: jax.Array,
    A_beta: jax.Array,
    B_x: jax.Array,
    B_w_r: jax.Array,
    B_w_gate: jax.Array,
    B_w_up: jax.Array,
    B_w_down: jax.Array,
):
    del B_x
    hbm = pl.BlockSpec(memory_space=pltpu.HBM)
    out_t = pl.pallas_call(
        _kernel,
        in_specs=[hbm] * 10,
        out_specs=hbm,
        out_shape=jax.ShapeDtypeStruct((D, S), BF16),
        scratch_shapes=[
            pltpu.VMEM((H,), BF16),
            pltpu.VMEM((D,), BF16),
            pltpu.VMEM((D, S + T), BF16),
            pltpu.VMEM((4, D, D), BF16),
            pltpu.VMEM((NSEG - 1, D, FC + T), BF16),
            pltpu.VMEM((NSEG - 1, D, FC + T), BF16),
            pltpu.VMEM((NSEG - 1, D, FC + T), BF16),
            pltpu.VMEM((D, D), U32),
            pltpu.VMEM((D + 8, D), F32),
            pltpu.VMEM((D // 2, D + 16), U32),
            pltpu.VMEM((S // T, D // 2, T), U32),
            pltpu.VMEM((NT_L, H, 16, T), U32),
            pltpu.VMEM((NW, L // 2, WK), U32),
            pltpu.VMEM((NT_L, D, T), F32),
            pltpu.VMEM((NT_L, D, T), F32),
            pltpu.VMEM((S // T, D, T), F32),
            pltpu.VMEM((8, S), F32),
            pltpu.VMEM((NT_L, D, T), F32),
            pltpu.VMEM((S // T, D // 2, T), U32),
            pltpu.VMEM((NT_L, D // 2, T), U32),
            pltpu.VMEM((NT_L, D, T), F32),
            pltpu.VMEM((NB, QT, T), F32),
            pltpu.VMEM((NW, WR, WR), F32),
            pltpu.VMEM((H, T), F32),
            pltpu.VMEM((len(DIAG), QT, T), F32),
            pltpu.VMEM((16, L), F32),
            pltpu.VMEM((D, T), F32),
            pltpu.VMEM((NT_L, NW, 8, T), F32),
            pltpu.VMEM((D, S + T), BF16),
            pltpu.SemaphoreType.DMA((5 + NSEG - 1,)),
            pltpu.SemaphoreType.REGULAR,
        ],
        compiler_params=pltpu.CompilerParams(vmem_limit_bytes=100 * 1024 * 1024),
        name="infini_mod",
    )(A_beta, B_w_r, A_x[0].T, A_wq, A_wk, A_wv, A_wo, B_w_gate, B_w_up, B_w_down.T)
    return out_t.T[None]
```

```python
import math

import jax
import jax.numpy as jnp
from jax import lax
import jax.experimental.pallas as pl
import jax.experimental.pallas.tpu as pltpu

S = 2048
D = 576
H = 32
DH = D // H
NSEG = 4
L = S // NSEG
F = 4608
T = 128
HT = T // 2
QT = T // 4
NT_L = L // T
GH = 8
NG = H // GH
GR = GH * DH
WR = 4 * DH
NW = H // 4
WK = 80
FC = F // (NSEG - 1)
QSCALE = (DH ** -0.5) * math.log2(math.e)
NEG = -1e30
NB = 192
MERGE = 0
LAG = 1024
LAG0 = 2800
SYNC1 = 3
FFN_LAG = 3

F32 = jnp.float32
BF16 = jnp.bfloat16
U32 = jnp.uint32
NN = (((1,), (0,)), ((), ()))
NT = (((1,), (1,)), ((), ()))
KT = [(k, min(k + T, D)) for k in range(0, D, T)]


def _dot(a, b, dims=NN):
    return lax.dot_general(a, b, dims, preferred_element_type=F32)


def _bf(x):
    return pltpu.bitcast(x, BF16)


def _u(x):
    return pltpu.bitcast(x, U32)


def _pack(x):
    return _u(x.astype(BF16))


def _round(x):
    return x.astype(BF16).astype(F32)


def _phi(t):
    return jnp.where(t > 0, t + 1.0, jnp.exp(t))


def _iota(shape, dim):
    return lax.broadcasted_iota(jnp.int32, shape, dim)


def _ds(start, size, align):
    return pl.ds(start if isinstance(start, int) else pl.multiple_of(start, align), size)


def _interleave(main, fillers, per_step=4):
    fillers = list(fillers)
    for _ in main:
        for _ in range(per_step):
            while fillers and next(fillers[0], "done") == "done":
                fillers.pop(0)
    for f in fillers:
        for _ in f:
            pass


ROT = (2, 0, 3, 1)
MIXES = {1: ((0, 0, 3, 0), (3, 1, 1, 1), (2, 2, 2, 3)), 2: ((0, 0, 1, 1), (3, 2, 2, 3)), 3: ((3, 0, 2, 1),)}
DIAG = [(0, (i,) * 4) for i in range(4)] + [(c, m) for c in MIXES for m in MIXES[c]]
assert all(sorted((m[p], (p - ROT[m[p]]) % 4) for cc, m in DIAG if cc == c for p in range(4))
           == [(i, a) for i in range(4) for a in range(c, 4)] for c in range(4))


def _attention_schedule():
    qk, pv = [], []
    for w in range(NW):
        for j in range(NT_L):
            qk += [(w, j, m, j * T + c * QT, QT) for c, m in DIAG[4:]]
            for i in range(4):
                own = [(t * T, T) for t in range(j)] + [(j * T, QT)]
                if MERGE and j > 0:
                    own = own[:-2] + [((j - 1) * T, T + QT)]
                qk += [(w, j, (i,) * 4, k0, n) for k0, n in own]
            pv += [(w, j, i, t) for i in range(4) for t in range(j)] + [(w, j, i, j) for i in range(4)]
    return qk, pv


def _kernel(beta_hbm, wr_hbm, x_hbm, wq_hbm, wk_hbm, wv_hbm, wo_hbm, wg_hbm, wu_hbm, wd_hbm,
            out_hbm,
            beta_v, wr_v, x_v, w_v, wg_v, wu_v, wd_v, wt, wvt, wot, xn, qs, kn, pq, pk, vv, rr, ot, ob, xs, vs, sc, mem, gt, bias, stat, zmem, ms,
            out_v, sem, fence):

    def seg(s):
        return _ds(s * L, L, L)

    def col(s, j):
        return _ds(s * L + j * T, T, T)

    def wide(ref, s, rows=slice(None)):
        return jnp.concatenate([ref[s * NT_L + n, rows, :] for n in range(NT_L)], axis=1)

    def put(ref, s, rows, value):
        for n in range(NT_L):
            ref[s * NT_L + n, rows, :] = value[:, n * T:(n + 1) * T]

    copy = pltpu.make_async_copy
    x_cols = [slice(0, L // 2), slice(L // 2, L), seg(1), slice(2 * L, S)]
    x_copies = [[copy(x_hbm.at[:, c], x_v.at[:, c], sem.at[i])] for i, c in enumerate(x_cols)]
    x_copies[0] = [copy(beta_hbm, beta_v, sem.at[0]), copy(wr_hbm, wr_v, sem.at[0])] + x_copies[0]
    wk_cols = [slice(0, 2 * T), slice(2 * T, D)]
    wk_copies = [[copy(wk_hbm.at[:, c], w_v.at[1, :, c], sem.at[4 + i])] for i, c in enumerate(wk_cols)]
    wq_copies = [copy(wq_hbm, w_v.at[0], sem.at[6])]
    wv_copies = [copy(wv_hbm, w_v.at[2], sem.at[7])]
    wo_copies = [copy(wo_hbm, w_v.at[3], sem.at[8])]

    def f_copies(i):
        return [copy(a.at[:, _ds(i * FC, FC, T)], b.at[i, :, 0:FC], sem.at[9 + i])
                for a, b in ((wg_hbm, wg_v), (wu_hbm, wu_v), (wd_hbm, wd_v))]

    o_parts = [(slice(0, D), s) for s in range(NSEG - 1)]
    o_parts += [(slice(g * GR, (g + 1) * GR), NSEG - 1) for g in range(NG)]
    o_copies = []

    def order():
        pl.semaphore_signal(fence, 1)
        pl.semaphore_wait(fence, 1)

    def wait(copies):
        for c in copies:
            c.wait()

    def layernorm(s, tiles=range(NT_L)):
        def chunks(n):
            for r in range(0, D, 16):
                yield r, x_v[r:r + 16, col(s, n)].astype(F32)

        def total(parts):
            a = b = None
            for part in parts:
                a = part[0:8] if a is None else a + part[0:8]
                b = part[8:16] if b is None else b + part[8:16]
            return jnp.broadcast_to(jnp.sum(a + b, axis=0, keepdims=True) * (1.0 / D), (8, T))

        for n in tiles:
            stat[0:8, col(0, n)] = total(x for _, x in chunks(n))
        for n in tiles:
            mean = stat[0:1, col(0, n)]
            var = total(jnp.square(x - mean) for _, x in chunks(n))
            sd = _round(jnp.sqrt(_round(_round(var) + _round(jnp.full((8, T), 1e-5, F32)))))
            stat[8:16, col(0, n)] = 1.0 / sd
        for n in tiles:
            mean, inv = _round(stat[0:1, col(0, n)]), stat[8:9, col(0, n)]
            for r, x in chunks(n):
                xn[s * NT_L + n, r // 2:r // 2 + 8, :] = _pack(_round(x - mean) * inv)
        return inv

    def load_weight(i):
        wt[i * D // 2:(i + 1) * D // 2, :] = _u(w_v[i].T)

    def finish_q(g, n, q, first=False):
        qb = _pack(q * QSCALE)
        r16 = _iota((16, T), 0)
        for hg in range(GH):
            q2 = qb[8 * hg:8 * hg + 16]
            q2 = pltpu.roll(q2, ROT[hg % 4] * QT, 1) if ROT[hg % 4] else q2
            qs[n, g * GH + hg] = jnp.where((r16 >= hg) & (r16 < hg + DH // 2), q2, jnp.uint32(0))
        if not first:
            phi_q = _phi(q)
            pq[n, g * GR:(g + 1) * GR, :] = phi_q
            for w in range(2):
                memory_scale(2 * g + w, n, phi_q[w * WR:(w + 1) * WR])

    def finish_k(g, n, k):
        pk[n, g * GR:(g + 1) * GR, :] = _phi(k)
        kb = _u(k.astype(BF16))
        for w in range(2):
            blk = _bf(kb[w * (GR - WK) // 2:w * (GR - WK) // 2 + WK // 2])
            kn[2 * g + w, n * HT:(n + 1) * HT, :] = _u(blk.T)

    def project_group(i, g, finish, s=None):
        src, s = (xs, 0) if s is None else (xn, s)
        rows = slice((i * D + g * GR) // 2, (i * D + (g + 1) * GR) // 2)
        tail = _dot(_bf(wt[rows, 4 * T:D]), _bf(wide(src, s, slice(2 * T, D // 2))))
        yield
        for n in range(NT_L):
            r = _dot(_bf(wt[rows, 0:4 * T]), _bf(src[s * NT_L + n, 0:2 * T, :])) + tail[:, n * T:(n + 1) * T]
            yield
            finish(g, n, r)

    for stage in (x_copies[0], x_copies[1], wk_copies[0], wk_copies[1], wq_copies, wv_copies, x_copies[2],
                  x_copies[3], f_copies(0), f_copies(1), f_copies(2), wo_copies):
        for c in stage:
            c.start()
        order()

    key, lane = _iota((QT, T), 0), _iota((QT, T), 1)
    for n, (c, mix) in enumerate(DIAG):
        hidden = key > lane % QT
        on_diag = [p for p in range(4) if (p - ROT[mix[p]]) % 4 == c]
        if len(on_diag) < 4:
            hidden = hidden & ((lane // QT == on_diag[0]) | (lane // QT == on_diag[-1]))
        bias[n] = jnp.where(hidden, NEG, 0.0)
    mem[...] = jnp.zeros(mem.shape, F32)
    zmem[...] = jnp.zeros(zmem.shape, F32)
    ot[...] = jnp.zeros(ot.shape, F32)

    def wait_w(copies, after):
        w_v[4, 0:16, 0:T] = jnp.broadcast_to(after[0:1], (16, T)).astype(BF16)
        wait(copies)

    def wait_x(copies, after):
        x_v[0:16, S:S + T] = jnp.broadcast_to(after[0:1], (16, T)).astype(BF16)
        wait(copies)

    def load_wk(i):
        c = wk_cols[i]
        wt[(D + c.start) // 2:(D + c.stop) // 2, :] = _u(w_v[1, :, c].T)

    order()
    wait(x_copies[0])
    g = jax.nn.sigmoid(beta_v[...].astype(F32)).reshape(1, H)
    own = _iota((H, H), 0) == _iota((H, H), 1)
    gcol = jnp.sum(jnp.where(own, jnp.broadcast_to(g, (H, H)), 0.0), axis=1, keepdims=True)
    gt[...] = jnp.broadcast_to(gcol, (H, T))
    wvt[D:, :] = jnp.broadcast_to(wr_v[...].astype(F32).reshape(1, D), (8, D))
    wait_x(x_copies[1], layernorm(0, range(0, 2)))
    wait_w(wk_copies[0], layernorm(0, range(2, 4)))
    load_wk(0)

    def hooked(finish, hooks):
        def run(g, n, r):
            finish(g, n, r)
            hooks.get((g, n), lambda r: None)(r)
        return run

    def put_wv(r):
        wait_w(wv_copies, r)
        wvt[0:D, :] = w_v[2].T.astype(F32)

    k_hooks = {(0, 1): lambda r: (wait_w(wk_copies[1], r), load_wk(1)),
               (2, 2): lambda r: (wait_w(wq_copies, r), load_weight(0))}
    q_hooks = {(0, 3): put_wv, (2, 1): lambda r: (wait_x(x_copies[2], r), layernorm(1))}
    first_q = hooked(lambda *a: finish_q(*a, first=True), q_hooks)
    for g in range(NG):
        _interleave(project_group(1, g, hooked(finish_k, k_hooks), 0), [])
    for g in range(NG - 1):
        _interleave(project_group(0, g, first_q, 0), [])
    for s in range(NSEG):
        v = _dot(wvt[...], _bf(wide(xn, s)))
        put(*((vv, s) if s else (vs, 0)), slice(0, D), v[0:D])
        rr[:, seg(s)] = v[D:D + 8]
        if s == 0:
            wait_x(x_copies[3], v[0:8, T:2 * T])
        if s < NSEG - 2:
            layernorm(s + 2)

    def top2():
        r = _round(rr[...])
        pos = _iota((8, S), 1).astype(F32)
        r0 = jnp.max(r, axis=1, keepdims=True)
        i0 = jnp.min(jnp.where(r == r0, pos, float(S)), axis=1, keepdims=True)
        r1 = jnp.max(jnp.where(pos == i0, -jnp.inf, r), axis=1, keepdims=True)
        i1 = jnp.min(jnp.where((r == r1) & (pos != i0), pos, float(S)), axis=1, keepdims=True)
        return (r0, r1), (i0, i1)

    def gather(idx, xsel):
        for t in range(2):
            tile = idx[t] // T
            onehot = ((_iota((8, T), 0) == t) & (_iota((8, T), 1) == idx[t] - tile * T)).astype(F32)
            for q, (k0, k1) in enumerate(KT):
                part = _dot(onehot, _bf(xn[tile, k0 // 2:k1 // 2, :]), NT)
                xsel[q] = xsel[q] + part if t else part
                yield

    (r0, r1), picks = top2()
    _interleave(project_group(0, NG - 1, first_q, 0), [])
    idx = [jnp.clip(i[0, 0].astype(jnp.int32), 0, S - 1) for i in picks]

    def ffn_steps(i, xsel, ys):
        n = FC // T
        hid = {}
        for f in range(n + FFN_LAG):
            if f < n:
                ab = []
                for w in (wg_v, wu_v):
                    a = None
                    for q, (k0, k1) in enumerate(KT):
                        d = _dot(xsel[q], w[i, k0:k1, f * T:(f + 1) * T])
                        a = d if a is None else a + d
                        yield
                    ab.append(a)
                hid[f] = ab[0] * jax.nn.sigmoid(ab[0]) * ab[1]
            if f >= FFN_LAG:
                h = hid.pop(f - FFN_LAG)
                for q, (k0, k1) in enumerate(KT):
                    ys[q] = ys[q] + _dot(h, wd_v[i, k0:k1, (f - FFN_LAG) * T:(f - FFN_LAG + 1) * T], NT)
                    yield

    qk, pv = _attention_schedule()

    def attend():
        row8 = _iota((8, T), 0)
        zero = jnp.uint32(0)
        qrows, mx, acc, slot, mixed = {}, {}, {}, {}, {}

        def lanes(mix, i, rows):
            grp = _iota((rows, T), 1) // QT
            own = [p for p in range(4) if mix[p] == i]
            if len(own) > 2:
                return grp != [p for p in range(4) if p not in own][0]
            return (grp == own[0]) | (grp == own[-1])

        def q_operand(mix):
            blocks = []
            for r in range(max(mix) + 2):
                blk = jnp.zeros((8, T), U32)
                for i in (r - 1, r):
                    if i in mix:
                        part = qrows[i][8 * (r - i):8 * (r - i) + 8]
                        blk = part if len(set(mix)) == 1 else jnp.where(lanes(mix, i, 8), part, blk)
                blocks.append(blk)
            return _bf(jnp.concatenate(blocks, axis=0))

        def scores(w, j, mix, k0, n):
            if mix == DIAG[4][1]:
                for i in range(4):
                    qrows[i] = qs[j, 4 * w + i]
            rhs = q_operand(mix)
            z = _dot(_bf(kn[w, k0 // 2:(k0 + n) // 2, 0:rhs.shape[0]]), rhs)
            m8 = None
            for b in range(n // QT):
                zb = z[b * QT:(b + 1) * QT]
                key = k0 + b * QT
                if key >= j * T:
                    zb = zb + bias[DIAG.index(((key - j * T) // QT, mix))]
                slot[w, j, mix, key] = len(slot)
                sc[slot[w, j, mix, key] % NB] = zb
                for rb in range(QT // 8):
                    m8 = zb[8 * rb:8 * rb + 8] if m8 is None else jnp.maximum(m8, zb[8 * rb:8 * rb + 8])
            for i in sorted(set(mix)):
                mi = m8 if len(set(mix)) == 1 else jnp.where(lanes(mix, i, 8), m8, NEG)
                mx[w, j, i] = jnp.maximum(mx[w, j, i], mi) if (w, j, i) in mx else mi
            if len(set(mix)) == 1 and k0 + n > j * T:
                mx[w, j, mix[0]] = jnp.max(mx[w, j, mix[0]], axis=0, keepdims=True)

        def probs(w, j, mix, key):
            assert len(slot) - slot[w, j, mix, key] <= NB
            heads = sorted(set(mix))
            m = mx[w, j, heads[0]]
            for i in heads[1:]:
                m = jnp.where(lanes(mix, i, 1), mx[w, j, i], m)
            return jnp.exp2(sc[slot[w, j, mix, key] % NB] - m)

        def values(w, j, i, t):
            own = (i,) * 4
            if t < j:
                p = jnp.concatenate([probs(w, j, own, t * T + c * QT) for c in range(4)], axis=0).astype(BF16)
            else:
                parts = [_pack(probs(w, j, own, j * T))]
                for c in MIXES:
                    part = jnp.zeros((QT // 2, T), U32)
                    for m in MIXES[c]:
                        if i in m:
                            if (w, j, m) not in mixed:
                                mixed[w, j, m] = _pack(probs(w, j, m, j * T + c * QT))
                            part = jnp.where(lanes(m, i, QT // 2), mixed[w, j, m], part)
                    parts.append(part)
                p = _bf(jnp.concatenate(parts, axis=0))
            v3 = vs[t, w * WR + 16 * i:w * WR + 16 * i + 24, :]
            if i < 3:
                v3 = jnp.concatenate([v3[0:16], jnp.where(row8 == 7, 1.0, v3[16:24])], axis=0)
            else:
                v3 = jnp.concatenate([jnp.where(row8 == 0, 1.0, v3[0:8]), v3[8:24]], axis=0)
            o = _dot(v3, p)
            if t > 0:
                o = o + acc[i]
            acc[i] = o
            if t == j:
                h = 4 * w + i
                if ROT[i]:
                    o = pltpu.roll(o, T - ROT[i] * QT, 1)
                den = o[23:24] if i < 3 else o[0:1]
                inv = pl.reciprocal(den, approx=True)
                res = o * ((1.0 - gt[h:h + 1, :]) * (inv * (2.0 - den * inv)))
                ot[j, h * DH:(h + 1) * DH, :] += res[2 * i:2 * i + DH]

        total, ready = 0, {}
        for w, j, mix, _, n in qk:
            total += n
            ready[w, j, mix[0]] = total
        issued, tv = 0, 0
        for piece in qk:
            scores(*piece)
            issued += piece[4]
            while True:
                w, j, i, t = pv[tv]
                if issued < max(ready[w, j, 3 if t == j else i] + LAG, LAG0 + tv * total / len(pv)):
                    break
                values(w, j, i, t)
                tv += 1

        def drain():
            for tile in pv[tv:]:
                values(*tile)
                yield

        return drain()

    def memory_update(w):
        e = _iota((WR, WR), 0)
        d = _iota((WR, WR), 1)
        same_head = None
        for i in range(4):
            m = (d >= DH * i) & (d < DH * (i + 1)) & (e >= DH * i) & (e < DH * (i + 1))
            same_head = m if same_head is None else same_head | m
        rows = slice(w * WR, (w + 1) * WR)
        ksum = jnp.sum(sum(pk[n, rows, :] for n in range(1, NT_L)) + pk[0, rows, :], axis=1, keepdims=True)
        zmem[rows, :] += jnp.broadcast_to(ksum, (WR, T))
        return jnp.where(same_head, _dot(wide(vs, 0, rows), wide(pk, 0, rows), NT), 0.0)

    def by_head(b, of_head):
        lo, hi = 8 * b // DH, (8 * b + 7) // DH
        return of_head(lo) if lo == hi else jnp.where(_iota((8, T), 0) < hi * DH - 8 * b, of_head(lo), of_head(hi))

    def memory_scale(w, n, phi_q):
        prod = phi_q * zmem[w * WR:(w + 1) * WR, :]
        r8 = _iota((8, T), 0)
        den = gate = jnp.zeros((8, T), F32)
        for i in range(4):
            part = None
            for b in range(DH * i // 8, (DH * (i + 1) + 7) // 8):
                blk = prod[8 * b:8 * b + 8]
                if 8 * b < DH * i:
                    blk = jnp.where(r8 >= DH * i - 8 * b, blk, 0.0)
                elif 8 * b + 8 > DH * (i + 1):
                    blk = jnp.where(r8 < DH * (i + 1) - 8 * b, blk, 0.0)
                part = blk if part is None else part + blk
            den = jnp.where(r8 == i, jnp.sum(part, axis=0, keepdims=True), den)
            gate = jnp.where(r8 == i, gt[4 * w + i:4 * w + i + 1, :], gate)
        ms[n, w] = gate / (den + 1e-6)

    def memory_read(w):
        rt = _dot(mem[w], wide(pq, 0, slice(w * WR, (w + 1) * WR)))
        for n in range(NT_L):
            scale = ms[n, w]
            ot[n, w * WR:(w + 1) * WR, :] = jnp.concatenate(
                [rt[8 * b:8 * b + 8, n * T:(n + 1) * T] * by_head(b, lambda i: scale[i:i + 1])
                 for b in range(WR // 8)], axis=0)

    def save_heads(s, g):
        for n in range(NT_L):
            ob[s * NT_L + n, g * GR // 2:(g + 1) * GR // 2, :] = _pack(ot[n, g * GR:(g + 1) * GR, :])

    def next_segment(s):
        for w in range(NW):
            upd = memory_update(w)
            yield
            mem[w] += upd
        for i, g, reads in ((0, 0, ()), (1, 0, (0,)), (0, 1, (1,)), (1, 1, (2,)), (0, 2, (3,)), (1, 2, ()),
                            (0, 3, ()), (1, 3, (4, 5, 6, 7))):
            yield from project_group(i, g, finish_k if i else finish_q)
            if i == 0:
                save_heads(s, g)
                vs[g] = vv[(s + 1) * NT_L + g]
            for w in reads:
                memory_read(w)
                yield

    def segment(s, y):
        wait(f_copies(s))
        order()
        for n in range(NT_L):
            xs[n] = xn[(s + 1) * NT_L + n]
        ys = [y[:, k0:k1] for k0, k1 in KT]
        xsel = {}
        _interleave(next_segment(s), [gather(idx, xsel), attend(), ffn_steps(s, xsel, ys)])
        return jnp.concatenate(ys, axis=1)

    y = lax.fori_loop(0, NSEG - 1, segment, jnp.zeros((8, D), F32))
    wait(wo_copies)

    gate = jax.nn.sigmoid(jnp.where(_iota((8, D), 0) == 0, r0, r1))
    y = jnp.where(_iota((8, D), 0) < 2, y * gate, 0.0)
    wot[:, 0:4 * T] = _u(w_v[3, 0:4 * T, :].T)
    tail = jnp.concatenate(
        [w_v[3, 4 * T:D, :], jnp.concatenate([y, jnp.zeros((8, D), F32)], axis=0).astype(BF16)], axis=0)
    wot[:, 4 * T:] = _u(tail.T)

    def project_out(i):
        rows, s = o_parts[i]
        half = slice(rows.start // 2, rows.stop // 2)
        tok = _iota((16, L), 1) + s * L
        r16 = _iota((16, L), 0)
        onehot = (((r16 == 0) & (tok == idx[0])) | ((r16 == 1) & (tok == idx[1]))).astype(F32)
        rhs = _bf(jnp.concatenate([wide(ob, s, slice(2 * T, D // 2)), _pack(onehot)], axis=0))
        last = _dot(_bf(wot[half, 4 * T:]), rhs)
        yield
        for n in range(NT_L):
            a = _dot(_bf(wot[half, 0:4 * T]), _bf(ob[s * NT_L + n, 0:2 * T, :])) + last[:, n * T:(n + 1) * T]
            res = x_v[rows, col(s, n)].astype(F32) + _bf(xn[s * NT_L + n, half, :]).astype(F32)
            out_v[rows, col(s, n)] = (a + res).astype(BF16)
            last_part = i == len(o_parts) - 1 and n >= NT_L - 2
            if last_part or n == NT_L - 1:
                c = slice(s * L + (n * T if last_part and n == NT_L - 1 else 0), s * L + (n + 1) * T)
                o_copies.append(copy(out_v.at[rows, c], out_hbm.at[rows, c], sem.at[0]))
                o_copies[-1].start()
            yield

    drain = attend()
    _interleave(project_out(0), [drain])
    for g in range(NG):
        save_heads(NSEG - 1, g)
    for i in range(1, len(o_parts)):
        _interleave(project_out(i), [])
    wait(o_copies)


@jax.jit
def pallas_parallel_sum__memory_aug_infini_attn__moe_arch_mod__prompt_kernel(
    A_x: jax.Array,
    A_wq: jax.Array,
    A_wk: jax.Array,
    A_wv: jax.Array,
    A_wo: jax.Array,
    A_beta: jax.Array,
    B_x: jax.Array,
    B_w_r: jax.Array,
    B_w_gate: jax.Array,
    B_w_up: jax.Array,
    B_w_down: jax.Array,
):
    del B_x
    hbm = pl.BlockSpec(memory_space=pltpu.HBM)
    out_t = pl.pallas_call(
        _kernel,
        in_specs=[hbm] * 10,
        out_specs=hbm,
        out_shape=jax.ShapeDtypeStruct((D, S), BF16),
        scratch_shapes=[
            pltpu.VMEM((H,), BF16),
            pltpu.VMEM((D,), BF16),
            pltpu.VMEM((D, S + T), BF16),
            pltpu.VMEM((5, D, D), BF16),
            pltpu.VMEM((NSEG - 1, D, FC + T), BF16),
            pltpu.VMEM((NSEG - 1, D, FC + T), BF16),
            pltpu.VMEM((NSEG - 1, D, FC + T), BF16),
            pltpu.VMEM((D, D), U32),
            pltpu.VMEM((D + 8, D), F32),
            pltpu.VMEM((D // 2, D + 16), U32),
            pltpu.VMEM((S // T, D // 2, T), U32),
            pltpu.VMEM((NT_L, H, 16, T), U32),
            pltpu.VMEM((NW, L // 2, WK), U32),
            pltpu.VMEM((NT_L, D, T), F32),
            pltpu.VMEM((NT_L, D, T), F32),
            pltpu.VMEM((S // T, D, T), F32),
            pltpu.VMEM((8, S), F32),
            pltpu.VMEM((NT_L, D, T), F32),
            pltpu.VMEM((S // T, D // 2, T), U32),
            pltpu.VMEM((NT_L, D // 2, T), U32),
            pltpu.VMEM((NT_L, D, T), F32),
            pltpu.VMEM((NB, QT, T), F32),
            pltpu.VMEM((NW, WR, WR), F32),
            pltpu.VMEM((H, T), F32),
            pltpu.VMEM((len(DIAG), QT, T), F32),
            pltpu.VMEM((16, L), F32),
            pltpu.VMEM((D, T), F32),
            pltpu.VMEM((NT_L, NW, 8, T), F32),
            pltpu.VMEM((D, S + T), BF16),
            pltpu.SemaphoreType.DMA((9 + NSEG - 1,)),
            pltpu.SemaphoreType.REGULAR,
        ],
        compiler_params=pltpu.CompilerParams(vmem_limit_bytes=100 * 1024 * 1024, flags={"XLA_TPU_RESCHEDULE_DMA_DONES": True}),
        name="infini_mod",
    )(A_beta, B_w_r, A_x[0].T, A_wq, A_wk, A_wv, A_wo, B_w_gate, B_w_up, B_w_down.T)
    return out_t.T[None]
```

```python
import functools
import math

import jax
import jax.numpy as jnp
from jax import lax
import jax.experimental.pallas as pl
import jax.experimental.pallas.tpu as pltpu

S = 2048
D = 576
H = 32
DH = D // H
NSEG = 4
L = S // NSEG
F = 4608
T = 128
QT = T // 4
NTL = L // T
GH = 8
NG = H // GH
GR = GH * DH
WR = 4 * DH
NW = H // 4
WK = 80
FC = F // (NSEG - 1)
QSCALE = DH ** -0.5 * math.log2(math.e)
RING = 192
LAG = 1024
LEAD = 2800
FFN_LAG = 3

F32 = jnp.float32
BF16 = jnp.bfloat16
U32 = jnp.uint32
NN = (((1,), (0,)), ((), ()))
NT = (((1,), (1,)), ((), ()))
KT = [(k, min(k + T, D)) for k in range(0, D, T)]

ROT = (2, 0, 3, 1)
MIXES = {1: ((0, 0, 3, 0), (3, 1, 1, 1), (2, 2, 2, 3)), 2: ((0, 0, 1, 1), (3, 2, 2, 3)), 3: ((3, 0, 2, 1),)}
DIAG = [(0, (i,) * 4) for i in range(4)] + [(c, m) for c in MIXES for m in MIXES[c]]
assert all(sorted((m[p], (p - ROT[m[p]]) % 4) for cc, m in DIAG if cc == c for p in range(4))
           == [(i, a) for i in range(4) for a in range(c, 4)] for c in range(4))


def _dot(a, b, dims=NN):
    return lax.dot_general(a, b, dims, preferred_element_type=F32)


def _bf(x):
    return pltpu.bitcast(x, BF16)


def _u(x):
    return pltpu.bitcast(x, U32)


def _pack(x):
    return _u(x.astype(BF16))


def _round(x):
    return x.astype(BF16).astype(F32)


def _phi(t):
    return jnp.where(t > 0, t + 1.0, jnp.exp(t))


def _iota(shape, dim):
    return lax.broadcasted_iota(jnp.int32, shape, dim)


def _span(i, n):
    return slice(i * n, (i + 1) * n)


def _wide(ref, s, rows=slice(None)):
    return jnp.concatenate([ref[s * NTL + n, rows, :] for n in range(NTL)], axis=1)


def _start(copies):
    for c in copies:
        c.start()


def _wait(copies):
    for c in copies:
        c.wait()


def _interleave(main, fillers=(), per_step=4):
    fillers = list(fillers)
    for _ in main:
        for _ in range(per_step):
            while fillers and next(fillers[0], "done") == "done":
                fillers.pop(0)
    for f in fillers:
        for _ in f:
            pass


def _attention_schedule():
    qk, pv = [], []
    for w in range(NW):
        for j in (0, 2, 1, 3):
            qk += [(w, j, m, j * T + c * QT, QT) for c, m in DIAG[4:]]
            for i in range(4):
                qk += [(w, j, (i,) * 4, j * T, QT)] + [(w, j, (i,) * 4, t * T, T) for t in range(j)]
            pv += [(w, j, i, t) for i in range(4) for t in range(j)] + [(w, j, i, j) for i in range(4)]
    return qk, pv


def _compute(beta_hbm, wr_hbm, x_hbm, wq_hbm, wk_hbm, wv_hbm, wo_hbm, wg_hbm, wu_hbm, wd_hbm, out_hbm,
             beta_v, wr_v, x_v, w_v, wg_v, wu_v, wd_v, out_v, wt, wvt, wot, stat, xn, xs, qs, kn, pq, pk,
             vv, vs, rr, sc, ot, ob, mem, zmem, ms, gt, bias, out_sem, *, out_copies, sem, fence):
    copy = pltpu.make_async_copy
    x_cols = [slice(0, L // 2), slice(L // 2, L), _span(1, L), slice(2 * L, S)]
    x_copies = [[copy(x_hbm.at[:, c], x_v.at[:, c], sem.at[i])] for i, c in enumerate(x_cols)]
    x_copies[0] = [copy(beta_hbm, beta_v, sem.at[0]), copy(wr_hbm, wr_v, sem.at[0])] + x_copies[0]
    wk_cols = [slice(0, 2 * T), slice(2 * T, D)]
    wk_copies = [[copy(wk_hbm.at[:, c], w_v.at[1, :, c], sem.at[4 + i])] for i, c in enumerate(wk_cols)]
    wq_copies = [copy(wq_hbm, w_v.at[0], sem.at[6])]
    wv_copies = [copy(wv_hbm, w_v.at[2], sem.at[7])]
    wo_copies = [copy(wo_hbm, w_v.at[3], sem.at[8])]

    def ffn_copies(i):
        c = _span(i, FC) if isinstance(i, int) else pl.ds(pl.multiple_of(i * FC, T), FC)
        return [copy(a.at[:, c], b.at[i, :, 0:FC], sem.at[9 + i])
                for a, b in ((wg_hbm, wg_v), (wu_hbm, wu_v), (wd_hbm, wd_v))]

    def order():
        pl.semaphore_signal(fence, 1)
        pl.semaphore_wait(fence, 1)

    def wait_w(copies, after):
        w_v[4, 0:16, 0:T] = jnp.broadcast_to(after[0:1], (16, T)).astype(BF16)
        _wait(copies)

    def wait_x(copies, after):
        x_v[0:16, S:S + T] = jnp.broadcast_to(after[0:1], (16, T)).astype(BF16)
        _wait(copies)

    for stage in (x_copies[0], x_copies[1], wk_copies[0], wk_copies[1], wq_copies, wv_copies, x_copies[2],
                  x_copies[3], ffn_copies(0), ffn_copies(1), ffn_copies(2), wo_copies):
        _start(stage)
        order()

    key, lane = _iota((QT, T), 0), _iota((QT, T), 1)
    for n, (c, mix) in enumerate(DIAG):
        hidden = key > lane % QT
        on_diag = [p for p in range(4) if (p - ROT[mix[p]]) % 4 == c]
        if len(on_diag) < 4:
            hidden = hidden & ((lane // QT == on_diag[0]) | (lane // QT == on_diag[-1]))
        bias[n] = jnp.where(hidden, -jnp.inf, 0.0)
    mem[...] = jnp.zeros(mem.shape, F32)
    zmem[...] = jnp.zeros(zmem.shape, F32)
    ot[...] = jnp.zeros(ot.shape, F32)
    ob[NTL:3 * NTL] = jnp.zeros((2 * NTL, D // 2, T), U32)
    order()

    def layernorm(s, tiles=range(NTL)):
        def chunks(n):
            for r in range(0, D, 16):
                yield r, x_v[r:r + 16, _span(s * NTL + n, T)].astype(F32)

        def mean_of(parts):
            a = b = None
            for part in parts:
                a = part[0:8] if a is None else a + part[0:8]
                b = part[8:16] if b is None else b + part[8:16]
            return jnp.broadcast_to(jnp.sum(a + b, axis=0, keepdims=True) * (1.0 / D), (8, T))

        for n in tiles:
            stat[0:8, _span(n, T)] = mean_of(x for _, x in chunks(n))
        for n in tiles:
            mean = stat[0:1, _span(n, T)]
            var = mean_of(jnp.square(x - mean) for _, x in chunks(n))
            sd = _round(jnp.sqrt(_round(_round(var) + _round(jnp.full((8, T), 1e-5, F32)))))
            stat[8:16, _span(n, T)] = 1.0 / sd
        for n in tiles:
            mean, inv = _round(stat[0:1, _span(n, T)]), stat[8:9, _span(n, T)]
            for r, x in chunks(n):
                y = _pack(_round(x - mean) * inv)
                xn[s * NTL + n, r // 2:r // 2 + 8, :] = y
                if s:
                    xs[s * NTL + n, r // 2:r // 2 + 8, :] = y
        return inv

    def finish_q(g, n, q, reads_memory=True):
        qb = _pack(q * QSCALE)
        r16 = _iota((16, T), 0)
        for hg in range(GH):
            q2 = qb[8 * hg:8 * hg + 16]
            q2 = pltpu.roll(q2, ROT[hg % 4] * QT, 1) if ROT[hg % 4] else q2
            qs[n, g * GH + hg] = jnp.where((r16 >= hg) & (r16 < hg + DH // 2), q2, jnp.uint32(0))
        if reads_memory:
            phi_q = _phi(q)
            pq[n, _span(g, GR), :] = phi_q
            for w in range(2):
                memory_scale(2 * g + w, n, phi_q[_span(w, WR)])

    def finish_k(g, n, k):
        pk[n, _span(g, GR), :] = _phi(k)
        kb = _pack(k)
        for w in range(2):
            r0 = w * (GR - WK) // 2
            kn[2 * g + w, _span(n, T // 2), :] = _u(_bf(kb[r0:r0 + WK // 2]).T)

    def project(i, g, finish, src):
        rows = _span(i * NG + g, GR // 2)
        last = _dot(_bf(wt[rows, 4 * T:D]), _bf(_wide(src, 0, slice(2 * T, D // 2))))
        yield
        for n in range(NTL):
            r = _dot(_bf(wt[rows, 0:4 * T]), _bf(src[n, 0:2 * T, :])) + last[:, _span(n, T)]
            yield
            finish(g, n, r)

    def top2():
        r = _round(rr[...])
        pos = _iota((8, S), 1).astype(F32)
        r0 = jnp.max(r, axis=1, keepdims=True)
        i0 = jnp.min(jnp.where(r == r0, pos, float(S)), axis=1, keepdims=True)
        r1 = jnp.max(jnp.where(pos == i0, -jnp.inf, r), axis=1, keepdims=True)
        i1 = jnp.min(jnp.where((r == r1) & (pos != i0), pos, float(S)), axis=1, keepdims=True)
        return (r0, r1), (i0, i1)

    def gather(idx, xsel):
        for t in range(2):
            tile = idx[t] // T
            onehot = ((_iota((8, T), 0) == t) & (_iota((8, T), 1) == idx[t] - tile * T)).astype(F32)
            for q, (k0, k1) in enumerate(KT):
                part = _dot(onehot, _bf(xn[tile, k0 // 2:k1 // 2, :]), NT)
                xsel[q] = xsel[q] + part if t else part
                yield

    def ffn(i, xsel, ys):
        hid = {}
        for f in range(FC // T + FFN_LAG):
            if f < FC // T:
                ab = []
                for w in (wg_v, wu_v):
                    a = None
                    for q, (k0, k1) in enumerate(KT):
                        d = _dot(xsel[q], w[i, k0:k1, _span(f, T)])
                        a = d if a is None else a + d
                        yield
                    ab.append(a)
                hid[f] = ab[0] * jax.nn.sigmoid(ab[0]) * ab[1]
            if f >= FFN_LAG:
                h = hid.pop(f - FFN_LAG)
                for q, (k0, k1) in enumerate(KT):
                    ys[q] = ys[q] + _dot(h, wd_v[i, k0:k1, _span(f - FFN_LAG, T)], NT)
                    yield

    def attend():
        qk, pv = _attention_schedule()
        row8 = _iota((8, T), 0)
        qrows, mx, acc, slot, mixed = {}, {}, {}, {}, {}

        def lanes(mix, i, rows):
            grp = _iota((rows, T), 1) // QT
            own = [p for p in range(4) if mix[p] == i]
            if len(own) == 3:
                return grp != [p for p in range(4) if p not in own][0]
            return (grp == own[0]) | (grp == own[-1])

        def q_operand(mix):
            blocks = []
            for r in range(max(mix) + 2):
                blk = jnp.zeros((8, T), U32)
                for i in (r - 1, r):
                    if i in mix:
                        part = qrows[i][_span(r - i, 8)]
                        blk = part if len(set(mix)) == 1 else jnp.where(lanes(mix, i, 8), part, blk)
                blocks.append(blk)
            return _bf(jnp.concatenate(blocks, axis=0))

        def scores(w, j, mix, k0, n):
            if mix == DIAG[4][1]:
                for i in range(4):
                    qrows[i] = qs[j, 4 * w + i]
            rhs = q_operand(mix)
            z = _dot(_bf(kn[w, k0 // 2:(k0 + n) // 2, 0:rhs.shape[0]]), rhs)
            m8 = None
            for b in range(n // QT):
                zb = z[_span(b, QT)]
                key = k0 + b * QT
                if key >= j * T:
                    zb = zb + bias[DIAG.index(((key - j * T) // QT, mix))]
                slot[w, j, mix, key] = len(slot)
                sc[slot[w, j, mix, key] % RING] = zb
                for rb in range(QT // 8):
                    m8 = zb[_span(rb, 8)] if m8 is None else jnp.maximum(m8, zb[_span(rb, 8)])
            for i in sorted(set(mix)):
                mi = m8 if len(set(mix)) == 1 else jnp.where(lanes(mix, i, 8), m8, -jnp.inf)
                mx[w, j, i] = jnp.maximum(mx[w, j, i], mi) if (w, j, i) in mx else mi
            if len(set(mix)) == 1 and (j == 0 or k0 + n == j * T):
                mx[w, j, mix[0]] = jnp.max(mx[w, j, mix[0]], axis=0, keepdims=True)

        def probs(w, j, mix, key):
            heads = sorted(set(mix))
            assert len(slot) - slot[w, j, mix, key] <= RING and all(mx[w, j, i].shape[0] == 1 for i in heads)
            m = mx[w, j, heads[0]]
            for i in heads[1:]:
                m = jnp.where(lanes(mix, i, 1), mx[w, j, i], m)
            return jnp.exp2(sc[slot[w, j, mix, key] % RING] - m)

        def values(w, j, i, t):
            own = (i,) * 4
            if t < j:
                p = jnp.concatenate([probs(w, j, own, t * T + c * QT) for c in range(4)], axis=0).astype(BF16)
            else:
                parts = [_pack(probs(w, j, own, j * T))]
                for c in MIXES:
                    part = jnp.zeros((QT // 2, T), U32)
                    for m in MIXES[c]:
                        if i in m:
                            if (w, j, m) not in mixed:
                                mixed[w, j, m] = _pack(probs(w, j, m, j * T + c * QT))
                            part = jnp.where(lanes(m, i, QT // 2), mixed[w, j, m], part)
                    parts.append(part)
                p = _bf(jnp.concatenate(parts, axis=0))
            v3 = vs[t, w * WR + 16 * i:w * WR + 16 * i + 24, :]
            if i < 3:
                v3 = jnp.concatenate([v3[0:16], jnp.where(row8 == 7, 1.0, v3[16:24])], axis=0)
            else:
                v3 = jnp.concatenate([jnp.where(row8 == 0, 1.0, v3[0:8]), v3[8:24]], axis=0)
            o = _dot(v3, p)
            if t > 0:
                o = o + acc[i]
            acc[i] = o
            if t == j:
                h = 4 * w + i
                if ROT[i]:
                    o = pltpu.roll(o, T - ROT[i] * QT, 1)
                den = o[23:24] if i < 3 else o[0:1]
                inv = pl.reciprocal(den, approx=True)
                res = o * ((1.0 - gt[h:h + 1, :]) * (inv * (2.0 - den * inv)))
                ot[j, _span(h, DH), :] += res[2 * i:2 * i + DH]

        total, ready = 0, {}
        for w, j, mix, _, n in qk:
            total += n
            ready[w, j, mix[0]] = total
        issued, step = 0, total / len(pv)
        due = LEAD
        for piece in qk:
            scores(*piece)
            issued += piece[4]
            while True:
                w, j, i, t = pv[0]
                if issued < max(ready[w, j, 3 if t == j else i] + LAG, due):
                    break
                values(*pv.pop(0))
                due += step

        def drain():
            while pv:
                values(*pv.pop(0))
                yield

        return drain(), pv

    def memory_update(w):
        e, d = _iota((WR, WR), 0), _iota((WR, WR), 1)
        same_head = None
        for i in range(4):
            m = (d >= DH * i) & (d < DH * (i + 1)) & (e >= DH * i) & (e < DH * (i + 1))
            same_head = m if same_head is None else same_head | m
        rows = _span(w, WR)
        ksum = (pk[0, rows, :] + pk[1, rows, :]) + (pk[2, rows, :] + pk[3, rows, :])
        zmem[rows, :] += jnp.broadcast_to(jnp.sum(ksum, axis=1, keepdims=True), (WR, T))
        return jnp.where(same_head, _dot(_wide(vs, 0, rows), _wide(pk, 0, rows), NT), 0.0)

    def memory_scale(w, n, phi_q):
        prod = phi_q * zmem[_span(w, WR), :]
        r8 = _iota((8, T), 0)
        den = gate = jnp.zeros((8, T), F32)
        for i in range(4):
            part = None
            for b in range(DH * i // 8, (DH * (i + 1) + 7) // 8):
                blk = prod[_span(b, 8)]
                if 8 * b < DH * i:
                    blk = jnp.where(r8 >= DH * i - 8 * b, blk, 0.0)
                elif 8 * b + 8 > DH * (i + 1):
                    blk = jnp.where(r8 < DH * (i + 1) - 8 * b, blk, 0.0)
                part = blk if part is None else part + blk
            den = jnp.where(r8 == i, jnp.sum(part, axis=0, keepdims=True), den)
            gate = jnp.where(r8 == i, gt[4 * w + i:4 * w + i + 1, :], gate)
        ms[n, w] = gate / (den + 1e-6)

    def memory_read(w):
        num = _dot(mem[w], _wide(pq, 0, _span(w, WR)))
        for n in range(NTL):
            scale, blocks = ms[n, w], []
            for b in range(WR // 8):
                lo, hi = 8 * b // DH, (8 * b + 7) // DH
                c = scale[lo:lo + 1]
                if hi != lo:
                    c = jnp.where(_iota((8, T), 0) < hi * DH - 8 * b, c, scale[hi:hi + 1])
                blocks.append(num[_span(b, 8), _span(n, T)] * c)
            ot[n, _span(w, WR), :] = jnp.concatenate(blocks, axis=0)

    def save_heads(s, g):
        for n in range(NTL):
            ob[s * NTL + n, _span(g, GR // 2), :] = _pack(ot[n, _span(g, GR), :])

    def next_segment(outstanding):
        for w in range(NW):
            update = memory_update(w)
            yield
            mem[w] += update
        for i, g, reads in ((0, 0, ()), (1, 0, (0,)), (0, 1, (1,)), (1, 1, (2,)), (0, 2, (3,)), (1, 2, ()),
                            (0, 3, ()), (1, 3, (4, 5, 6, 7))):
            yield from project(i, g, finish_k if i else finish_q, xs)
            if i == 0:
                assert not outstanding
                save_heads(NSEG - 2, g)
                vs[g] = _bf(vv[g]).astype(F32)
            for w in reads:
                memory_read(w)
                yield

    _wait(x_copies[0])
    gate = jnp.broadcast_to(jax.nn.sigmoid(beta_v[...].astype(F32)).reshape(1, H), (H, H))
    gate = jnp.sum(jnp.where(_iota((H, H), 0) == _iota((H, H), 1), gate, 0.0), axis=1, keepdims=True)
    gt[...] = jnp.broadcast_to(gate, (H, T))
    wvt[D:, :] = jnp.broadcast_to(wr_v[...].astype(F32).reshape(1, D), (8, D))
    wait_x(x_copies[1], layernorm(0, range(0, 2)))

    def load_wk(i, after):
        wait_w(wk_copies[i], after)
        c = wk_cols[i]
        wt[(D + c.start) // 2:(D + c.stop) // 2, :] = _u(w_v[1, :, c].T)

    def first_k(g, n, r):
        finish_k(g, n, r)
        if (g, n) == (0, 1):
            load_wk(1, r)
        elif (g, n) == (2, 2):
            wait_w(wq_copies, r)
            wt[0:D // 2, :] = _u(w_v[0].T)

    def first_q(g, n, r):
        finish_q(g, n, r, reads_memory=False)
        if (g, n) == (0, 3):
            wait_w(wv_copies, r)
            wvt[0:D, :] = w_v[2].T.astype(F32)
        elif (g, n) == (2, 1):
            wait_x(x_copies[2], r)
            layernorm(1)

    load_wk(0, layernorm(0, range(2, 4)))
    for g in range(NG):
        _interleave(project(1, g, first_k, xn))
    for g in range(NG - 1):
        _interleave(project(0, g, first_q, xn))
    for s in range(NSEG):
        v = _dot(wvt[...], _bf(_wide(xn, s)))
        for n in range(NTL):
            if s:
                vv[s * NTL + n] = _pack(v[0:D, _span(n, T)])
            else:
                vs[n] = v[0:D, _span(n, T)]
        rr[:, _span(s, L)] = v[D:]
        if s == 0:
            wait_x(x_copies[3], v[0:8, _span(1, T)])
        if s < NSEG - 2:
            layernorm(s + 2)
    (r0, r1), picks = top2()
    _interleave(project(0, NG - 1, first_q, xn))
    idx = [jnp.clip(i[0, 0].astype(jnp.int32), 0, S - 1) for i in picks]

    def segment(s, y):
        _wait(ffn_copies(s))
        order()
        for n in range(NTL):
            for i in range(NSEG - 1):
                xs[i * NTL + n] = xs[(i + 1) * NTL + n]
                vv[i * NTL + n] = vv[(i + 1) * NTL + n]
            for i in range(NSEG - 2):
                ob[i * NTL + n] = ob[(i + 1) * NTL + n]
        ys = [y[:, k0:k1] for k0, k1 in KT]
        xsel = {}
        drain, outstanding = attend()
        _interleave(next_segment(outstanding), [gather(idx, xsel), drain, ffn(s, xsel, ys)])
        return jnp.concatenate(ys, axis=1)

    y = lax.fori_loop(0, NSEG - 1, segment, jnp.zeros((8, D), F32))

    _wait(wo_copies)
    row = _iota((8, D), 0)
    y = jnp.where(row < 2, y * jax.nn.sigmoid(jnp.where(row == 0, r0, r1)), 0.0)
    wot[:, 0:4 * T] = _u(w_v[3, 0:4 * T, :].T)
    y = jnp.concatenate([y, jnp.zeros((8, D), F32)], axis=0).astype(BF16)
    wot[:, 4 * T:] = _u(jnp.concatenate([w_v[3, 4 * T:D, :], y], axis=0).T)

    def project_out(rows, s, cuts=(0, NTL)):
        half = slice(rows.start // 2, rows.stop // 2)
        tok, r16 = _iota((16, L), 1) + s * L, _iota((16, L), 0)
        onehot = (((r16 == 0) & (tok == idx[0])) | ((r16 == 1) & (tok == idx[1]))).astype(F32)
        rhs = jnp.concatenate([_wide(ob, s, slice(2 * T, D // 2)), _pack(onehot)], axis=0)
        last = _dot(_bf(wot[half, 4 * T:]), _bf(rhs))
        yield
        for n in range(NTL):
            tile = s * NTL + n
            a = _dot(_bf(wot[half, 0:4 * T]), _bf(ob[tile, 0:2 * T, :])) + last[:, _span(n, T)]
            res = x_v[rows, _span(tile, T)].astype(F32) + _bf(xn[tile, half, :]).astype(F32)
            out_v[rows, _span(tile, T)] = (a + res).astype(BF16)
            if n + 1 in cuts:
                c = slice(s * L + cuts[cuts.index(n + 1) - 1] * T, (tile + 1) * T)
                out_copies.append(copy(out_v.at[rows, c], out_hbm.at[rows, c], out_sem))
                out_copies[-1].start()
            yield

    _interleave(project_out(slice(0, D), 0), [attend()[0]])
    for g in range(NG):
        save_heads(NSEG - 1, g)
    for s in range(1, NSEG - 1):
        _interleave(project_out(slice(0, D), s))
    for g in range(NG):
        _interleave(project_out(_span(g, GR), NSEG - 1, (0, NTL) if g < NG - 1 else (0, NTL - 1, NTL)))


def _kernel(*refs):
    out_copies = []
    pl.run_scoped(functools.partial(_compute, *refs, out_copies=out_copies),
                  sem=pltpu.SemaphoreType.DMA((9 + NSEG - 1,)), fence=pltpu.SemaphoreType.REGULAR)
    _wait(out_copies)


@jax.jit
def pallas_parallel_sum__memory_aug_infini_attn__moe_arch_mod__prompt_kernel(
    A_x: jax.Array,
    A_wq: jax.Array,
    A_wk: jax.Array,
    A_wv: jax.Array,
    A_wo: jax.Array,
    A_beta: jax.Array,
    B_x: jax.Array,
    B_w_r: jax.Array,
    B_w_gate: jax.Array,
    B_w_up: jax.Array,
    B_w_down: jax.Array,
):
    del B_x
    hbm = pl.BlockSpec(memory_space=pltpu.HBM)
    packed = pltpu.VMEM((S // T, D // 2, T), U32)
    segment = pltpu.VMEM((NTL, D, T), F32)
    ffn_weight = pltpu.VMEM((NSEG - 1, D, FC + T), BF16)
    out_t = pl.pallas_call(
        _kernel,
        in_specs=[hbm] * 10,
        out_specs=hbm,
        out_shape=jax.ShapeDtypeStruct((D, S), BF16),
        scratch_shapes=[
            pltpu.VMEM((H,), BF16),
            pltpu.VMEM((D,), BF16),
            pltpu.VMEM((D, S + T), BF16),
            pltpu.VMEM((5, D, D), BF16),
            ffn_weight, ffn_weight, ffn_weight,
            pltpu.VMEM((D, S + T), BF16),
            pltpu.VMEM((D, D), U32),
            pltpu.VMEM((D + 8, D), F32),
            pltpu.VMEM((D // 2, D + 16), U32),
            pltpu.VMEM((16, L), F32),
            packed, packed,
            pltpu.VMEM((NTL, H, 16, T), U32),
            pltpu.VMEM((NW, L // 2, WK), U32),
            segment, segment,
            packed, segment,
            pltpu.VMEM((8, S), F32),
            pltpu.VMEM((RING, QT, T), F32),
            segment, packed,
            pltpu.VMEM((NW, WR, WR), F32),
            pltpu.VMEM((D, T), F32),
            pltpu.VMEM((NTL, NW, 8, T), F32),
            pltpu.VMEM((H, T), F32),
            pltpu.VMEM((len(DIAG), QT, T), F32),
            pltpu.SemaphoreType.DMA,
        ],
        compiler_params=pltpu.CompilerParams(
            vmem_limit_bytes=100 * 1024 * 1024,
            flags={"XLA_TPU_RESCHEDULE_DMA_DONES": True},
        ),
        name="infini_mod",
    )(A_beta, B_w_r, A_x[0].T, A_wq, A_wk, A_wv, A_wo, B_w_gate, B_w_up, B_w_down.T)
    return out_t.T[None]
```

```python
import functools
import math

import jax
import jax.numpy as jnp
from jax import lax
import jax.experimental.pallas as pl
import jax.experimental.pallas.tpu as pltpu

S = 2048
D = 576
H = 32
DH = D // H
NSEG = 4
L = S // NSEG
F = 4608
T = 128
QT = T // 4
NTL = L // T
GH = 8
NG = H // GH
GR = GH * DH
WR = 4 * DH
NW = H // 4
WK = 80
FC = F // (NSEG - 1)
QSCALE = DH ** -0.5 * math.log2(math.e)
RING = 192
LAG = 1024
LEAD = 2800
FFN_LAG = 3

F32 = jnp.float32
BF16 = jnp.bfloat16
U32 = jnp.uint32
NN = (((1,), (0,)), ((), ()))
NT = (((1,), (1,)), ((), ()))
KT = [(k, min(k + T, D)) for k in range(0, D, T)]

ROT = (2, 0, 3, 1)
MIXES = {1: ((0, 0, 3, 0), (3, 1, 1, 1), (2, 2, 2, 3)), 2: ((0, 0, 1, 1), (3, 2, 2, 3)), 3: ((3, 0, 2, 1),)}
DIAG = [(0, (i,) * 4) for i in range(4)] + [(c, m) for c in MIXES for m in MIXES[c]]
assert all(sorted((m[p], (p - ROT[m[p]]) % 4) for cc, m in DIAG if cc == c for p in range(4))
           == [(i, a) for i in range(4) for a in range(c, 4)] for c in range(4))


def _dot(a, b, dims=NN):
    return lax.dot_general(a, b, dims, preferred_element_type=F32)


def _bf(x):
    return pltpu.bitcast(x, BF16)


def _u(x):
    return pltpu.bitcast(x, U32)


def _pack(x):
    return _u(x.astype(BF16))


def _round(x):
    return x.astype(BF16).astype(F32)


def _phi(t):
    return jnp.where(t > 0, t + 1.0, jnp.exp(t))


def _iota(shape, dim):
    return lax.broadcasted_iota(jnp.int32, shape, dim)


def _span(i, n):
    return slice(i * n, (i + 1) * n)


def _wide(ref, s, rows=slice(None)):
    return jnp.concatenate([ref[s * NTL + n, rows, :] for n in range(NTL)], axis=1)


def _start(copies):
    for c in copies:
        c.start()


def _wait(copies):
    for c in copies:
        c.wait()


def _interleave(main, fillers=(), per_step=4):
    fillers = list(fillers)
    for _ in main:
        for _ in range(per_step):
            while fillers and next(fillers[0], "done") == "done":
                fillers.pop(0)
    for f in fillers:
        for _ in f:
            pass


def _attention_schedule():
    qk, pv = [], []
    for w in range(NW):
        for j in (0, 2, 1, 3):
            qk += [(w, j, m, j * T + c * QT, QT) for c, m in DIAG[4:]]
            for i in range(4):
                qk += [(w, j, (i,) * 4, j * T, QT)] + [(w, j, (i,) * 4, t * T, T) for t in range(j)]
            pv += [(w, j, i, t) for i in range(4) for t in range(j)] + [(w, j, i, j) for i in range(4)]
    return qk, pv


def _compute(beta_hbm, wr_hbm, x_hbm, wq_hbm, wk_hbm, wv_hbm, wo_hbm, wg_hbm, wu_hbm, wd_hbm, out_hbm,
             beta_v, wr_v, x_v, w_v, wg_v, wu_v, wd_v, out_v, wt, wvt, wot, stat, xn, xs, qs, kn, pq, pk,
             vv, vs, rr, sc, ot, ob, mem, zmem, ms, gt, bias, out_sem, *, out_copies, sem, fence):
    copy = pltpu.make_async_copy
    x_cols = [slice(0, L // 2), slice(L // 2, L), _span(1, L), slice(2 * L, S)]
    x_copies = [[copy(x_hbm.at[:, c], x_v.at[:, c], sem.at[i])] for i, c in enumerate(x_cols)]
    x_copies[0] = [copy(beta_hbm, beta_v, sem.at[0]), copy(wr_hbm, wr_v, sem.at[0])] + x_copies[0]
    wk_cols = [slice(0, 2 * T), slice(2 * T, D)]
    wk_copies = [[copy(wk_hbm.at[:, c], w_v.at[1, :, c], sem.at[4 + i])] for i, c in enumerate(wk_cols)]
    wq_copies = [copy(wq_hbm, w_v.at[0], sem.at[6])]
    wv_copies = [copy(wv_hbm, w_v.at[2], sem.at[7])]
    wo_copies = [copy(wo_hbm, w_v.at[3], sem.at[8])]

    def ffn_copies(i):
        c = _span(i, FC) if isinstance(i, int) else pl.ds(pl.multiple_of(i * FC, T), FC)
        return [copy(a.at[:, c], b.at[i, :, 0:FC], sem.at[9 + i])
                for a, b in ((wg_hbm, wg_v), (wu_hbm, wu_v), (wd_hbm, wd_v))]

    def order():
        pl.semaphore_signal(fence, 1)
        pl.semaphore_wait(fence, 1)

    def wait_w(copies, after):
        w_v[4, 0:16, 0:T] = jnp.broadcast_to(after[0:1], (16, T)).astype(BF16)
        _wait(copies)

    def wait_x(copies, after):
        x_v[0:16, S:S + T] = jnp.broadcast_to(after[0:1], (16, T)).astype(BF16)
        _wait(copies)

    for stage in (x_copies[0], x_copies[1], wk_copies[0], wk_copies[1], wq_copies, wv_copies, x_copies[2],
                  x_copies[3], ffn_copies(0), ffn_copies(1), ffn_copies(2), wo_copies):
        _start(stage)
        order()

    key, lane = _iota((QT, T), 0), _iota((QT, T), 1)
    for n, (c, mix) in enumerate(DIAG):
        hidden = key > lane % QT
        on_diag = [p for p in range(4) if (p - ROT[mix[p]]) % 4 == c]
        if len(on_diag) < 4:
            hidden = hidden & ((lane // QT == on_diag[0]) | (lane // QT == on_diag[-1]))
        bias[n] = jnp.where(hidden, -jnp.inf, 0.0)
    mem[...] = jnp.zeros(mem.shape, F32)
    zmem[...] = jnp.zeros(zmem.shape, F32)
    ot[...] = jnp.zeros(ot.shape, F32)
    ob[NTL:3 * NTL] = jnp.zeros((2 * NTL, D // 2, T), U32)
    order()

    def layernorm(s, tiles=range(NTL)):
        def chunks(n):
            for r in range(0, D, 16):
                yield r, x_v[r:r + 16, _span(s * NTL + n, T)].astype(F32)

        def mean_of(parts):
            a = b = None
            for part in parts:
                a = part[0:8] if a is None else a + part[0:8]
                b = part[8:16] if b is None else b + part[8:16]
            return jnp.broadcast_to(jnp.sum(a + b, axis=0, keepdims=True) * (1.0 / D), (8, T))

        for n in tiles:
            stat[0:8, _span(n, T)] = mean_of(x for _, x in chunks(n))
        for n in tiles:
            mean = stat[0:1, _span(n, T)]
            var = mean_of(jnp.square(x - mean) for _, x in chunks(n))
            sd = _round(jnp.sqrt(_round(_round(var) + _round(jnp.full((8, T), 1e-5, F32)))))
            stat[8:16, _span(n, T)] = 1.0 / sd
        for n in tiles:
            mean, inv = _round(stat[0:1, _span(n, T)]), stat[8:9, _span(n, T)]
            for r, x in chunks(n):
                last = _round(x - mean) * inv
                y = _pack(last)
                xn[s * NTL + n, r // 2:r // 2 + 8, :] = y
                if s:
                    xs[s * NTL + n, r // 2:r // 2 + 8, :] = y
        return inv, last

    def finish_q(g, n, q, reads_memory=True):
        qb = _pack(q * QSCALE)
        r16 = _iota((16, T), 0)
        for hg in range(GH):
            q2 = qb[8 * hg:8 * hg + 16]
            q2 = pltpu.roll(q2, ROT[hg % 4] * QT, 1) if ROT[hg % 4] else q2
            qs[n, g * GH + hg] = jnp.where((r16 >= hg) & (r16 < hg + DH // 2), q2, jnp.uint32(0))
        if reads_memory:
            phi_q = _phi(q)
            pq[n, _span(g, GR), :] = phi_q
            for w in range(2):
                memory_scale(2 * g + w, n, phi_q[_span(w, WR)])

    def finish_k(g, n, k):
        pk[n, _span(g, GR), :] = _phi(k)
        kb = _pack(k)
        for w in range(2):
            r0 = w * (GR - WK) // 2
            kn[2 * g + w, _span(n, T // 2), :] = _u(_bf(kb[r0:r0 + WK // 2]).T)

    def project(i, g, finish, src):
        rows = _span(i * NG + g, GR // 2)
        last = _dot(_bf(wt[rows, 4 * T:D]), _bf(_wide(src, 0, slice(2 * T, D // 2))))
        yield
        for n in range(NTL):
            r = _dot(_bf(wt[rows, 0:4 * T]), _bf(src[n, 0:2 * T, :])) + last[:, _span(n, T)]
            yield
            finish(g, n, r)

    def top2():
        r = _round(rr[...])
        pos = _iota((8, S), 1).astype(F32)
        r0 = jnp.max(r, axis=1, keepdims=True)
        i0 = jnp.min(jnp.where(r == r0, pos, float(S)), axis=1, keepdims=True)
        r1 = jnp.max(jnp.where(pos == i0, -jnp.inf, r), axis=1, keepdims=True)
        i1 = jnp.min(jnp.where((r == r1) & (pos != i0), pos, float(S)), axis=1, keepdims=True)
        return (r0, r1), (i0, i1)

    def gather(idx, xsel):
        for t in range(2):
            tile = idx[t] // T
            onehot = ((_iota((8, T), 0) == t) & (_iota((8, T), 1) == idx[t] - tile * T)).astype(F32)
            for q, (k0, k1) in enumerate(KT):
                part = _dot(onehot, _bf(xn[tile, k0 // 2:k1 // 2, :]), NT)
                xsel[q] = xsel[q] + part if t else part
                yield

    def ffn(i, xsel, ys):
        hid = {}
        for f in range(FC // T + FFN_LAG):
            if f < FC // T:
                ab = []
                for w in (wg_v, wu_v):
                    a = None
                    for q, (k0, k1) in enumerate(KT):
                        d = _dot(xsel[q], w[i, k0:k1, _span(f, T)])
                        a = d if a is None else a + d
                        yield
                    ab.append(a)
                hid[f] = ab[0] * jax.nn.sigmoid(ab[0]) * ab[1]
            if f >= FFN_LAG:
                h = hid.pop(f - FFN_LAG)
                for q, (k0, k1) in enumerate(KT):
                    ys[q] = ys[q] + _dot(h, wd_v[i, k0:k1, _span(f - FFN_LAG, T)], NT)
                    yield

    def attend():
        qk, pv = _attention_schedule()
        row8 = _iota((8, T), 0)
        qrows, mx, acc, slot, mixed = {}, {}, {}, {}, {}

        def lanes(mix, i, rows):
            grp = _iota((rows, T), 1) // QT
            own = [p for p in range(4) if mix[p] == i]
            if len(own) == 3:
                return grp != [p for p in range(4) if p not in own][0]
            return (grp == own[0]) | (grp == own[-1])

        def q_operand(mix):
            blocks = []
            for r in range(max(mix) + 2):
                blk = jnp.zeros((8, T), U32)
                for i in (r - 1, r):
                    if i in mix:
                        part = qrows[i][_span(r - i, 8)]
                        blk = part if len(set(mix)) == 1 else jnp.where(lanes(mix, i, 8), part, blk)
                blocks.append(blk)
            return _bf(jnp.concatenate(blocks, axis=0))

        def scores(w, j, mix, k0, n):
            if mix == DIAG[4][1]:
                for i in range(4):
                    qrows[i] = qs[j, 4 * w + i]
            rhs = q_operand(mix)
            z = _dot(_bf(kn[w, k0 // 2:(k0 + n) // 2, 0:rhs.shape[0]]), rhs)
            m8 = None
            for b in range(n // QT):
                zb = z[_span(b, QT)]
                key = k0 + b * QT
                if key >= j * T:
                    zb = zb + bias[DIAG.index(((key - j * T) // QT, mix))]
                slot[w, j, mix, key] = len(slot)
                sc[slot[w, j, mix, key] % RING] = zb
                for rb in range(QT // 8):
                    m8 = zb[_span(rb, 8)] if m8 is None else jnp.maximum(m8, zb[_span(rb, 8)])
            for i in sorted(set(mix)):
                mi = m8 if len(set(mix)) == 1 else jnp.where(lanes(mix, i, 8), m8, -jnp.inf)
                mx[w, j, i] = jnp.maximum(mx[w, j, i], mi) if (w, j, i) in mx else mi
            if len(set(mix)) == 1 and (j == 0 or k0 + n == j * T):
                mx[w, j, mix[0]] = jnp.max(mx[w, j, mix[0]], axis=0, keepdims=True)

        def probs(w, j, mix, key):
            heads = sorted(set(mix))
            assert len(slot) - slot[w, j, mix, key] <= RING and all(mx[w, j, i].shape[0] == 1 for i in heads)
            m = mx[w, j, heads[0]]
            for i in heads[1:]:
                m = jnp.where(lanes(mix, i, 1), mx[w, j, i], m)
            return jnp.exp2(sc[slot[w, j, mix, key] % RING] - m)

        def values(w, j, i, t):
            own = (i,) * 4
            if t < j:
                p = jnp.concatenate([probs(w, j, own, t * T + c * QT) for c in range(4)], axis=0).astype(BF16)
            else:
                parts = [_pack(probs(w, j, own, j * T))]
                for c in MIXES:
                    part = jnp.zeros((QT // 2, T), U32)
                    for m in MIXES[c]:
                        if i in m:
                            if (w, j, m) not in mixed:
                                mixed[w, j, m] = _pack(probs(w, j, m, j * T + c * QT))
                            part = jnp.where(lanes(m, i, QT // 2), mixed[w, j, m], part)
                    parts.append(part)
                p = _bf(jnp.concatenate(parts, axis=0))
            v3 = vs[t, w * WR + 16 * i:w * WR + 16 * i + 24, :]
            if i < 3:
                v3 = jnp.concatenate([v3[0:16], jnp.where(row8 == 7, 1.0, v3[16:24])], axis=0)
            else:
                v3 = jnp.concatenate([jnp.where(row8 == 0, 1.0, v3[0:8]), v3[8:24]], axis=0)
            o = _dot(v3, p)
            if t > 0:
                o = o + acc[i]
            acc[i] = o
            if t == j:
                h = 4 * w + i
                if ROT[i]:
                    o = pltpu.roll(o, T - ROT[i] * QT, 1)
                den = o[23:24] if i < 3 else o[0:1]
                inv = pl.reciprocal(den, approx=True)
                res = o * ((1.0 - gt[h:h + 1, :]) * (inv * (2.0 - den * inv)))
                ot[j, _span(h, DH), :] += res[2 * i:2 * i + DH]

        total, ready = 0, {}
        for w, j, mix, _, n in qk:
            total += n
            ready[w, j, mix[0]] = total
        issued, step = 0, total / len(pv)
        due = LEAD
        for piece in qk:
            scores(*piece)
            issued += piece[4]
            while True:
                w, j, i, t = pv[0]
                if issued < max(ready[w, j, 3 if t == j else i] + LAG, due):
                    break
                values(*pv.pop(0))
                due += step

        def drain():
            while pv:
                values(*pv.pop(0))
                yield

        return drain(), pv

    def memory_update(w):
        e, d = _iota((WR, WR), 0), _iota((WR, WR), 1)
        same_head = None
        for i in range(4):
            m = (d >= DH * i) & (d < DH * (i + 1)) & (e >= DH * i) & (e < DH * (i + 1))
            same_head = m if same_head is None else same_head | m
        rows = _span(w, WR)
        ksum = (pk[0, rows, :] + pk[1, rows, :]) + (pk[2, rows, :] + pk[3, rows, :])
        zmem[rows, :] += jnp.broadcast_to(jnp.sum(ksum, axis=1, keepdims=True), (WR, T))
        return jnp.where(same_head, _dot(_wide(vs, 0, rows), _wide(pk, 0, rows), NT), 0.0)

    def memory_scale(w, n, phi_q):
        prod = phi_q * zmem[_span(w, WR), :]
        r8 = _iota((8, T), 0)
        den = gate = jnp.zeros((8, T), F32)
        for i in range(4):
            part = None
            for b in range(DH * i // 8, (DH * (i + 1) + 7) // 8):
                blk = prod[_span(b, 8)]
                if 8 * b < DH * i:
                    blk = jnp.where(r8 >= DH * i - 8 * b, blk, 0.0)
                elif 8 * b + 8 > DH * (i + 1):
                    blk = jnp.where(r8 < DH * (i + 1) - 8 * b, blk, 0.0)
                part = blk if part is None else part + blk
            den = jnp.where(r8 == i, jnp.sum(part, axis=0, keepdims=True), den)
            gate = jnp.where(r8 == i, gt[4 * w + i:4 * w + i + 1, :], gate)
        ms[n, w] = gate / (den + 1e-6)

    def memory_read(w):
        num = _dot(mem[w], _wide(pq, 0, _span(w, WR)))
        for n in range(NTL):
            scale, blocks = ms[n, w], []
            for b in range(WR // 8):
                lo, hi = 8 * b // DH, (8 * b + 7) // DH
                c = scale[lo:lo + 1]
                if hi != lo:
                    c = jnp.where(_iota((8, T), 0) < hi * DH - 8 * b, c, scale[hi:hi + 1])
                blocks.append(num[_span(b, 8), _span(n, T)] * c)
            ot[n, _span(w, WR), :] = jnp.concatenate(blocks, axis=0)

    def save_heads(s, g):
        for n in range(NTL):
            ob[s * NTL + n, _span(g, GR // 2), :] = _pack(ot[n, _span(g, GR), :])

    def next_segment(outstanding):
        for w in range(NW):
            update = memory_update(w)
            yield
            mem[w] += update
        for i, g, reads in ((0, 0, ()), (1, 0, (0,)), (0, 1, (1,)), (1, 1, (2,)), (0, 2, (3,)), (1, 2, ()),
                            (0, 3, ()), (1, 3, (4, 5, 6, 7))):
            yield from project(i, g, finish_k if i else finish_q, xs)
            if i == 0:
                assert not outstanding
                save_heads(NSEG - 2, g)
                vs[g] = _bf(vv[g]).astype(F32)
            for w in reads:
                memory_read(w)
                yield

    _wait(x_copies[0])
    gate = jnp.broadcast_to(jax.nn.sigmoid(beta_v[...].astype(F32)).reshape(1, H), (H, H))
    gate = jnp.sum(jnp.where(_iota((H, H), 0) == _iota((H, H), 1), gate, 0.0), axis=1, keepdims=True)
    gt[...] = jnp.broadcast_to(gate, (H, T))
    wvt[D:, :] = jnp.broadcast_to(wr_v[...].astype(F32).reshape(1, D), (8, D))
    wait_x(x_copies[1], layernorm(0, range(0, 2))[1])

    def load_wk(i, after):
        wait_w(wk_copies[i], after)
        c = wk_cols[i]
        wt[(D + c.start) // 2:(D + c.stop) // 2, :] = _u(w_v[1, :, c].T)

    def first_k(g, n, r):
        finish_k(g, n, r)
        if (g, n) == (0, 1):
            load_wk(1, r)
        elif (g, n) == (2, 2):
            wait_w(wq_copies, r)
            wt[0:D // 2, :] = _u(w_v[0].T)

    def first_q(g, n, r):
        finish_q(g, n, r, reads_memory=False)
        if (g, n) == (0, 3):
            wait_w(wv_copies, r)
            wvt[0:D, :] = w_v[2].T.astype(F32)
        elif (g, n) == (2, 1):
            wait_x(x_copies[2], r)

    load_wk(0, layernorm(0, range(2, 4))[1])
    for g in range(NG):
        _interleave(project(1, g, first_k, xn))
    for g in range(NG - 1):
        _interleave(project(0, g, first_q, xn))
    for s in range(NSEG):
        v = _dot(wvt[...], _bf(_wide(xn, s)))
        for n in range(NTL):
            if s:
                vv[s * NTL + n] = _pack(v[0:D, _span(n, T)])
            else:
                vs[n] = v[0:D, _span(n, T)]
        rr[:, _span(s, L)] = v[D:]
        if s < NSEG - 1:
            done = layernorm(s + 1)
        if s == 0:
            wait_x(x_copies[3], done[0])
    (r0, r1), picks = top2()
    _interleave(project(0, NG - 1, first_q, xn))
    idx = [jnp.clip(i[0, 0].astype(jnp.int32), 0, S - 1) for i in picks]

    def segment(s, y):
        _wait(ffn_copies(s))
        order()
        for n in range(NTL):
            for i in range(NSEG - 1):
                xs[i * NTL + n] = xs[(i + 1) * NTL + n]
                vv[i * NTL + n] = vv[(i + 1) * NTL + n]
            for i in range(NSEG - 2):
                ob[i * NTL + n] = ob[(i + 1) * NTL + n]
        ys = [y[:, k0:k1] for k0, k1 in KT]
        xsel = {}
        drain, outstanding = attend()
        _interleave(next_segment(outstanding), [gather(idx, xsel), drain, ffn(s, xsel, ys)])
        return jnp.concatenate(ys, axis=1)

    y = lax.fori_loop(0, NSEG - 1, segment, jnp.zeros((8, D), F32))

    _wait(wo_copies)
    row = _iota((8, D), 0)
    y = jnp.where(row < 2, y * jax.nn.sigmoid(jnp.where(row == 0, r0, r1)), 0.0)
    wot[:, 0:4 * T] = _u(w_v[3, 0:4 * T, :].T)
    y = jnp.concatenate([y, jnp.zeros((8, D), F32)], axis=0).astype(BF16)
    wot[:, 4 * T:] = _u(jnp.concatenate([w_v[3, 4 * T:D, :], y], axis=0).T)

    def project_out(rows, s, cuts=(0, NTL)):
        half = slice(rows.start // 2, rows.stop // 2)
        tok, r16 = _iota((16, L), 1) + s * L, _iota((16, L), 0)
        onehot = (((r16 == 0) & (tok == idx[0])) | ((r16 == 1) & (tok == idx[1]))).astype(F32)
        rhs = jnp.concatenate([_wide(ob, s, slice(2 * T, D // 2)), _pack(onehot)], axis=0)
        last = _dot(_bf(wot[half, 4 * T:]), _bf(rhs))
        yield
        for n in range(NTL):
            tile = s * NTL + n
            a = _dot(_bf(wot[half, 0:4 * T]), _bf(ob[tile, 0:2 * T, :])) + last[:, _span(n, T)]
            res = x_v[rows, _span(tile, T)].astype(F32) + _bf(xn[tile, half, :]).astype(F32)
            out_v[rows, _span(tile, T)] = (a + res).astype(BF16)
            if n + 1 in cuts:
                c = slice(s * L + cuts[cuts.index(n + 1) - 1] * T, (tile + 1) * T)
                out_copies.append(copy(out_v.at[rows, c], out_hbm.at[rows, c], out_sem))
                out_copies[-1].start()
            yield

    _interleave(project_out(slice(0, D), 0), [attend()[0]])
    for g in range(NG):
        save_heads(NSEG - 1, g)
    for s in range(1, NSEG - 1):
        _interleave(project_out(slice(0, D), s))
    for g in range(NG):
        _interleave(project_out(_span(g, GR), NSEG - 1, (0, NTL) if g < NG - 1 else (0, NTL - 1, NTL)))


def _kernel(*refs):
    out_copies = []
    pl.run_scoped(functools.partial(_compute, *refs, out_copies=out_copies),
                  sem=pltpu.SemaphoreType.DMA((9 + NSEG - 1,)), fence=pltpu.SemaphoreType.REGULAR)
    _wait(out_copies)


@jax.jit
def pallas_parallel_sum__memory_aug_infini_attn__moe_arch_mod__prompt_kernel(
    A_x: jax.Array,
    A_wq: jax.Array,
    A_wk: jax.Array,
    A_wv: jax.Array,
    A_wo: jax.Array,
    A_beta: jax.Array,
    B_x: jax.Array,
    B_w_r: jax.Array,
    B_w_gate: jax.Array,
    B_w_up: jax.Array,
    B_w_down: jax.Array,
):
    del B_x
    hbm = pl.BlockSpec(memory_space=pltpu.HBM)
    packed = pltpu.VMEM((S // T, D // 2, T), U32)
    segment = pltpu.VMEM((NTL, D, T), F32)
    ffn_weight = pltpu.VMEM((NSEG - 1, D, FC + T), BF16)
    out_t = pl.pallas_call(
        _kernel,
        in_specs=[hbm] * 10,
        out_specs=hbm,
        out_shape=jax.ShapeDtypeStruct((D, S), BF16),
        scratch_shapes=[
            pltpu.VMEM((H,), BF16),
            pltpu.VMEM((D,), BF16),
            pltpu.VMEM((D, S + T), BF16),
            pltpu.VMEM((5, D, D), BF16),
            ffn_weight, ffn_weight, ffn_weight,
            pltpu.VMEM((D, S + T), BF16),
            pltpu.VMEM((D, D), U32),
            pltpu.VMEM((D + 8, D), F32),
            pltpu.VMEM((D // 2, D + 16), U32),
            pltpu.VMEM((16, L), F32),
            packed, packed,
            pltpu.VMEM((NTL, H, 16, T), U32),
            pltpu.VMEM((NW, L // 2, WK), U32),
            segment, segment,
            packed, segment,
            pltpu.VMEM((8, S), F32),
            pltpu.VMEM((RING, QT, T), F32),
            segment, packed,
            pltpu.VMEM((NW, WR, WR), F32),
            pltpu.VMEM((D, T), F32),
            pltpu.VMEM((NTL, NW, 8, T), F32),
            pltpu.VMEM((H, T), F32),
            pltpu.VMEM((len(DIAG), QT, T), F32),
            pltpu.SemaphoreType.DMA,
        ],
        compiler_params=pltpu.CompilerParams(
            vmem_limit_bytes=100 * 1024 * 1024,
            flags={"XLA_TPU_RESCHEDULE_DMA_DONES": True},
        ),
        name="infini_mod",
    )(A_beta, B_w_r, A_x[0].T, A_wq, A_wk, A_wv, A_wo, B_w_gate, B_w_up, B_w_down.T)
    return out_t.T[None]
```

```python
import functools
import math

import jax
import jax.numpy as jnp
from jax import lax
import jax.experimental.pallas as pl
import jax.experimental.pallas.tpu as pltpu

S = 2048
D = 576
H = 32
DH = D // H
NSEG = 4
L = S // NSEG
F = 4608
T = 128
QT = T // 4
NTL = L // T
GH = 8
NG = H // GH
GR = GH * DH
WR = 4 * DH
NW = H // 4
WK = 80
FC = F // (NSEG - 1)
QSCALE = DH ** -0.5 * math.log2(math.e)
RING = 192
LAG = 1024
LEAD = 2800
FFN_LAG = 3

F32 = jnp.float32
BF16 = jnp.bfloat16
U32 = jnp.uint32
NN = (((1,), (0,)), ((), ()))
NT = (((1,), (1,)), ((), ()))
KT = [(k, min(k + T, D)) for k in range(0, D, T)]

ROT = (2, 0, 3, 1)
MIXES = {1: ((0, 0, 3, 0), (3, 1, 1, 1), (2, 2, 2, 3)), 2: ((0, 0, 1, 1), (3, 2, 2, 3)), 3: ((3, 0, 2, 1),)}
DIAG = [(0, (i,) * 4) for i in range(4)] + [(c, m) for c in MIXES for m in MIXES[c]]
assert all(sorted((m[p], (p - ROT[m[p]]) % 4) for cc, m in DIAG if cc == c for p in range(4))
           == [(i, a) for i in range(4) for a in range(c, 4)] for c in range(4))


def _dot(a, b, dims=NN):
    return lax.dot_general(a, b, dims, preferred_element_type=F32)


def _bf(x):
    return pltpu.bitcast(x, BF16)


def _u(x):
    return pltpu.bitcast(x, U32)


def _pack(x):
    return _u(x.astype(BF16))


def _round(x):
    return x.astype(BF16).astype(F32)


def _phi(t):
    return jnp.where(t > 0, t + 1.0, jnp.exp(t))


def _iota(shape, dim):
    return lax.broadcasted_iota(jnp.int32, shape, dim)


def _span(i, n):
    return slice(i * n, (i + 1) * n)


def _wide(ref, s, rows=slice(None)):
    return jnp.concatenate([ref[s * NTL + n, rows, :] for n in range(NTL)], axis=1)


def _start(copies):
    for c in copies:
        c.start()


def _wait(copies):
    for c in copies:
        c.wait()


def _interleave(main, fillers=(), per_step=4):
    fillers = list(fillers)
    for _ in main:
        for _ in range(per_step):
            while fillers and next(fillers[0], "done") == "done":
                fillers.pop(0)
    for f in fillers:
        for _ in f:
            pass


def _attention_schedule():
    qk, pv = [], []
    for w in range(NW):
        for j in (0, 2, 1, 3):
            qk += [(w, j, m, j * T + c * QT, QT) for c, m in DIAG[4:]]
            for i in range(4):
                qk += [(w, j, (i,) * 4, j * T, QT)] + [(w, j, (i,) * 4, t * T, T) for t in range(j)]
            pv += [(w, j, i, t) for i in range(4) for t in range(j)] + [(w, j, i, j) for i in range(4)]
    return qk, pv


def _compute(beta_hbm, wr_hbm, x_hbm, wq_hbm, wk_hbm, wv_hbm, wo_hbm, wg_hbm, wu_hbm, wd_hbm, out_hbm,
             beta_v, wr_v, x_v, w_v, wg_v, wu_v, wd_v, out_v, wt, wvt, wot, stat, xn, xs, qs, kn, pk,
             vv, vs, rr, sc, ot, ob, mem, zmem, gt, bias, out_sem, *, out_copies, sem, fence):
    copy = pltpu.make_async_copy
    x_cols = [slice(0, L // 2), slice(L // 2, L), _span(1, L), slice(2 * L, S)]
    x_copies = [[copy(x_hbm.at[:, c], x_v.at[:, c], sem.at[i])] for i, c in enumerate(x_cols)]
    x_copies[0] = [copy(beta_hbm, beta_v, sem.at[0]), copy(wr_hbm, wr_v, sem.at[0])] + x_copies[0]
    wk_cols = [slice(0, 2 * T), slice(2 * T, D)]
    wk_copies = [[copy(wk_hbm.at[:, c], w_v.at[1, :, c], sem.at[4 + i])] for i, c in enumerate(wk_cols)]
    wq_copies = [copy(wq_hbm, w_v.at[0], sem.at[6])]
    wv_copies = [copy(wv_hbm, w_v.at[2], sem.at[7])]
    wo_copies = [copy(wo_hbm, w_v.at[3], sem.at[8])]

    def ffn_copies(i):
        c = _span(i, FC) if isinstance(i, int) else pl.ds(pl.multiple_of(i * FC, T), FC)
        return [copy(a.at[:, c], b.at[i, :, 0:FC], sem.at[9 + i])
                for a, b in ((wg_hbm, wg_v), (wu_hbm, wu_v), (wd_hbm, wd_v))]

    def order():
        pl.semaphore_signal(fence, 1)
        pl.semaphore_wait(fence, 1)

    def wait_w(copies, after):
        w_v[4, 0:16, 0:T] = jnp.broadcast_to(after[0:1], (16, T)).astype(BF16)
        _wait(copies)

    def wait_x(copies, after):
        x_v[0:16, S:S + T] = jnp.broadcast_to(after[0:1], (16, T)).astype(BF16)
        _wait(copies)

    for stage in (x_copies[0], x_copies[1], wk_copies[0], wk_copies[1], wq_copies, wv_copies, x_copies[2],
                  x_copies[3], ffn_copies(0), ffn_copies(1), ffn_copies(2), wo_copies):
        _start(stage)
        order()

    key, lane = _iota((QT, T), 0), _iota((QT, T), 1)
    for n, (c, mix) in enumerate(DIAG):
        hidden = key > lane % QT
        on_diag = [p for p in range(4) if (p - ROT[mix[p]]) % 4 == c]
        if len(on_diag) < 4:
            hidden = hidden & ((lane // QT == on_diag[0]) | (lane // QT == on_diag[-1]))
        bias[n] = jnp.where(hidden, -jnp.inf, 0.0)
    mem[...] = jnp.zeros(mem.shape, F32)
    zmem[...] = jnp.zeros(zmem.shape, F32)
    ob[NTL:3 * NTL] = jnp.zeros((2 * NTL, D // 2, T), U32)
    order()

    def layernorm(s, tiles=range(NTL)):
        def chunks(n):
            for r in range(0, D, 16):
                yield r, x_v[r:r + 16, _span(s * NTL + n, T)].astype(F32)

        def mean_of(parts):
            a = b = None
            for part in parts:
                a = part[0:8] if a is None else a + part[0:8]
                b = part[8:16] if b is None else b + part[8:16]
            return jnp.broadcast_to(jnp.sum(a + b, axis=0, keepdims=True) * (1.0 / D), (8, T))

        for n in tiles:
            stat[0:8, _span(n, T)] = mean_of(x for _, x in chunks(n))
        for n in tiles:
            mean = stat[0:1, _span(n, T)]
            var = mean_of(jnp.square(x - mean) for _, x in chunks(n))
            sd = _round(jnp.sqrt(_round(_round(var) + _round(jnp.full((8, T), 1e-5, F32)))))
            stat[8:16, _span(n, T)] = 1.0 / sd
        for n in tiles:
            mean, inv = _round(stat[0:1, _span(n, T)]), stat[8:9, _span(n, T)]
            for r, x in chunks(n):
                last = _round(x - mean) * inv
                y = _pack(last)
                xn[s * NTL + n, r // 2:r // 2 + 8, :] = y
                if s:
                    xs[s * NTL + n, r // 2:r // 2 + 8, :] = y
        return inv, last

    pq, ms, zs = {}, {}, {}

    def finish_q(g, n, q):
        qb = _pack(q * QSCALE)
        r16 = _iota((16, T), 0)
        for hg in range(GH):
            q2 = qb[8 * hg:8 * hg + 16]
            q2 = pltpu.roll(q2, ROT[hg % 4] * QT, 1) if ROT[hg % 4] else q2
            qs[n, g * GH + hg] = jnp.where((r16 >= hg) & (r16 < hg + DH // 2), q2, jnp.zeros((16, T), U32))
        phi_q = _phi(q)
        for w in (2 * g, 2 * g + 1):
            pq[n, w] = phi_q[_span(w % 2, WR)]
            ms[n, w] = memory_scale(w, pq[n, w])

    def finish_k(g, n, k):
        pk[n, _span(g, GR), :] = _phi(k)
        for w in range(2):
            r0 = w * (GR - WK)
            kn[2 * g + w, _span(n, T // 2), :] = _u(k[r0:r0 + WK].astype(BF16).T)

    def project(i, g, finish, src):
        rows = _span(i * NG + g, GR // 2)
        last = _dot(_bf(wt[rows, 4 * T:D]), _bf(_wide(src, 0, slice(2 * T, D // 2))))
        yield
        for n in range(NTL):
            r = _dot(_bf(wt[rows, 0:4 * T]), _bf(src[n, 0:2 * T, :])) + last[:, _span(n, T)]
            yield
            finish(g, n, r)

    def top2():
        r = _round(rr[...])
        pos = _iota((8, S), 1).astype(F32)
        r0 = jnp.max(r, axis=1, keepdims=True)
        i0 = jnp.min(jnp.where(r == r0, pos, float(S)), axis=1, keepdims=True)
        r1 = jnp.max(jnp.where(pos == i0, -jnp.inf, r), axis=1, keepdims=True)
        i1 = jnp.min(jnp.where((r == r1) & (pos != i0), pos, float(S)), axis=1, keepdims=True)
        return (r0, r1), (i0, i1)

    def gather(idx, xsel):
        for t in range(2):
            tile = idx[t] // T
            onehot = ((_iota((8, T), 0) == t) & (_iota((8, T), 1) == idx[t] - tile * T)).astype(F32)
            for q, (k0, k1) in enumerate(KT):
                part = _dot(onehot, _bf(xn[tile, k0 // 2:k1 // 2, :]), NT)
                xsel[q] = xsel[q] + part if t else part
                yield

    def ffn(i, xsel, ys):
        hid = {}
        for f in range(FC // T + FFN_LAG):
            if f < FC // T:
                ab = []
                for w in (wg_v, wu_v):
                    a = None
                    for q, (k0, k1) in enumerate(KT):
                        d = _dot(xsel[q], w[i, k0:k1, _span(f, T)])
                        a = d if a is None else a + d
                        yield
                    ab.append(a)
                hid[f] = ab[0] * jax.nn.sigmoid(ab[0]) * ab[1]
            if f >= FFN_LAG:
                h = hid.pop(f - FFN_LAG)
                for q, (k0, k1) in enumerate(KT):
                    ys[q] = ys[q] + _dot(h, wd_v[i, k0:k1, _span(f - FFN_LAG, T)], NT)
                    yield

    def attend():
        qk, pv = _attention_schedule()
        row8 = _iota((8, T), 0)
        qrows, mx, acc, slot, mixed = {}, {}, {}, {}, {}

        def lanes(mix, i, rows):
            grp = _iota((rows, T), 1) // QT
            own = [p for p in range(4) if mix[p] == i]
            if len(own) == 3:
                return grp != [p for p in range(4) if p not in own][0]
            return (grp == own[0]) | (grp == own[-1])

        def q_operand(mix):
            blocks = []
            for r in range(max(mix) + 2):
                blk = jnp.zeros((8, T), U32)
                for i in (r - 1, r):
                    if i in mix:
                        part = qrows[i][_span(r - i, 8)]
                        blk = part if len(set(mix)) == 1 else jnp.where(lanes(mix, i, 8), part, blk)
                blocks.append(blk)
            return _bf(jnp.concatenate(blocks, axis=0))

        def scores(w, j, mix, k0, n):
            if mix == DIAG[4][1]:
                for i in range(4):
                    qrows[i] = qs[j, 4 * w + i]
            rhs = q_operand(mix)
            z = _dot(_bf(kn[w, k0 // 2:(k0 + n) // 2, 0:rhs.shape[0]]), rhs)
            m8 = None
            for b in range(n // QT):
                zb = z[_span(b, QT)]
                key = k0 + b * QT
                if key >= j * T:
                    zb = zb + bias[DIAG.index(((key - j * T) // QT, mix))]
                slot[w, j, mix, key] = len(slot)
                sc[slot[w, j, mix, key] % RING] = zb
                for rb in range(QT // 8):
                    m8 = zb[_span(rb, 8)] if m8 is None else jnp.maximum(m8, zb[_span(rb, 8)])
            for i in sorted(set(mix)):
                mi = m8 if len(set(mix)) == 1 else jnp.where(lanes(mix, i, 8), m8, -jnp.inf)
                mx[w, j, i] = jnp.maximum(mx[w, j, i], mi) if (w, j, i) in mx else mi
            if len(set(mix)) == 1 and (j == 0 or k0 + n == j * T):
                mx[w, j, mix[0]] = jnp.max(mx[w, j, mix[0]], axis=0, keepdims=True)

        def probs(w, j, mix, key):
            heads = sorted(set(mix))
            assert len(slot) - slot[w, j, mix, key] <= RING and all(mx[w, j, i].shape[0] == 1 for i in heads)
            m = mx[w, j, heads[0]]
            for i in heads[1:]:
                m = jnp.where(lanes(mix, i, 1), mx[w, j, i], m)
            return jnp.exp2(sc[slot[w, j, mix, key] % RING] - m)

        def values(w, j, i, t):
            own = (i,) * 4
            if t < j:
                p = jnp.concatenate([probs(w, j, own, t * T + c * QT) for c in range(4)], axis=0).astype(BF16)
            else:
                parts = [probs(w, j, own, j * T)]
                for c in MIXES:
                    part = jnp.zeros((QT, T), F32)
                    for m in MIXES[c]:
                        if i in m:
                            if (w, j, m) not in mixed:
                                mixed[w, j, m] = probs(w, j, m, j * T + c * QT)
                            part = jnp.where(lanes(m, i, QT), mixed[w, j, m], part)
                    parts.append(part)
                p = jnp.concatenate(parts, axis=0).astype(BF16)
            v3 = vs[t, w * WR + 16 * i:w * WR + 16 * i + 24, :]
            if i < 3:
                v3 = jnp.concatenate([v3[0:16], jnp.where(row8 == 7, 1.0, v3[16:24])], axis=0)
            else:
                v3 = jnp.concatenate([jnp.where(row8 == 0, 1.0, v3[0:8]), v3[8:24]], axis=0)
            o = _dot(v3, p)
            if t > 0:
                o = o + acc[i]
            acc[i] = o
            if t == j:
                h = 4 * w + i
                if ROT[i]:
                    o = pltpu.roll(o, T - ROT[i] * QT, 1)
                den = o[23:24] if i < 3 else o[0:1]
                res = o * ((1.0 - gt[h:h + 1, :]) / den)
                ot[j, _span(h, DH), :] += res[2 * i:2 * i + DH]

        total, ready = 0, {}
        for w, j, mix, _, n in qk:
            total += n
            ready[w, j, mix[0]] = total
        issued, step = 0, total / len(pv)
        due = LEAD
        for piece in qk:
            scores(*piece)
            issued += piece[4]
            while True:
                w, j, i, t = pv[0]
                if issued < max(ready[w, j, 3 if t == j else i] + LAG, due):
                    break
                values(*pv.pop(0))
                due += step

        def drain():
            while pv:
                values(*pv.pop(0))
                yield

        return drain(), pv

    def memory_update(w):
        e, d = _iota((WR, WR), 0), _iota((WR, WR), 1)
        same_head = None
        for i in range(4):
            m = (d >= DH * i) & (d < DH * (i + 1)) & (e >= DH * i) & (e < DH * (i + 1))
            same_head = m if same_head is None else same_head | m
        rows = _span(w, WR)
        ksum = (pk[0, rows, :] + pk[1, rows, :]) + (pk[2, rows, :] + pk[3, rows, :])
        zs[w] = zmem[rows, :] + jnp.broadcast_to(jnp.sum(ksum, axis=1, keepdims=True), (WR, T))
        zmem[rows, :] = zs[w]
        return jnp.where(same_head, _dot(_wide(vs, 0, rows), _wide(pk, 0, rows), NT), 0.0)

    def memory_scale(w, phi_q):
        prod = phi_q * (zs[w] if w in zs else zmem[_span(w, WR), :])
        r8 = _iota((8, T), 0)
        den = gate = jnp.zeros((8, T), F32)
        for i in range(4):
            part = None
            for b in range(DH * i // 8, (DH * (i + 1) + 7) // 8):
                blk = prod[_span(b, 8)]
                if 8 * b < DH * i:
                    blk = jnp.where(r8 >= DH * i - 8 * b, blk, 0.0)
                elif 8 * b + 8 > DH * (i + 1):
                    blk = jnp.where(r8 < DH * (i + 1) - 8 * b, blk, 0.0)
                part = blk if part is None else part + blk
            den = jnp.where(r8 == i, jnp.sum(part, axis=0, keepdims=True), den)
            gate = jnp.where(r8 == i, gt[4 * w + i:4 * w + i + 1, :], gate)
        return gate / (den + 1e-6)

    def memory_read(w):
        num = _dot(mem[w], jnp.concatenate([pq.pop((n, w)) for n in range(NTL)], axis=1))
        for n in range(NTL):
            scale, blocks = ms.pop((n, w)), []
            for b in range(WR // 8):
                lo, hi = 8 * b // DH, (8 * b + 7) // DH
                c = scale[lo:lo + 1]
                if hi != lo:
                    c = jnp.where(_iota((8, T), 0) < hi * DH - 8 * b, c, scale[hi:hi + 1])
                blocks.append(num[_span(b, 8), _span(n, T)] * c)
            ot[n, _span(w, WR), :] = jnp.concatenate(blocks, axis=0)

    def save_heads(s, g):
        for n in range(NTL):
            ob[s * NTL + n, _span(g, GR // 2), :] = _pack(ot[n, _span(g, GR), :])

    def next_segment(outstanding):
        for w in range(NW):
            update = memory_update(w)
            yield
            mem[w] += update
        for i, g, reads in ((0, 0, ()), (1, 0, (0,)), (0, 1, (1,)), (1, 1, (2,)), (1, 2, (3,)), (1, 3, ()),
                            (0, 2, ()), (0, 3, (4, 5, 6, 7))):
            yield from project(i, g, finish_k if i else finish_q, xs)
            if i == 0:
                assert not outstanding
                save_heads(NSEG - 2, g)
                vs[g] = _bf(vv[NTL + g]).astype(F32)
                for q in range(1, NSEG - 1):
                    vv[q * NTL + g] = vv[(q + 1) * NTL + g]
            for w in reads:
                memory_read(w)
                yield

    _wait(x_copies[0])
    gate = jnp.broadcast_to(jax.nn.sigmoid(beta_v[...].astype(F32)).reshape(1, H), (H, H))
    gate = jnp.sum(jnp.where(_iota((H, H), 0) == _iota((H, H), 1), gate, 0.0), axis=1, keepdims=True)
    gt[...] = jnp.broadcast_to(gate, (H, T))
    wvt[D:, :] = jnp.broadcast_to(wr_v[...].astype(F32).reshape(1, D), (8, D))
    wait_x(x_copies[1], layernorm(0, range(0, 2))[1])

    def load_wk(i, after):
        wait_w(wk_copies[i], after)
        c = wk_cols[i]
        wt[(D + c.start) // 2:(D + c.stop) // 2, :] = _u(w_v[1, :, c].T)

    def first_k(g, n, r):
        finish_k(g, n, r)
        if (g, n) == (0, 1):
            load_wk(1, r)
        elif (g, n) == (2, 2):
            wait_w(wq_copies, r)
            wt[0:D // 2, :] = _u(w_v[0].T)

    def first_q(g, n, r):
        finish_q(g, n, r)
        if (g, n) == (0, 3):
            wait_w(wv_copies, r)
            wvt[0:D, :] = w_v[2].T.astype(F32)
        elif (g, n) == (2, 1):
            wait_x(x_copies[2], r)

    load_wk(0, layernorm(0, range(2, 4))[1])
    for g in range(NG):
        _interleave(project(1, g, first_k, xn))
    for g in range(NG - 1):
        _interleave(project(0, g, first_q, xn))
    for w in range(3):
        memory_read(w)
    for s in range(NSEG):
        v = _dot(wvt[...], _bf(_wide(xn, s)))
        for n in range(NTL):
            if s:
                vv[s * NTL + n] = _pack(v[0:D, _span(n, T)])
            else:
                vs[n] = v[0:D, _span(n, T)]
        rr[:, _span(s, L)] = v[D:]
        if s < NSEG - 1:
            done = layernorm(s + 1)
        if s == 0:
            wait_x(x_copies[3], done[0])
    (r0, r1), picks = top2()
    _interleave(project(0, NG - 1, first_q, xn))
    for w in range(3, NW):
        memory_read(w)
    idx = [jnp.clip(i[0, 0].astype(jnp.int32), 0, S - 1) for i in picks]

    def segment(s, y):
        _wait(ffn_copies(s))
        order()
        for n in range(NTL):
            for i in range(NSEG - 1):
                xs[i * NTL + n] = xs[(i + 1) * NTL + n]
            for i in range(NSEG - 2):
                ob[i * NTL + n] = ob[(i + 1) * NTL + n]
        ys = [y[:, k0:k1] for k0, k1 in KT]
        xsel = {}
        drain, outstanding = attend()
        _interleave(next_segment(outstanding), [gather(idx, xsel), drain, ffn(s, xsel, ys)])
        return jnp.concatenate(ys, axis=1)

    y = lax.fori_loop(0, NSEG - 1, segment, jnp.zeros((8, D), F32))

    _wait(wo_copies)
    row = _iota((8, D), 0)
    y = jnp.where(row < 2, y * jax.nn.sigmoid(jnp.where(row == 0, r0, r1)), 0.0)
    wot[:, 0:4 * T] = _u(w_v[3, 0:4 * T, :].T)
    y = jnp.concatenate([y, jnp.zeros((8, D), F32)], axis=0).astype(BF16)
    wot[:, 4 * T:] = _u(jnp.concatenate([w_v[3, 4 * T:D, :], y], axis=0).T)

    def project_out(rows, s, cuts=(0, NTL)):
        half = slice(rows.start // 2, rows.stop // 2)
        tok, r16 = _iota((16, L), 1) + s * L, _iota((16, L), 0)
        onehot = (((r16 == 0) & (tok == idx[0])) | ((r16 == 1) & (tok == idx[1]))).astype(F32)
        rhs = jnp.concatenate([_wide(ob, s, slice(2 * T, D // 2)), _pack(onehot)], axis=0)
        last = _dot(_bf(wot[half, 4 * T:]), _bf(rhs))
        yield
        for n in range(NTL):
            tile = s * NTL + n
            a = _dot(_bf(wot[half, 0:4 * T]), _bf(ob[tile, 0:2 * T, :])) + last[:, _span(n, T)]
            res = x_v[rows, _span(tile, T)].astype(F32) + _bf(xn[tile, half, :]).astype(F32)
            out_v[rows, _span(tile, T)] = (a + res).astype(BF16)
            if n + 1 in cuts:
                c = slice(s * L + cuts[cuts.index(n + 1) - 1] * T, (tile + 1) * T)
                out_copies.append(copy(out_v.at[rows, c], out_hbm.at[rows, c], out_sem))
                out_copies[-1].start()
            yield

    _interleave(project_out(slice(0, D), 0), [attend()[0]])
    for g in range(NG):
        save_heads(NSEG - 1, g)
    for s in range(1, NSEG - 1):
        _interleave(project_out(slice(0, D), s))
    for g in range(NG):
        _interleave(project_out(_span(g, GR), NSEG - 1, (0, NTL) if g < NG - 1 else (0, NTL - 1, NTL)))


def _kernel(*refs):
    out_copies = []
    pl.run_scoped(functools.partial(_compute, *refs, out_copies=out_copies),
                  sem=pltpu.SemaphoreType.DMA((9 + NSEG - 1,)), fence=pltpu.SemaphoreType.REGULAR)
    _wait(out_copies)


@jax.jit
def pallas_parallel_sum__memory_aug_infini_attn__moe_arch_mod__prompt_kernel(
    A_x: jax.Array,
    A_wq: jax.Array,
    A_wk: jax.Array,
    A_wv: jax.Array,
    A_wo: jax.Array,
    A_beta: jax.Array,
    B_x: jax.Array,
    B_w_r: jax.Array,
    B_w_gate: jax.Array,
    B_w_up: jax.Array,
    B_w_down: jax.Array,
):
    del B_x
    hbm = pl.BlockSpec(memory_space=pltpu.HBM)
    packed = pltpu.VMEM((S // T, D // 2, T), U32)
    segment = pltpu.VMEM((NTL, D, T), F32)
    ffn_weight = pltpu.VMEM((NSEG - 1, D, FC + T), BF16)
    out_t = pl.pallas_call(
        _kernel,
        in_specs=[hbm] * 10,
        out_specs=hbm,
        out_shape=jax.ShapeDtypeStruct((D, S), BF16),
        scratch_shapes=[
            pltpu.VMEM((H,), BF16),
            pltpu.VMEM((D,), BF16),
            pltpu.VMEM((D, S + T), BF16),
            pltpu.VMEM((5, D, D), BF16),
            ffn_weight, ffn_weight, ffn_weight,
            pltpu.VMEM((D, S + T), BF16),
            pltpu.VMEM((D, D), U32),
            pltpu.VMEM((D + 8, D), F32),
            pltpu.VMEM((D // 2, D + 16), U32),
            pltpu.VMEM((16, L), F32),
            packed, packed,
            pltpu.VMEM((NTL, H, 16, T), U32),
            pltpu.VMEM((NW, L // 2, WK), U32),
            segment,
            packed, segment,
            pltpu.VMEM((8, S), F32),
            pltpu.VMEM((RING, QT, T), F32),
            segment, packed,
            pltpu.VMEM((NW, WR, WR), F32),
            pltpu.VMEM((D, T), F32),
            pltpu.VMEM((H, T), F32),
            pltpu.VMEM((len(DIAG), QT, T), F32),
            pltpu.SemaphoreType.DMA,
        ],
        compiler_params=pltpu.CompilerParams(
            vmem_limit_bytes=100 * 1024 * 1024,
            flags={"XLA_TPU_RESCHEDULE_DMA_DONES": True},
        ),
        name="infini_mod",
    )(A_beta, B_w_r, A_x.reshape(S, D).T, A_wq, A_wk, A_wv, A_wo, B_w_gate, B_w_up, B_w_down.T)
    return out_t.T.reshape(1, S, D)
```
